```python
import jax
import jax.numpy as jnp

def _softmax(x, axis=-1):
    return jax.nn.softmax(x, axis=axis)
def _gelu(x):
    return jax.nn.gelu(x, approximate=True)
def _silu(x):
    return jax.nn.silu(x)
def _sigmoid(x):
    return jax.nn.sigmoid(x)
def _layernorm(x, axis=-1, eps=1e-5):
    m = jnp.mean(x, axis=axis, keepdims=True)
    v = jnp.var(x, axis=axis, keepdims=True)
    return (x - m) / jnp.sqrt(v + eps)
def _scatter_add(tgt, idx, src, axis=0):
    return tgt.at[idx].add(src)
def _segment_sum(src, seg, n):
    return jax.ops.segment_sum(src, seg, n)
class _Rng:
    def __init__(self, key):
        self._k = key
    def _next(self):
        self._k, sub = jax.random.split(self._k)
        return sub
    def normal(self, shape):
        return jax.random.normal(self._next(), shape, dtype=jnp.bfloat16)
    def randint(self, lo, hi, shape):
        return jax.random.randint(self._next(), shape, lo, hi, dtype=jnp.int32)
    def uniform(self, shape, lo=0.0, hi=1.0):
        return jax.random.uniform(self._next(), shape, jnp.bfloat16, lo, hi)
    def permutation(self, n):
        return jax.random.permutation(self._next(), n)


kernel_name = 'concat_heads__compressed_kv_cla__spectral_gfnet__prompt'

def setup_inputs():
    _rng = _Rng(jax.random.key(int.from_bytes(__import__("os").urandom(4), "little")))
    _w = (lambda a: (lambda t: t.astype(jnp.bfloat16) if jnp.issubdtype(t.dtype, jnp.floating) else t)(jnp.asarray(a)))
    def _A_setup():
        B, H, Sq, Sk, D, M = 1, 32, 2048, 2048, 128, 1024
        Dc = 4 * D
        return {
            "x": _w((lambda *s: _rng.normal(s) * 0.05)(B, Sq, M)),
            "c_kv": _w((lambda *s: _rng.normal(s) * 0.05)(B, Sk, Dc)),
            "w_q": _w((lambda *s: _rng.normal(s) * 0.05)(M, H, D) * (M ** -0.5)),
            "w_uk": _w((lambda *s: _rng.normal(s) * 0.05)(Dc, H, D) * (Dc ** -0.5)),
            "w_uv": _w((lambda *s: _rng.normal(s) * 0.05)(Dc, H, D) * (Dc ** -0.5)),
            "w_o": _w((lambda *s: _rng.normal(s) * 0.05)(H, D, M) * ((H * D) ** -0.5)),
        }
    _A_in = _A_setup()

    def _B_setup():
        B, S, D = 1, 2048, 1024
        Df = D // 2 + 1
        return {
            "x": _w((lambda *s: _rng.normal(s) * 0.05)(B, S, D)),
            "w_r": _w((lambda *s: _rng.normal(s) * 0.05)(S, Df) * 0.02),
            "w_i": _w((lambda *s: _rng.normal(s) * 0.05)(S, Df) * 0.02),
        }
    _B_in = _B_setup()

    return {
        "A_x": _A_in["x"],
        "A_c_kv": _A_in["c_kv"],
        "A_w_q": _A_in["w_q"],
        "A_w_uk": _A_in["w_uk"],
        "A_w_uv": _A_in["w_uv"],
        "A_w_o": _A_in["w_o"],
        "B_x": _B_in["x"],
        "B_w_r": _B_in["w_r"],
        "B_w_i": _B_in["w_i"],
    }

def reference(A_x, A_c_kv, A_w_q, A_w_uk, A_w_uv, A_w_o, B_x, B_w_r, B_w_i):
    def _A_ref(x, c_kv, w_q, w_uk, w_uv, w_o):
        B, Sq, M = x.shape[0], x.shape[1], x.shape[2]
        Sk = c_kv.shape[1]
        H, D = w_q.shape[1], w_q.shape[2]
        q = jnp.einsum("bqm,mhd->bhqd", x, w_q)
        k = jnp.einsum("bkc,chd->bhkd", c_kv, w_uk)
        v = jnp.einsum("bkc,chd->bhkd", c_kv, w_uv)
        scores = jnp.einsum("bhqd,bhkd->bhqk", q, k) * (D ** -0.5)
        off = Sk - Sq
        qi = jnp.arange(Sq)[:, None]
        kj = jnp.arange(Sk)[None, :]
        cmask = kj <= (qi + off)
        scores = jnp.where(cmask[None, None], scores, -1e9)
        p = _softmax(scores, axis=-1)
        ctx = jnp.einsum("bhqk,bhkd->bhqd", p, v)
        return jnp.einsum("bhqd,hdm->bqm", ctx, w_o)

    def _B_ref(x, w_r, w_i):
        B, S, D = x.shape
        X = (lambda x, axes=(-2,-1): jnp.fft.rfft2(x.astype(jnp.float32), axes=axes))(x, axes=(-2, -1))
        W = w_r + 1j * w_i
        X = X * W
        y = (lambda x, s, axes=(-2,-1): jnp.fft.irfft2(x, s=s, axes=axes).astype(jnp.bfloat16))(X, (S, D), axes=(-2, -1))
        return y

    a = _A_ref(A_x, A_c_kv, A_w_q, A_w_uk, A_w_uv, A_w_o)
    b = _B_ref(B_x, B_w_r, B_w_i)
    return jnp.concatenate([a, b], axis=-1)
```

```python
import functools
import math

import numpy as np
import jax
import jax.numpy as jnp
from jax import lax
import jax.experimental.pallas as pl
import jax.experimental.pallas.tpu as pltpu

S = 2048
M = 1024
H = 32
D = 128
C = 512
DB = 1024
DF = DB // 2 + 1

F32 = jnp.float32
BF16 = jnp.bfloat16
U32 = jnp.uint32
NT = (((1,), (1,)), ((), ()))
NEG = -1e30


def _np_bf16(a):
    return np.asarray(a, np.float32).astype(jnp.bfloat16)


def _make_consts():
    th = 2.0 * np.pi / DB
    n = np.arange(512, dtype=np.float64)[:, None] + 0.5
    k = np.arange(512, dtype=np.float64)[None, :]
    c2 = np.cos(th * n * k)
    k2 = np.arange(640, dtype=np.float64)[None, :]
    s2 = -np.sin(th * n * k2)
    s2[:, 513:] = 0.0
    jrev = np.zeros((512, 128))
    jrev[:128] = np.eye(128)[::-1]
    fwd = np.concatenate([c2, s2, jrev], axis=1)
    scale = 1.0 / (S * DB)
    kk = np.arange(512, dtype=np.float64)[:, None]
    nn = np.arange(512, dtype=np.float64)[None, :] + 0.5
    ck = np.full((512, 1), 2.0)
    ck[0] = 1.0
    ci = np.cos(th * kk * nn) * ck * scale
    ks = kk.copy()
    ks[0] = 512.0
    si = np.sin(th * ks * nn) * ck * scale
    inv = np.concatenate([ci, si], axis=1)
    q = np.arange(128, dtype=np.float64)[None, :]
    kq = np.arange(128, dtype=np.float64)[:, None]
    hs, hs_t = [], []
    for kp in range(16):
        ang = -2.0 * np.pi * q * (kp + 16 * kq) / S
        hr, hi = np.cos(ang), np.sin(ang)
        blk = np.block([[hr, -hi], [hi, hr]])
        hs.append(blk)
        hs_t.append(blk.T)
    hmat = np.concatenate(hs + hs_t, axis=0)
    return _np_bf16(fwd), _np_bf16(inv), _np_bf16(hmat)


_FWD_NP, _INV_NP, _H_NP = _make_consts()


def _dot(a, b):
    return jnp.dot(a, b, preferred_element_type=F32)


def _dot_nt(a, b):
    return lax.dot_general(a, b, NT, preferred_element_type=F32)


def _add(a, b):
    if a is None:
        return b
    if b is None:
        return a
    return a + b


def _sub(a, b):
    if b is None:
        return a
    if a is None:
        return -b
    return a - b


def _neg(a):
    return None if a is None else -a


def _scale(a, c):
    return None if a is None else a * c


def _twiddle(z, e, n, sign):
    re, im = z
    e = e % n
    if e == 0:
        return re, im
    if 4 * e == n:
        return (_neg(im), re) if sign > 0 else (im, _neg(re))
    if 2 * e == n:
        return _neg(re), _neg(im)
    if 4 * e == 3 * n:
        return (im, _neg(re)) if sign > 0 else (_neg(im), re)
    c = math.cos(2.0 * math.pi * e / n)
    s = sign * math.sin(2.0 * math.pi * e / n)
    if 8 * e % n == 0:
        r = abs(c)
        sc, ss = (1 if c > 0 else -1), (1 if s > 0 else -1)
        a = _sub(_scale_sign(re, sc), _scale_sign(im, ss))
        b = _add(_scale_sign(re, ss), _scale_sign(im, sc))
        return _scale(a, r), _scale(b, r)
    return (_sub(_scale(re, c), _scale(im, s)), _add(_scale(re, s), _scale(im, c)))


def _scale_sign(a, sgn):
    return a if sgn > 0 else _neg(a)


def _fft(zs, sign):
    n = len(zs)
    if n == 1:
        return [zs[0]]
    ev = _fft(zs[0::2], sign)
    od = _fft(zs[1::2], sign)
    out = [None] * n
    for k in range(n // 2):
        t = _twiddle(od[k], k, n, sign)
        out[k] = (_add(ev[k][0], t[0]), _add(ev[k][1], t[1]))
        out[k + n // 2] = (_sub(ev[k][0], t[0]), _sub(ev[k][1], t[1]))
    return out


def _lo_half(w):
    return pltpu.bitcast(w << 16, F32)


def _hi_half(w):
    return pltpu.bitcast(w & jnp.uint32(0xFFFF0000), F32)


def _interleave(gens):
    live = list(gens)
    while live:
        nxt = []
        for g in live:
            try:
                next(g)
                nxt.append(g)
            except StopIteration:
                pass
        live = nxt


def _drain(g):
    for _ in g:
        pass


BQ = 512
RB = 256


def _kernel(x_h, c_h, wq_h, wk_h, wv_h, wo_h, xb_h, wr_h, wi_h, fwd_h, inv_h, hm_h,
            out_h,
            x_v, c_v, wq_raw, wk_raw, wv_raw, wo_v, wq_v, wk_v, wv_v,
            xb_v, wr_v, wi_v, wr5_v, wi5_v, fwd_v, inv_v, hm_v,
            xr_v, xi_v, a_buf, b_buf,
            acc_v, qa, ka, va, qb, kb, vb, s_v,
            sems, osems):
    cp = {}
    nsem = [0]

    def start(name, src, dst):
        c = pltpu.make_async_copy(src, dst, sems.at[nsem[0]])
        nsem[0] += 1
        c.start()
        cp[name] = c

    start("xb0", xb_h.at[0:512], xb_v.at[0:512])
    start("fwd", fwd_h, fwd_v)
    start("xb1", xb_h.at[512:S], xb_v.at[512:S])
    start("hm", hm_h, hm_v)
    for t in range(4):
        start(f"wr{t}", wr_h.at[:, t * 128:(t + 1) * 128], wr_v.at[t])
        start(f"wi{t}", wi_h.at[:, t * 128:(t + 1) * 128], wi_v.at[t])
    start("wr4", wr_h.at[:, 512:513], wr5_v)
    start("wi4", wi_h.at[:, 512:513], wi5_v)
    start("inv", inv_h, inv_v)
    start("wq", wq_h, wq_raw)
    start("wk", wk_h, wk_raw)
    start("wv", wv_h, wv_raw)
    start("c", c_h, c_v)
    start("x", x_h, x_v)
    start("wo", wo_h, wo_v)

    def wait(*names):
        for nm in names:
            cp[nm].wait()

    def d_fwd(rb):
        rows = slice(rb * RB, (rb + 1) * RB)
        jm = fwd_v[0:128, 1152:1280]
        rev = jnp.concatenate(
            [_dot(xb_v[rows, (7 - a) * 128:(8 - a) * 128], jm) for a in range(4)], axis=1)
        lo = xb_v[rows, 0:512].astype(F32)
        xe = (lo + rev).astype(BF16)
        xo = (lo - rev).astype(BF16)
        xr_v[rows, :] = _dot(xe, fwd_v[:, 0:512]).astype(BF16)
        xi_v[rows, :] = _dot(xo, fwd_v[:, 512:1152]).astype(BF16)

    wait("xb0", "fwd")
    for rb in range(2):
        d_fwd(rb)
    wait("xb1")
    for rb in range(2, S // RB):
        d_fwd(rb)

    wait("hm", *[f"wr{t}" for t in range(5)], *[f"wi{t}" for t in range(5)])
    wr_v[4] = jnp.broadcast_to(wr5_v[...], (S, 128))
    wi_v[4] = jnp.broadcast_to(wi5_v[...], (S, 128))
    wr32 = wr_v.bitcast(U32)
    wi32 = wi_v.bitcast(U32)

    def s_fft(ct):
        cs = slice(ct * 128, (ct + 1) * 128)
        slot = ct % 2
        for g in range(8):
            zs = []
            for p in range(16):
                rows = slice(128 * p + 16 * g, 128 * p + 16 * g + 16)
                re = xr_v[rows, cs].astype(F32) if ct < 4 else None
                zs.append((re, xi_v[rows, cs].astype(F32)))
            outs = _fft(zs, -1)
            for kp in range(16):
                re = outs[kp][0]
                re = jnp.zeros((16, 128), F32) if re is None else re
                a_buf[slot, kp, 16 * g:16 * g + 16, :] = re.astype(BF16)
                a_buf[slot, kp, 128 + 16 * g:128 + 16 * g + 16, :] = outs[kp][1].astype(BF16)
            yield

    def s_mid(ct):
        slot = ct % 2
        for j in range(8):
            wr_w = wr32[ct, pl.ds(j, 128, stride=8), :]
            wi_w = wi32[ct, pl.ds(j, 128, stride=8), :]
            for e in range(2):
                kp = 2 * j + e
                half = _lo_half if e == 0 else _hi_half
                fr, fi = half(wr_w), half(wi_w)
                y = _dot(hm_v[kp * 256:(kp + 1) * 256, :], a_buf[slot, kp])
                yr, yi = y[0:128], y[128:256]
                z = jnp.concatenate([yr * fr - yi * fi, yr * fi + yi * fr], axis=0).astype(BF16)
                b_buf[slot, kp] = _dot(hm_v[4096 + kp * 256:4096 + (kp + 1) * 256, :], z)
            yield

    def s_ifft(ct):
        cs = slice(ct * 128, (ct + 1) * 128)
        slot = ct % 2
        for g in range(8):
            zs = [(b_buf[slot, kp, 16 * g:16 * g + 16, :],
                   b_buf[slot, kp, 128 + 16 * g:128 + 16 * g + 16, :]) for kp in range(16)]
            outs = _fft(zs, +1)
            for p in range(16):
                rows = slice(128 * p + 16 * g, 128 * p + 16 * g + 16)
                if ct < 4:
                    xr_v[rows, cs] = outs[p][0].astype(BF16)
                xi_v[rows, cs] = outs[p][1].astype(BF16)
            yield

    _drain(s_fft(0))
    for ct in range(5):
        gens = [s_mid(ct)]
        if ct + 1 < 5:
            gens.append(s_fft(ct + 1))
        if ct >= 1:
            gens.append(s_ifft(ct - 1))
        _interleave(gens)
    _drain(s_ifft(4))

    wait("inv", "wq", "wk", "wv")
    lane = lax.broadcasted_iota(jnp.int32, (RB, 128), 1)
    yb_v = xb_v

    def d_inv(rb):
        rows = slice(rb * RB, (rb + 1) * RB)
        ev = _dot(xr_v[rows, :], inv_v[:, 0:512])
        zi0 = jnp.where(lane == 0, xi_v[rows, 512:640].astype(F32),
                        xi_v[rows, 0:128].astype(F32)).astype(BF16)
        od = _dot(jnp.concatenate([zi0, xi_v[rows, 128:512]], axis=1), inv_v[:, 512:1024])
        yb_v[rows, 0:512] = (ev - od).astype(BF16)
        yh = (ev + od).astype(BF16)
        jm = fwd_v[0:128, 1152:1280]
        for a in range(4):
            yb_v[rows, (7 - a) * 128:(8 - a) * 128] = _dot(
                yh[:, a * 128:(a + 1) * 128], jm).astype(BF16)

    def relayout(raw, dst, m0, nm):
        w32 = raw.bitcast(U32)
        for j in range(H // 2):
            w = w32[pl.ds(16 * m0 + j, nm, stride=16), :]
            dst[2 * j, m0:m0 + nm, :] = _lo_half(w).astype(BF16)
            dst[2 * j + 1, m0:m0 + nm, :] = _hi_half(w).astype(BF16)

    ob = []
    for rb in range(S // RB):
        d_inv(rb)
        relayout(wq_raw, wq_v, rb * 128, 128)
        relayout(wk_raw, wk_v, rb * 64, 64)
        relayout(wv_raw, wv_v, rb * 64, 64)
        c = pltpu.make_async_copy(yb_v.at[rb * RB:(rb + 1) * RB],
                                  out_h.at[rb * RB:(rb + 1) * RB, M:M + DB], osems.at[rb])
        c.start()
        ob.append(c)
    acc_v[...] = jnp.zeros(acc_v.shape, F32)

    wait("c", "x", "wo")
    nq = S // BQ
    nsub = BQ // 128
    row = lax.broadcasted_iota(jnp.int32, (128, 128), 0)
    col = lax.broadcasted_iota(jnp.int32, (128, 128), 1)
    tri = col <= row
    qscale = (D ** -0.5) * math.log2(math.e)

    def mx(a, b):
        return b if a is None else jnp.maximum(a, b)

    class St:
        pass

    def proj_steps(h, qd, kd, vd, pm=256):
        for i in range(S // pm):
            rows = slice(i * pm, (i + 1) * pm)
            qd[rows, :] = (_dot(x_v[rows, :], wq_v[h]) * qscale).astype(BF16)
            yield
            kd[rows, :] = _dot(c_v[rows, :], wk_v[h]).astype(BF16)
            vd[rows, :] = _dot(c_v[rows, :], wv_v[h]).astype(BF16)
            yield

    def qk_steps(i, st, qs, ks, kw=2):
        r0 = i * BQ
        st.sv = s_v.at[:, pl.ds(BQ * i * (i + 1) // 2, (i + 1) * BQ)]
        ntf = r0 // 128
        msub = [None] * nsub
        kt = 0
        while kt < ntf:
            w = min(kw, ntf - kt)
            s = _dot_nt(qs[r0:r0 + BQ, :], ks[kt * 128:(kt + w) * 128, :])
            st.sv[:, kt * 128:(kt + w) * 128] = s
            for u in range(nsub):
                for j in range(w):
                    msub[u] = mx(msub[u], s[u * 128:(u + 1) * 128, j * 128:(j + 1) * 128])
            kt += w
            yield
        for t in range(nsub):
            s = _dot_nt(qs[r0 + t * 128:r0 + BQ, :], ks[r0 + t * 128:r0 + (t + 1) * 128, :])
            s0 = jnp.where(tri, s[:128], NEG)
            s = jnp.concatenate([s0, s[128:]], axis=0) if t < nsub - 1 else s0
            st.sv[t * 128:, r0 + t * 128:r0 + (t + 1) * 128] = s
            for u in range(t, nsub):
                msub[u] = mx(msub[u], s[(u - t) * 128:(u - t + 1) * 128])
            yield
        st.m = jnp.concatenate(
            [jnp.max(msub[u], axis=1, keepdims=True) for u in range(nsub)], axis=0)

    def pv_steps(i, st, vs, kw=2):
        r0 = i * BQ
        ntf = r0 // 128
        lacc = [None] * nsub
        acc = [None] * nsub
        m = st.m
        kt = 0
        while kt < ntf:
            w = min(kw, ntf - kt)
            p = jnp.exp2(st.sv[:, kt * 128:(kt + w) * 128] - m)
            for u in range(nsub):
                for j in range(w):
                    lacc[u] = _add(lacc[u], p[u * 128:(u + 1) * 128, j * 128:(j + 1) * 128])
            o = _dot(p.astype(BF16), vs[kt * 128:(kt + w) * 128, :])
            for u in range(nsub):
                acc[u] = _add(acc[u], o[u * 128:(u + 1) * 128])
            kt += w
            yield
        for t in range(nsub):
            p = jnp.exp2(st.sv[t * 128:, r0 + t * 128:r0 + (t + 1) * 128] - m[t * 128:])
            for u in range(t, nsub):
                lacc[u] = _add(lacc[u], p[(u - t) * 128:(u - t + 1) * 128])
            o = _dot(p.astype(BF16), vs[r0 + t * 128:r0 + (t + 1) * 128, :])
            for u in range(t, nsub):
                acc[u] = _add(acc[u], o[(u - t) * 128:(u - t + 1) * 128])
            yield
        l = jnp.sum(jnp.concatenate(lacc, axis=0), axis=1, keepdims=True)
        st.ctx = (jnp.concatenate(acc, axis=0) / l).astype(BF16)

    def out_steps(h, i, st, nsplit=4):
        rows = slice(i * BQ, (i + 1) * BQ)
        w = M // nsplit
        for t in range(nsplit):
            cs = slice(t * w, (t + 1) * w)
            wo = wo_v[pl.ds(pl.multiple_of(h * D, D), D), cs]
            acc_v[rows, cs] = acc_v[rows, cs] + _dot(st.ctx, wo)
            yield

    def head(h, hn, cur, nxt):
        pg = proj_steps(hn, *nxt)
        seq = list(range(nq))[::-1]
        sts = {i: St() for i in seq}
        _drain(qk_steps(seq[0], sts[seq[0]], cur[0], cur[1]))
        per = 2 * (S // 256) // nq

        def take(k):
            for _ in range(k):
                try:
                    next(pg)
                except StopIteration:
                    return
                yield

        for n, i in enumerate(seq):
            gens = []
            if n + 1 < nq:
                gens.append(qk_steps(seq[n + 1], sts[seq[n + 1]], cur[0], cur[1]))
            gens.append(pv_steps(i, sts[i], cur[2]))
            if n >= 1:
                gens.append(out_steps(h, seq[n - 1], sts[seq[n - 1]]))
            gens.append(take(per))
            _interleave(gens)
        _drain(out_steps(h, seq[-1], sts[seq[-1]]))
        _drain(pg)

    sa, sb = (qa, ka, va), (qb, kb, vb)
    _drain(proj_steps(0, *sa))

    def body(hp, carry):
        h = 2 * hp
        head(h, h + 1, sa, sb)
        head(h + 1, jnp.minimum(h + 2, H - 1), sb, sa)
        return carry

    lax.fori_loop(0, H // 2, body, 0)

    for c in ob:
        c.wait()
    oa = []
    for rb in range(S // RB):
        rows = slice(rb * RB, (rb + 1) * RB)
        yb_v[rows, :] = acc_v[rows, :].astype(BF16)
        c = pltpu.make_async_copy(yb_v.at[rows], out_h.at[rows, 0:M], osems.at[rb])
        c.start()
        oa.append(c)
    for c in oa:
        c.wait()


@jax.jit
def pallas_concat_heads__compressed_kv_cla__spectral_gfnet__prompt_kernel(
    A_x: jax.Array,
    A_c_kv: jax.Array,
    A_w_q: jax.Array,
    A_w_uk: jax.Array,
    A_w_uv: jax.Array,
    A_w_o: jax.Array,
    B_x: jax.Array,
    B_w_r: jax.Array,
    B_w_i: jax.Array,
):
    nq = S // BQ
    sq = BQ * nq * (nq + 1) // 2
    vm = pltpu.VMEM
    scratch = [
        vm((S, M), BF16), vm((S, C), BF16),
        vm((M * H, D), BF16), vm((C * H, D), BF16), vm((C * H, D), BF16),
        vm((H * D, M), BF16),
        vm((H, M, D), BF16), vm((H, C, D), BF16), vm((H, C, D), BF16),
        vm((S, DB), BF16),
        vm((5, S, 128), BF16), vm((5, S, 128), BF16),
        vm((S, 1), BF16), vm((S, 1), BF16),
        vm(_FWD_NP.shape, BF16), vm(_INV_NP.shape, BF16), vm(_H_NP.shape, BF16),
        vm((S, 512), BF16), vm((S, 640), BF16),
        vm((2, 16, 256, 128), BF16), vm((2, 16, 256, 128), F32),
        vm((S, M), F32),
    ] + [vm((S, D), BF16)] * 6 + [
        vm((BQ, sq), F32),
        pltpu.SemaphoreType.DMA((24,)),
        pltpu.SemaphoreType.DMA((8,)),
    ]
    anyspec = pl.BlockSpec(memory_space=pl.ANY)
    out = pl.pallas_call(
        _kernel,
        out_shape=jax.ShapeDtypeStruct((S, M + DB), BF16),
        in_specs=[anyspec] * 12,
        out_specs=anyspec,
        scratch_shapes=scratch,
        compiler_params=pltpu.CompilerParams(vmem_limit_bytes=120 * 1024 * 1024),
        name="mla_gfnet_fused",
    )(
        A_x.reshape(S, M), A_c_kv.reshape(S, C),
        A_w_q.reshape(M * H, D), A_w_uk.reshape(C * H, D), A_w_uv.reshape(C * H, D),
        A_w_o.reshape(H * D, M),
        B_x.reshape(S, DB), B_w_r, B_w_i,
        jnp.asarray(_FWD_NP), jnp.asarray(_INV_NP), jnp.asarray(_H_NP),
    )
    return out.reshape(1, S, M + DB)
```

```python
import math

import numpy as np
import jax
import jax.numpy as jnp
from jax import lax
import jax.experimental.pallas as pl
import jax.experimental.pallas.tpu as pltpu

S = 2048
M = 1024
H = 32
D = 128
C = 512
DB = 1024
KR = 528

F32 = jnp.float32
BF16 = jnp.bfloat16
U32 = jnp.uint32
NT = (((1,), (1,)), ((), ()))
NEG = -1e30


def _np_bf16(a):
    return np.asarray(a, np.float32).astype(jnp.bfloat16)


def _make_consts():
    th = 2.0 * np.pi / DB
    b = np.arange(128)[None, :]
    k2 = np.arange(64)[:, None]
    lf = []
    for k1 in (1, 2, 3):
        g = np.exp(-1j * th * b * (k1 + 8 * k2))
        gp = np.exp(-1j * th * b * (8 - k1 + 8 * k2))
        lf.append(np.block([[g.real, -g.imag], [g.imag, g.real],
                            [gp.real, gp.imag], [gp.imag, -gp.real]]))
    g0 = np.exp(-1j * th * b * (8 * k2))
    g4 = np.exp(-1j * th * b * (4 + 8 * k2))
    l0 = np.concatenate([g0.real, g0.imag, np.cos(th * b * 512), np.zeros((127, 128))], 0)
    l4 = np.concatenate([g4.real, g4.imag, np.zeros((128, 128))], 0)
    lf.append(np.concatenate([l0, l4], 1))
    sc = 1.0 / (S * DB)
    bb = np.arange(128)[:, None]
    kk = np.arange(64)[None, :]
    li = []
    for k1 in (1, 2, 3):
        ph, pp = th * bb * (k1 + 8 * kk), th * bb * (8 - k1 + 8 * kk)
        c, s_, cp, sp = np.cos(ph), np.sin(ph), np.cos(pp), np.sin(pp)
        li.append(2 * sc * np.block([[c, -s_, cp, -sp], [s_, c, -sp, -cp]]))
    ph = th * bb * (8 * kk)
    c0, s0 = 2 * np.cos(ph), -2 * np.sin(ph)
    c0[:, 0] = 1.0
    s0[:, 0] = np.cos(th * bb[:, 0] * 512)
    i0 = sc * np.concatenate([c0, s0], 1)
    ph = th * bb * (4 + 8 * kk)
    i4 = sc * np.concatenate([2 * np.cos(ph), -2 * np.sin(ph)], 1)
    li.append(np.concatenate([np.concatenate([i0, i4], 1), np.zeros((128, 256))], 0))
    lmat = np.concatenate(lf + li, axis=0)
    p = np.arange(128)[None, :]
    kp = np.arange(128)[:, None]
    gf, gi = [], []
    for q in range(16):
        g = np.exp(-2j * np.pi * (16 * p + q) * kp / S)
        gf.append(np.block([[g.real.T, g.imag.T], [-g.imag.T, g.real.T]]))
        gi.append(np.block([[g.real, -g.imag], [g.imag, g.real]]))
    return (_np_bf16(lmat), _np_bf16(np.concatenate(gf, 0)), _np_bf16(np.concatenate(gi, 0)))


_L_NP, _GF_NP, _GI_NP = _make_consts()


def _dot(a, b):
    return jnp.dot(a, b, preferred_element_type=F32)


def _dot_nt(a, b):
    return lax.dot_general(a, b, NT, preferred_element_type=F32)


def _t(x):
    return None if x is None else (1, x)


def _tneg(a):
    return None if a is None else (-a[0], a[1])


def _tadd(a, b):
    if a is None:
        return b
    if b is None:
        return a
    if a[0] == b[0]:
        return (a[0], a[1] + b[1])
    return (1, a[1] - b[1]) if a[0] > 0 else (1, b[1] - a[1])


def _tsub(a, b):
    return _tadd(a, _tneg(b))


def _tscale(a, c):
    return None if a is None else (1, a[1] * (c * a[0]))


def _tmul(a, v):
    return None if a is None else (a[0], a[1] * v)


def _tval(a):
    return a[1] if a[0] > 0 else -a[1]


def _twiddle(z, e, n, sign):
    re, im = z
    if e == 0:
        return re, im
    if 4 * e == n:
        return (_tneg(im), re) if sign > 0 else (im, _tneg(re))
    c = math.cos(2.0 * math.pi * e / n)
    s = sign * math.sin(2.0 * math.pi * e / n)
    if 8 * e % n == 0:
        r = abs(c)
        rc = re if c > 0 else _tneg(re)
        rs = re if s > 0 else _tneg(re)
        ic = im if c > 0 else _tneg(im)
        is_ = im if s > 0 else _tneg(im)
        return _tscale(_tsub(rc, is_), r), _tscale(_tadd(rs, ic), r)
    return (_tsub(_tscale(re, c), _tscale(im, s)), _tadd(_tscale(re, s), _tscale(im, c)))


def _fft(zs, sign):
    n = len(zs)
    if n == 1:
        return [zs[0]]
    ev = _fft(zs[0::2], sign)
    od = _fft(zs[1::2], sign)
    out = [None] * n
    for k in range(n // 2):
        t = _twiddle(od[k], k, n, sign)
        out[k] = (_tadd(ev[k][0], t[0]), _tadd(ev[k][1], t[1]))
        out[k + n // 2] = (_tsub(ev[k][0], t[0]), _tsub(ev[k][1], t[1]))
    return out


def _irfft8(t0, t4, t1, t2, t3):
    r = math.sqrt(0.5)
    a0, a1 = t0 + t4, t0 - t4
    e0, e2 = a0 + t2[0], a0 - t2[0]
    e1, e3 = a1 - t2[1], a1 + t2[1]
    o0 = t1[0] + t3[0]
    o2 = t3[1] - t1[1]
    u, v = t1[0] - t3[0], t1[1] + t3[1]
    o1, o3 = (u - v) * r, (-u - v) * r
    return [e0 + o0, e1 + o1, e2 + o2, e3 + o3, e0 - o0, e1 - o1, e2 - o2, e3 - o3]


def _lo_half(w):
    return pltpu.bitcast(w << 16, F32)


def _hi_half(w):
    return pltpu.bitcast(w & jnp.uint32(0xFFFF0000), F32)


def _pack_words(lo, hi):
    lo = pltpu.bitcast(lo.astype(BF16).astype(F32), U32)
    hi = pltpu.bitcast(hi.astype(BF16).astype(F32), U32)
    return (lo >> 16) | hi


def _interleave(gens):
    live = list(gens)
    while live:
        nxt = []
        for g in live:
            try:
                next(g)
                nxt.append(g)
            except StopIteration:
                pass
        live = nxt


def _drain(g):
    for _ in g:
        pass


BQ = 512


def _kernel(x_h, c_h, wq_h, wk_h, wv_h, wo_h, xb_h, wr_h, wi_h, l_h, gf_h, gi_h,
            out_h,
            x_v, c_v, wq_raw, wk_raw, wv_raw, wo_v, ws_q, ws_k, ws_v,
            xb_v, wr_v, wi_v, wrn_v, win_v, l_v, gf_v, gi_v,
            u_v, y_v, z_v,
            acc_v, q_v, k_v, v_v, s_v,
            sems, osems, wsems, bsems):
    cp = {}
    nsem = [0]

    def start(name, src, dst):
        c = pltpu.make_async_copy(src, dst, sems.at[nsem[0]])
        nsem[0] += 1
        c.start()
        cp[name] = c

    def wait(*names):
        for nm in names:
            cp[nm].wait()

    wq32, wk32, wv32 = wq_h.bitcast(U32), wk_h.bitcast(U32), wv_h.bitcast(U32)

    def pair_copy(t, j):
        if t == 3:
            rows = pl.ds(pl.multiple_of(j * 2 * D, 2 * D), 2 * D)
            return pltpu.make_async_copy(wo_h.at[rows], wo_v.at[rows], wsems.at[3, j])
        src, dst = ((wq32, wq_raw), (wk32, wk_raw), (wv32, wv_raw))[t]
        return pltpu.make_async_copy(src.at[:, j, :], dst.at[j], wsems.at[t, j])

    xb32 = xb_v.bitcast(U32)
    wr32 = wr_v.bitcast(U32)
    wi32 = wi_v.bitcast(U32)

    def word_rows(a, jj):
        return xb32.at[a, pl.ds(pl.multiple_of(4 * jj, 4), 1020)]

    def f1(jj, j0):
        views = [word_rows(a, jj) for a in range(8)]
        for g in range(8):
            words = [v[pl.ds(128 * g + j0, 16, stride=8), :] for v in views]
            for e in range(2):
                half = _lo_half if e == 0 else _hi_half
                o = _fft([(_t(half(w)), None) for w in words], -1)
                r0 = pl.multiple_of((8 * jj + 2 * j0 + e) * 128 + 16 * g, 16)
                parts = [o[0][0], o[4][0], o[1][0], o[1][1], o[2][0], o[2][1], o[3][0], o[3][1]]
                for t in range(8):
                    u_v[pl.ds(r0, 16), t * 128:(t + 1) * 128] = _tval(parts[t]).astype(BF16)

    def f23(q):
        rows = pl.ds(pl.multiple_of(q * 128, 128), 128)
        o = [_dot_nt(l_v[256 * i:256 * (i + 1), :], u_v[rows, 256 * (i + 1):256 * (i + 2)])
             .astype(BF16) for i in range(3)]
        o0 = _dot_nt(l_v[768:912, 0:128], u_v[rows, 0:128]).astype(BF16)
        o4 = _dot_nt(l_v[768:896, 128:256], u_v[rows, 128:256]).astype(BF16)

        def blk(k1, part):
            if k1 == 0:
                return o0[64 * part:64 * part + 64]
            if k1 == 4:
                return o4[64 * part:64 * part + 64]
            if k1 < 4:
                return o[k1 - 1][64 * part:64 * part + 64]
            return o[7 - k1][128 + 64 * part:128 + 64 * part + 64]

        re = jnp.concatenate([blk(k1, 0) for k1 in range(8)] + [o0[128:144]], axis=0)
        im = jnp.concatenate([blk(k1, 1) for k1 in range(8)] + [jnp.zeros((16, 128), BF16)],
                             axis=0)
        y_v[q] = _dot(jnp.concatenate([re, im], axis=1),
                      gf_v[pl.ds(pl.multiple_of(q * 256, 256), 256), :])

    def mid(rows, filt):
        xf = _fft([(_t(y_v[q, rows, 0:128]), _t(y_v[q, rows, 128:256])) for q in range(16)], -1)
        zs = []
        for kq in range(16):
            fr, fi = filt(kq)
            re, im = xf[kq]
            zs.append((_tsub(_tmul(re, fr), _tmul(im, fi)), _tadd(_tmul(re, fi), _tmul(im, fr))))
        us = _fft(zs, +1)
        for q in range(16):
            z_v[q, rows, 0:128] = _tval(us[q][0]).astype(BF16)
            z_v[q, rows, 128:256] = _tval(us[q][1]).astype(BF16)

    def mid_group(g2, carry):
        base = pl.multiple_of(64 * g2, 64)
        for k1 in range(8):
            half = _lo_half if k1 % 2 == 0 else _hi_half
            sl = pl.ds(k1 // 2, 16, stride=4)

            def filt(kq):
                return (half(wr32.at[kq, pl.ds(base, 64)][sl, :]),
                        half(wi32.at[kq, pl.ds(base, 64)][sl, :]))

            mid(pl.ds(pl.multiple_of(64 * k1 + 16 * g2, 16), 16), filt)
        return carry

    def mid_nyquist():
        def filt(kq):
            cs = slice(kq * 128, (kq + 1) * 128)
            return (jnp.broadcast_to(wrn_v[:, cs].astype(F32), (16, 128)),
                    jnp.broadcast_to(win_v[:, cs].astype(F32), (16, 128)))

        mid(slice(512, KR), filt)

    srow = lax.broadcasted_iota(jnp.int32, (64, 128), 0)

    def i32(jj, j0):
        ys = []
        for e in range(2):
            q = 8 * jj + 2 * j0 + e
            z = _dot(z_v[q], gi_v[pl.ds(pl.multiple_of(q * 256, 256), 256), :])
            zr, zi = z[:, 0:128], z[:, 128:256]
            zi0 = jnp.where(srow == 0, jnp.broadcast_to(zr[512:513], (64, 128)), zi[0:64])
            rhs0 = jnp.concatenate([zr[0:64], zi0], axis=0).astype(BF16)
            t0 = _dot(l_v[1792:1920, 0:128], rhs0)
            rhs4 = jnp.concatenate([zr[256:320], zi[256:320]], axis=0).astype(BF16)
            t4 = _dot(l_v[1792:1920, 128:256], rhs4)
            ts = []
            for k1 in (1, 2, 3):
                kc = 8 - k1
                rhs = jnp.concatenate([zr[64 * k1:64 * k1 + 64], zi[64 * k1:64 * k1 + 64],
                                       zr[64 * kc:64 * kc + 64], zi[64 * kc:64 * kc + 64]],
                                      axis=0).astype(BF16)
                o = _dot(l_v[1024 + 256 * (k1 - 1):1024 + 256 * k1, :], rhs)
                ts.append((o[0:128], o[128:256]))
            ys.append(_irfft8(t0, t4, *ts))
        for a in range(8):
            word_rows(a, jj)[pl.ds(j0, 128, stride=8), :] = _pack_words(ys[0][a], ys[1][a]).T

    nq = S // BQ
    nsub = BQ // 128
    row = lax.broadcasted_iota(jnp.int32, (128, 128), 0)
    col = lax.broadcasted_iota(jnp.int32, (128, 128), 1)
    tri = col <= row
    qscale = (D ** -0.5) * math.log2(math.e)

    def mx(a, b):
        return b if a is None else jnp.maximum(a, b)

    def addn(a, b):
        return b if a is None else a + b

    class St:
        pass

    def unpack_weights(h):
        j = h >> 1
        sh = jnp.asarray(16 * (1 - (h & 1))).astype(U32)
        for raw, w in ((wq_raw, ws_q), (wk_raw, ws_k), (wv_raw, ws_v)):
            w[...] = _hi_half(raw[j] << sh).astype(BF16)

    def proj_rows(slot, rows):
        q_v[slot, rows, :] = (_dot(x_v[rows, :], ws_q[...]) * qscale).astype(BF16)
        yield
        k_v[slot, rows, :] = _dot(c_v[rows, :], ws_k[...]).astype(BF16)
        v_v[slot, rows, :] = _dot(c_v[rows, :], ws_v[...]).astype(BF16)
        yield

    def proj_steps(slot, pm=256):
        for i in range(S // pm):
            yield from proj_rows(slot, slice(i * pm, (i + 1) * pm))

    def qk_steps(i, st, slot, kw=2):
        r0 = i * BQ
        st.sv = s_v.at[:, pl.ds(BQ * i * (i + 1) // 2, (i + 1) * BQ)]
        ntf = r0 // 128
        msub = [None] * nsub
        kt = 0
        while kt < ntf:
            w = min(kw, ntf - kt)
            s = _dot_nt(q_v[slot, r0:r0 + BQ, :], k_v[slot, kt * 128:(kt + w) * 128, :])
            st.sv[:, kt * 128:(kt + w) * 128] = s
            for u in range(nsub):
                for j in range(w):
                    msub[u] = mx(msub[u], s[u * 128:(u + 1) * 128, j * 128:(j + 1) * 128])
            kt += w
            yield
        for t in range(nsub):
            s = _dot_nt(q_v[slot, r0 + t * 128:r0 + BQ, :],
                        k_v[slot, r0 + t * 128:r0 + (t + 1) * 128, :])
            s0 = jnp.where(tri, s[:128], NEG)
            s = jnp.concatenate([s0, s[128:]], axis=0) if t < nsub - 1 else s0
            st.sv[t * 128:, r0 + t * 128:r0 + (t + 1) * 128] = s
            for u in range(t, nsub):
                msub[u] = mx(msub[u], s[(u - t) * 128:(u - t + 1) * 128])
            yield
        st.m = jnp.concatenate(
            [jnp.max(msub[u], axis=1, keepdims=True) for u in range(nsub)], axis=0)

    def pv_steps(i, st, slot, kw=2):
        r0 = i * BQ
        ntf = r0 // 128
        lacc = [None] * nsub
        acc = [None] * nsub
        m = st.m
        kt = 0
        while kt < ntf:
            w = min(kw, ntf - kt)
            p = jnp.exp2(st.sv[:, kt * 128:(kt + w) * 128] - m)
            for u in range(nsub):
                for j in range(w):
                    lacc[u] = addn(lacc[u], p[u * 128:(u + 1) * 128, j * 128:(j + 1) * 128])
            o = _dot(p.astype(BF16), v_v[slot, kt * 128:(kt + w) * 128, :])
            for u in range(nsub):
                acc[u] = addn(acc[u], o[u * 128:(u + 1) * 128])
            kt += w
            yield
        for t in range(nsub):
            p = jnp.exp2(st.sv[t * 128:, r0 + t * 128:r0 + (t + 1) * 128] - m[t * 128:])
            for u in range(t, nsub):
                lacc[u] = addn(lacc[u], p[(u - t) * 128:(u - t + 1) * 128])
            o = _dot(p.astype(BF16), v_v[slot, r0 + t * 128:r0 + (t + 1) * 128, :])
            for u in range(t, nsub):
                acc[u] = addn(acc[u], o[(u - t) * 128:(u - t + 1) * 128])
            yield
        l = jnp.sum(jnp.concatenate(lacc, axis=0), axis=1, keepdims=True)
        st.ctx = (jnp.concatenate(acc, axis=0) / l).astype(BF16)

    pending = []

    def out_steps(h, i, st, last, nsplit=4):
        rows = slice(i * BQ, (i + 1) * BQ)
        w = M // nsplit
        for t in range(nsplit):
            cs = slice(t * w, (t + 1) * w)
            o = acc_v[rows, cs] + _dot(st.ctx, wo_v[pl.ds(pl.multiple_of(h * D, D), D), cs])
            if last:
                u_v[rows, cs] = o.astype(BF16)
                c = pltpu.make_async_copy(u_v.at[rows, cs], out_h.at[rows, cs],
                                          osems.at[i * nsplit + t])
                c.start()
                pending.append(c)
            else:
                acc_v[rows, cs] = o
            yield

    def head(h, slot, pg, last=False):
        seq = list(range(nq))[::-1]
        sts = {i: St() for i in seq}
        _drain(qk_steps(seq[0], sts[seq[0]], slot))
        per = 2 * (S // 256) // nq

        def take(k):
            for _ in range(k):
                try:
                    next(pg)
                except StopIteration:
                    return
                yield

        for n, i in enumerate(seq):
            gens = []
            if n + 1 < nq:
                gens.append(qk_steps(seq[n + 1], sts[seq[n + 1]], slot))
            gens.append(pv_steps(i, sts[i], slot))
            if n >= 1:
                gens.append(out_steps(h, seq[n - 1], sts[seq[n - 1]], last))
            gens.append(take(per))
            _interleave(gens)
        _drain(out_steps(h, seq[-1], sts[seq[-1]], last))
        _drain(pg)

    for a in range(8):
        start(f"xb{a}", xb_h.at[:, a * 128:(a + 1) * 128], xb_v.at[a])
    start("l", l_h, l_v)
    start("gf", gf_h, gf_v)
    wait(*[f"xb{a}" for a in range(8)], "l", "gf")
    for t in range(16):
        start(f"wr{t}", wr_h.at[0:512, t * 128:(t + 1) * 128], wr_v.at[t])
        start(f"wi{t}", wi_h.at[0:512, t * 128:(t + 1) * 128], wi_v.at[t])
    start("wrn", wr_h.at[512:513, :], wrn_v)
    start("win", wi_h.at[512:513, :], win_v)
    start("gi", gi_h, gi_v)

    def fwd_half(jj, carry):
        f1(jj, 0)
        for j0 in range(4):
            if j0 + 1 < 4:
                f1(jj, j0 + 1)
            f23(8 * jj + 2 * j0)
            f23(8 * jj + 2 * j0 + 1)
        return carry

    lax.fori_loop(0, 2, fwd_half, 0)

    wait(*[f"wr{t}" for t in range(16)], *[f"wi{t}" for t in range(16)], "wrn", "win", "gi")
    start("c", c_h, c_v)
    start("x", x_h, x_v)
    for t in range(4):
        pair_copy(t, 0).start()
    lax.fori_loop(0, 4, mid_group, 0)
    mid_nyquist()

    def inv_half(jj, carry):
        for j0 in range(4):
            i32(jj, j0)
        return carry

    lax.fori_loop(0, 2, inv_half, 0)
    for a in range(8):
        c = pltpu.make_async_copy(xb_v.at[a], out_h.at[:, M + a * 128:M + (a + 1) * 128],
                                  bsems.at[a])
        c.start()
        pending.append(c)

    wait("c", "x")
    for t in range(4):
        pair_copy(t, 0).wait()
    for j in range(1, 5):
        for t in range(4):
            pair_copy(t, j).start()
    acc_v[...] = jnp.zeros(acc_v.shape, F32)
    unpack_weights(0)

    def proj0(i, carry):
        _drain(proj_rows(0, pl.ds(pl.multiple_of(i * 512, 512), 512)))
        return carry

    lax.fori_loop(0, S // 512, proj0, 0)
    for j in range(5, H // 2):
        for t in range(4):
            pair_copy(t, j).start()

    def body(h, carry):
        @pl.when((h & 1) == 1)
        def _():
            for t in range(4):
                pair_copy(t, (h + 1) >> 1).wait()

        unpack_weights(h + 1)
        head(h, h & 1, proj_steps((h + 1) & 1))
        return carry

    lax.fori_loop(0, H - 1, body, 0)
    head(H - 1, (H - 1) & 1, iter(()), last=True)
    for c in pending:
        c.wait()


@jax.jit
def pallas_concat_heads__compressed_kv_cla__spectral_gfnet__prompt_kernel(
    A_x: jax.Array,
    A_c_kv: jax.Array,
    A_w_q: jax.Array,
    A_w_uk: jax.Array,
    A_w_uv: jax.Array,
    A_w_o: jax.Array,
    B_x: jax.Array,
    B_w_r: jax.Array,
    B_w_i: jax.Array,
):
    nq = S // BQ
    sq = BQ * nq * (nq + 1) // 2
    vm = pltpu.VMEM
    scratch = [
        vm((S, M), BF16), vm((S, C), BF16),
        vm((H // 2, M, D), U32), vm((H // 2, C, D), U32), vm((H // 2, C, D), U32),
        vm((H * D, M), BF16),
        vm((M, D), BF16), vm((C, D), BF16), vm((C, D), BF16),
        vm((8, S, 128), BF16),
        vm((16, 512, 128), BF16), vm((16, 512, 128), BF16),
        vm((1, S), BF16), vm((1, S), BF16),
        vm(_L_NP.shape, BF16), vm(_GF_NP.shape, BF16), vm(_GI_NP.shape, BF16),
        vm((S, 1024), BF16),
        vm((16, KR, 256), F32), vm((16, KR, 256), BF16),
        vm((S, M), F32),
        vm((2, S, D), BF16), vm((2, S, D), BF16), vm((2, S, D), BF16),
        vm((BQ, sq), F32),
        pltpu.SemaphoreType.DMA((56,)),
        pltpu.SemaphoreType.DMA((16,)),
        pltpu.SemaphoreType.DMA((4, H // 2)),
        pltpu.SemaphoreType.DMA((8,)),
    ]
    anyspec = pl.BlockSpec(memory_space=pl.ANY)
    out = pl.pallas_call(
        _kernel,
        out_shape=jax.ShapeDtypeStruct((S, M + DB), BF16),
        in_specs=[anyspec] * 12,
        out_specs=anyspec,
        scratch_shapes=scratch,
        compiler_params=pltpu.CompilerParams(vmem_limit_bytes=122 * 1024 * 1024),
        name="mla_gfnet_fused",
    )(
        A_x.reshape(S, M), A_c_kv.reshape(S, C), A_w_q, A_w_uk, A_w_uv,
        A_w_o.reshape(H * D, M),
        B_x.reshape(S, DB), B_w_r.T, B_w_i.T,
        jnp.asarray(_L_NP), jnp.asarray(_GF_NP), jnp.asarray(_GI_NP),
    )
    return out.reshape(1, S, M + DB)
```

```python
import functools
import math

import numpy as np
import jax
import jax.numpy as jnp
from jax import lax
import jax.experimental.pallas as pl
import jax.experimental.pallas.tpu as pltpu

S = 2048
M = 1024
H = 32
D = 128
C = 512
DB = 1024
KR = 528

F32 = jnp.float32
BF16 = jnp.bfloat16
U32 = jnp.uint32
NT = (((1,), (1,)), ((), ()))
NEG = -1e30


def _np_bf16(a):
    return np.asarray(a, np.float32).astype(jnp.bfloat16)


def _make_consts():
    th = 2.0 * np.pi / DB
    b = np.arange(128)[None, :]
    k2 = np.arange(64)[:, None]
    lf = []
    for k1 in (1, 2, 3):
        g = np.exp(-1j * th * b * (k1 + 8 * k2))
        gp = np.exp(-1j * th * b * (8 - k1 + 8 * k2))
        lf.append(np.block([[g.real, -g.imag], [g.imag, g.real],
                            [gp.real, gp.imag], [gp.imag, -gp.real]]))
    g0 = np.exp(-1j * th * b * (8 * k2))
    g4 = np.exp(-1j * th * b * (4 + 8 * k2))
    l0 = np.concatenate([g0.real, g0.imag, np.cos(th * b * 512), np.zeros((127, 128))], 0)
    l4 = np.concatenate([g4.real, g4.imag, np.zeros((128, 128))], 0)
    lf.append(np.concatenate([l0, l4], 1))
    sc = 1.0 / (S * DB)
    bb = np.arange(128)[:, None]
    kk = np.arange(64)[None, :]
    li = []
    for k1 in (1, 2, 3):
        ph, pp = th * bb * (k1 + 8 * kk), th * bb * (8 - k1 + 8 * kk)
        c, s_, cp, sp = np.cos(ph), np.sin(ph), np.cos(pp), np.sin(pp)
        li.append(2 * sc * np.block([[c, -s_, cp, -sp], [s_, c, -sp, -cp]]))
    ph = th * bb * (8 * kk)
    c0, s0 = 2 * np.cos(ph), -2 * np.sin(ph)
    c0[:, 0] = 1.0
    s0[:, 0] = np.cos(th * bb[:, 0] * 512)
    i0 = sc * np.concatenate([c0, s0], 1)
    ph = th * bb * (4 + 8 * kk)
    i4 = sc * np.concatenate([2 * np.cos(ph), -2 * np.sin(ph)], 1)
    li.append(np.concatenate([np.concatenate([i0, i4], 1), np.zeros((128, 256))], 0))
    lmat = np.concatenate(lf + li, axis=0)
    p = np.arange(128)[None, :]
    kp = np.arange(128)[:, None]
    gf = []
    for q in range(16):
        g = np.exp(-2j * np.pi * (16 * p + q) * kp / S)
        gf.append(np.block([[g.real.T, g.imag.T], [-g.imag.T, g.real.T]]))
    return _np_bf16(lmat), _np_bf16(np.concatenate(gf, 0))


_L_NP, _GF_NP = _make_consts()


_dot = functools.partial(jnp.dot, preferred_element_type=F32)
_dot_nt = functools.partial(lax.dot_general, dimension_numbers=NT, preferred_element_type=F32)


def _t(x):
    return None if x is None else (1, x)


def _tneg(a):
    return None if a is None else (-a[0], a[1])


def _tadd(a, b):
    if a is None:
        return b
    if b is None:
        return a
    if a[0] == b[0]:
        return (a[0], a[1] + b[1])
    return (1, a[1] - b[1]) if a[0] > 0 else (1, b[1] - a[1])


def _tsub(a, b):
    return _tadd(a, _tneg(b))


def _tscale(a, c):
    return None if a is None else (1, a[1] * (c * a[0]))


def _tmul(a, v):
    return None if a is None else (a[0], a[1] * v)


def _tval(a):
    return a[1] if a[0] > 0 else -a[1]


def _twiddle(z, e, n, sign):
    re, im = z
    if e == 0:
        return re, im
    if 4 * e == n:
        return (_tneg(im), re) if sign > 0 else (im, _tneg(re))
    c = math.cos(2.0 * math.pi * e / n)
    s = sign * math.sin(2.0 * math.pi * e / n)
    if 8 * e % n == 0:
        r = abs(c)
        rc = re if c > 0 else _tneg(re)
        rs = re if s > 0 else _tneg(re)
        ic = im if c > 0 else _tneg(im)
        is_ = im if s > 0 else _tneg(im)
        return _tscale(_tsub(rc, is_), r), _tscale(_tadd(rs, ic), r)
    return (_tsub(_tscale(re, c), _tscale(im, s)), _tadd(_tscale(re, s), _tscale(im, c)))


def _fft(zs, sign):
    n = len(zs)
    if n == 1:
        return [zs[0]]
    ev = _fft(zs[0::2], sign)
    od = _fft(zs[1::2], sign)
    out = [None] * n
    for k in range(n // 2):
        t = _twiddle(od[k], k, n, sign)
        out[k] = (_tadd(ev[k][0], t[0]), _tadd(ev[k][1], t[1]))
        out[k + n // 2] = (_tsub(ev[k][0], t[0]), _tsub(ev[k][1], t[1]))
    return out


def _irfft8(t0, t4, t1, t2, t3):
    r = math.sqrt(0.5)
    a0, a1 = t0 + t4, t0 - t4
    e0, e2 = a0 + t2[0], a0 - t2[0]
    e1, e3 = a1 - t2[1], a1 + t2[1]
    o0 = t1[0] + t3[0]
    o2 = t3[1] - t1[1]
    u, v = t1[0] - t3[0], t1[1] + t3[1]
    o1, o3 = (u - v) * r, (-u - v) * r
    return [e0 + o0, e1 + o1, e2 + o2, e3 + o3, e0 - o0, e1 - o1, e2 - o2, e3 - o3]


def _lo_half(w):
    return pltpu.bitcast(w << 16, F32)


def _hi_half(w):
    return pltpu.bitcast(w & jnp.uint32(0xFFFF0000), F32)


def _pack_words(lo, hi):
    lo = pltpu.bitcast(lo.astype(BF16).astype(F32), U32)
    hi = pltpu.bitcast(hi.astype(BF16).astype(F32), U32)
    return (lo >> 16) | hi


def _interleave(gens):
    live = list(gens)
    while live:
        nxt = []
        for g in live:
            try:
                next(g)
                nxt.append(g)
            except StopIteration:
                pass
        live = nxt


def _drain(g):
    for _ in g:
        pass


BQ = 512
KW = 4
NSPLIT = 4
LAG_OUT = 16
F_LAG = 2
F_FILL = 1.0
SCORE_LIMIT = 60.0


def _kernel(x_h, c_h, wq_h, wk_h, wv_h, wo_h, xb_h, wr_h, wi_h, l_h, gf_h,
            out_h,
            x_v, c_v, wq_raw, wk_raw, wv_raw, wo_v, ws_q, ws_k, ws_v,
            xb_v, wr_v, wi_v, wrn_v, win_v, l_v, gf_v,
            u_v, y_v, z_v,
            acc_v, q_v, k_v, v_v, s_v, nrm_s,
            sems, osems, wsems, bsems):
    cp = {}
    nsem = [0]

    def start(name, src, dst):
        c = pltpu.make_async_copy(src, dst, sems.at[nsem[0]])
        nsem[0] += 1
        c.start()
        cp[name] = c

    def wait(*names):
        for nm in names:
            cp[nm].wait()

    wq32, wk32, wv32 = wq_h.bitcast(U32), wk_h.bitcast(U32), wv_h.bitcast(U32)

    def pair_copy(t, j):
        if t == 3:
            rows = pl.ds(pl.multiple_of(j * 2 * D, 2 * D), 2 * D)
            return pltpu.make_async_copy(wo_h.at[rows], wo_v.at[rows], wsems.at[3, j])
        src, dst = ((wq32, wq_raw), (wk32, wk_raw), (wv32, wv_raw))[t]
        return pltpu.make_async_copy(src.at[:, j, :], dst.at[j], wsems.at[t, j])

    xb32 = xb_v.bitcast(U32)
    wr32 = wr_v.bitcast(U32)
    wi32 = wi_v.bitcast(U32)

    def word_rows(a, jj):
        return xb32.at[a, pl.ds(pl.multiple_of(4 * jj, 4), 1020)]

    def f1(jj, j0):
        views = [word_rows(a, jj) for a in range(8)]
        for g in range(8):
            words = [v[pl.ds(128 * g + j0, 16, stride=8), :] for v in views]
            for e in range(2):
                half = _lo_half if e == 0 else _hi_half
                o = _fft([(_t(half(w)), None) for w in words], -1)
                r0 = pl.multiple_of((8 * jj + 2 * j0 + e) * 128 + 16 * g, 16)
                parts = [o[0][0], o[4][0], o[1][0], o[1][1], o[2][0], o[2][1], o[3][0], o[3][1]]
                for t in range(8):
                    u_v[pl.ds(r0, 16), t * 128:(t + 1) * 128] = _tval(parts[t]).astype(BF16)

    def f23(q):
        rows = pl.ds(pl.multiple_of(q * 128, 128), 128)
        o = [_dot_nt(l_v[256 * i:256 * (i + 1), :], u_v[rows, 256 * (i + 1):256 * (i + 2)])
             .astype(BF16) for i in range(3)]
        o0 = _dot_nt(l_v[768:912, 0:128], u_v[rows, 0:128]).astype(BF16)
        o4 = _dot_nt(l_v[768:896, 128:256], u_v[rows, 128:256]).astype(BF16)

        def blk(k1, part):
            if k1 == 0:
                return o0[64 * part:64 * part + 64]
            if k1 == 4:
                return o4[64 * part:64 * part + 64]
            if k1 < 4:
                return o[k1 - 1][64 * part:64 * part + 64]
            return o[7 - k1][128 + 64 * part:128 + 64 * part + 64]

        re = jnp.concatenate([blk(k1, 0) for k1 in range(8)] + [o0[128:144]], axis=0)
        im = jnp.concatenate([blk(k1, 1) for k1 in range(8)] + [jnp.zeros((16, 128), BF16)],
                             axis=0)
        y_v[q] = _dot(jnp.concatenate([re, im], axis=1),
                      gf_v[pl.ds(pl.multiple_of(q * 256, 256), 256), :])

    def mid(rows, filt):
        xf = _fft([(_t(y_v[q, rows, 0:128]), _t(y_v[q, rows, 128:256])) for q in range(16)], -1)
        zs = []
        for kq in range(16):
            fr, fi = filt(kq)
            re, im = xf[kq]
            zs.append((_tsub(_tmul(re, fr), _tmul(im, fi)), _tadd(_tmul(re, fi), _tmul(im, fr))))
        us = _fft(zs, +1)
        for q in range(16):
            z_v[q, rows, 0:128] = _tval(us[q][0]).astype(BF16)
            z_v[q, rows, 128:256] = _tval(us[q][1]).astype(BF16)

    def mid_group(g2, k1s):
        base = pl.multiple_of(64 * g2, 64)
        for k1 in k1s:
            half = _lo_half if k1 % 2 == 0 else _hi_half
            sl = pl.ds(k1 // 2, 16, stride=4)

            def filt(kq):
                return (half(wr32.at[kq, pl.ds(base, 64)][sl, :]),
                        half(wi32.at[kq, pl.ds(base, 64)][sl, :]))

            mid(pl.ds(pl.multiple_of(64 * k1 + 16 * g2, 16), 16), filt)

    def mid_nyquist():
        def filt(kq):
            cs = slice(kq * 128, (kq + 1) * 128)
            return (jnp.broadcast_to(wrn_v[:, cs].astype(F32), (16, 128)),
                    jnp.broadcast_to(win_v[:, cs].astype(F32), (16, 128)))

        mid(slice(512, KR), filt)

    srow = lax.broadcasted_iota(jnp.int32, (64, 128), 0)

    def i32(jj, j0):
        ys = []
        for e in range(2):
            q = 8 * jj + 2 * j0 + e
            z = _dot_nt(z_v[q], gf_v[pl.ds(pl.multiple_of(q * 256, 256), 256), :])
            zr, zi = z[:, 0:128], z[:, 128:256]
            zi0 = jnp.where(srow == 0, jnp.broadcast_to(zr[512:513], (64, 128)), zi[0:64])
            rhs0 = jnp.concatenate([zr[0:64], zi0], axis=0).astype(BF16)
            t0 = _dot(l_v[1792:1920, 0:128], rhs0)
            rhs4 = jnp.concatenate([zr[256:320], zi[256:320]], axis=0).astype(BF16)
            t4 = _dot(l_v[1792:1920, 128:256], rhs4)
            ts = []
            for k1 in (1, 2, 3):
                kc = 8 - k1
                rhs = jnp.concatenate([zr[64 * k1:64 * k1 + 64], zi[64 * k1:64 * k1 + 64],
                                       zr[64 * kc:64 * kc + 64], zi[64 * kc:64 * kc + 64]],
                                      axis=0).astype(BF16)
                o = _dot(l_v[1024 + 256 * (k1 - 1):1024 + 256 * k1, :], rhs)
                ts.append((o[0:128], o[128:256]))
            ys.append(_irfft8(t0, t4, *ts))
        for a in range(8):
            word_rows(a, jj)[pl.ds(j0, 128, stride=8), :] = _pack_words(ys[0][a], ys[1][a]).T

    nq = S // BQ
    nsub = BQ // 128
    row = lax.broadcasted_iota(jnp.int32, (128, 128), 0)
    col = lax.broadcasted_iota(jnp.int32, (128, 128), 1)
    tri = col <= row
    qscale = (D ** -0.5) * math.log2(math.e)

    def mx(a, b):
        return b if a is None else jnp.maximum(a, b)

    def addn(a, b):
        return b if a is None else a + b

    class St:
        pass

    def unpack_weights(h):
        j = h >> 1
        sh = jnp.asarray(16 * (1 - (h & 1))).astype(U32)
        for raw, w in ((wq_raw, ws_q), (wk_raw, ws_k), (wv_raw, ws_v)):
            w[...] = _hi_half(raw[j] << sh).astype(BF16)

    def track(nrm, name, a):
        n2 = jnp.max(jnp.sum(a * a, axis=1, keepdims=True), axis=0, keepdims=True)
        nrm[name] = mx(nrm.get(name), n2)

    def publish(nrm, slot, chunks):
        for w, name in enumerate(("q", "k")):
            val = jnp.max(nrm[name])
            for ch in chunks:
                nrm_s[4 * slot + 2 * ch + w] = val

    def proj_q(slot, rows, nrm):
        q = _dot(x_v[rows, :], ws_q[...]) * qscale
        track(nrm, "q", q)
        q_v[slot, rows, :] = q.astype(BF16)

    def proj_k(slot, rows, nrm):
        k = _dot(c_v[rows, :], ws_k[...])
        track(nrm, "k", k)
        k_v[slot, rows, :] = k.astype(BF16)

    def proj_v(slot, rows):
        v_v[slot, rows, :] = _dot(c_v[rows, :], ws_v[...]).astype(BF16)

    def proj_steps(slot, pm=256):
        steps = []
        nrm = {}
        for i in range(S // pm):
            rows = slice(i * pm, (i + 1) * pm)
            steps.append((8 * pm // 128, functools.partial(proj_q, slot, rows, nrm)))
            steps.append((4 * pm // 128, functools.partial(proj_k, slot, rows, nrm)))
            steps.append((4 * pm // 128, functools.partial(proj_v, slot, rows)))
        steps.append((0, functools.partial(publish, nrm, slot, (0, 1))))
        return steps

    pending = []

    def out_steps(h, i, st, last, nsplit=NSPLIT):
        rows = slice(i * BQ, (i + 1) * BQ)
        w = M // nsplit

        def step(t):
            cs = slice(t * w, (t + 1) * w)
            o = acc_v[rows, cs] + _dot(st.ctx, wo_v[pl.ds(pl.multiple_of(h * D, D), D), cs])
            if last:
                u_v[rows, cs] = o.astype(BF16)
                out_copy(i, t).start()
            else:
                acc_v[rows, cs] = o

        return [(nsub * w // 128, functools.partial(step, t)) for t in range(nsplit)]

    def fast_tiles(i, st, slot):
        r0 = i * BQ
        ntf = r0 // 128
        lacc = [None] * nsub
        acc = [None] * nsub
        left = [ntf + nsub]
        tiles = []

        def done(n):
            left[0] -= n
            if left[0] == 0:
                l = jnp.sum(jnp.concatenate(lacc, axis=0), axis=1, keepdims=True)
                st.ctx = (jnp.concatenate(acc, axis=0) / l).astype(BF16)

        def add_tile(t, c0, w):
            box = []

            def qk_exp():
                s = _dot_nt(q_v[slot, r0 + t * 128:r0 + BQ, :], k_v[slot, c0:c0 + w * 128, :])
                if c0 >= r0:
                    s0 = jnp.where(tri, s[:128], NEG)
                    s = jnp.concatenate([s0, s[128:]], axis=0) if t < nsub - 1 else s0
                p = jnp.exp2(s)
                for u in range(t, nsub):
                    lacc[u] = addn(lacc[u], functools.reduce(jnp.add, [
                        p[(u - t) * 128:(u - t + 1) * 128, j * 128:(j + 1) * 128]
                        for j in range(w)]))
                box.append(p.astype(BF16))

            def pv():
                o = _dot(box.pop(), v_v[slot, c0:c0 + w * 128, :])
                for u in range(t, nsub):
                    acc[u] = addn(acc[u], o[(u - t) * 128:(u - t + 1) * 128])
                done(w)

            tiles.append((w * (nsub - t), qk_exp, pv))

        kt = 0
        while kt < ntf:
            w = min(KW, ntf - kt)
            add_tile(0, kt * 128, w)
            kt += w
        for t in range(nsub):
            add_tile(t, r0 + t * 128, 1)
        return tiles

    def head_fast(h, slot, proj, last=False):
        sts = [St() for _ in range(nq)]
        order = list(range(nq))[::-1]
        tiles, ends = [], {}
        for i in order:
            tiles += fast_tiles(i, sts[i], slot)
            ends[len(tiles) - 1] = i
        proj = list(proj)
        outs = []
        t = [0.0]
        attn = 2 * sum(c for c, _, _ in tiles)
        fill = sum(c for c, _ in proj) + nq * nsub * (M // 128)
        debt = [0.0]

        def filler(force=False):
            while debt[0] > 0 or force:
                if outs and (outs[0][0] <= t[0] or not proj):
                    _, c, fn = outs.pop(0)
                elif proj:
                    c, fn = proj.pop(0)
                else:
                    return
                fn()
                t[0] += c
                debt[0] -= c

        n = len(tiles)
        for k in range(n + F_LAG):
            c = 0
            if k < n:
                tiles[k][1]()
                c += tiles[k][0]
            if k >= F_LAG:
                tiles[k - F_LAG][2]()
                c += tiles[k - F_LAG][0]
            t[0] += c
            if k - F_LAG in ends:
                i = ends[k - F_LAG]
                outs += [(t[0] + LAG_OUT, cc, fn) for cc, fn in out_steps(h, i, sts[i], last)]
            debt[0] += c * fill / attn * F_FILL
            filler()
        filler(force=True)

    def head_safe(h, slot, last=False):
        rr = lax.broadcasted_iota(jnp.int32, (256, 256), 0)
        cc = lax.broadcasted_iota(jnp.int32, (256, 256), 1)

        def q_block(qi, carry):
            rows = pl.ds(pl.multiple_of(qi * 256, 256), 256)
            q = q_v[slot, rows, :]

            def kv_block(kt, mla):
                m, l, acc = mla
                cols = pl.ds(pl.multiple_of(kt * 256, 256), 256)
                s = _dot_nt(q, k_v[slot, cols, :])
                s = jnp.where(cc + (kt - qi) * 256 <= rr, s, NEG)
                m_new = jnp.maximum(m, jnp.max(s, axis=1, keepdims=True))
                alpha = jnp.exp2(m - m_new)
                p = jnp.exp2(s - m_new)
                l = alpha * l + jnp.sum(p, axis=1, keepdims=True)
                acc = alpha * acc + _dot(p.astype(BF16), v_v[slot, cols, :])
                return m_new, l, acc

            init = (jnp.full((256, 1), NEG, F32), jnp.zeros((256, 1), F32),
                    jnp.zeros((256, D), F32))
            _, l, acc = lax.fori_loop(0, qi + 1, kv_block, init)
            ctx = (acc / l).astype(BF16)
            o = acc_v[rows, :] + _dot(ctx, wo_v[pl.ds(pl.multiple_of(h * D, D), D), :])
            if last:
                u_v[rows, :] = o.astype(BF16)
            else:
                acc_v[rows, :] = o
            return carry

        lax.fori_loop(0, S // 256, q_block, 0)

    def proj_safe(slot):
        def chunk(ch, carry):
            nrm = {}
            for i in range(2):
                rows = pl.ds(pl.multiple_of(ch * 1024 + i * 512, 512), 512)
                proj_q(slot, rows, nrm)
                proj_k(slot, rows, nrm)
                proj_v(slot, rows)
            publish(nrm, slot, (ch,))
            return carry

        lax.fori_loop(0, 2, chunk, 0)

    def out_copy(i, t):
        w = M // NSPLIT
        rows, cs = slice(i * BQ, (i + 1) * BQ), slice(t * w, (t + 1) * w)
        return pltpu.make_async_copy(u_v.at[rows, cs], out_h.at[rows, cs],
                                     osems.at[i * NSPLIT + t])

    def head(h, last=False):
        slot = h & 1
        q2 = jnp.maximum(nrm_s[4 * slot], nrm_s[4 * slot + 2])
        k2 = jnp.maximum(nrm_s[4 * slot + 1], nrm_s[4 * slot + 3])
        small = q2 * k2 <= SCORE_LIMIT ** 2

        @pl.when(small)
        def _():
            head_fast(h, slot, [] if last else proj_steps(1 - slot), last)

        @pl.when(jnp.logical_not(small))
        def _():
            head_safe(h, slot, last)
            if last:
                for i in range(nq):
                    for t in range(NSPLIT):
                        out_copy(i, t).start()
            else:
                proj_safe(1 - slot)

    for a in range(8):
        start(f"xb{a}", xb_h.at[:, a * 128:(a + 1) * 128], xb_v.at[a])
    start("l", l_h, l_v)
    start("gf", gf_h, gf_v)
    wait(*[f"xb{a}" for a in range(8)], "l", "gf")
    for t in range(16):
        start(f"wr{t}", wr_h.at[0:512, t * 128:(t + 1) * 128], wr_v.at[t])
        start(f"wi{t}", wi_h.at[0:512, t * 128:(t + 1) * 128], wi_v.at[t])
    start("wrn", wr_h.at[512:513, :], wrn_v)
    start("win", wi_h.at[512:513, :], win_v)
    start("c", c_h, c_v)
    start("x", x_h, x_v)
    for t in range(3):
        pair_copy(t, 0).start()

    def fwd_half(jj, carry):
        f1(jj, 0)
        for j0 in range(4):
            if j0 + 1 < 4:
                f1(jj, j0 + 1)
            f23(8 * jj + 2 * j0)
            f23(8 * jj + 2 * j0 + 1)
        return carry

    lax.fori_loop(0, 2, fwd_half, 0)

    wait(*[f"wr{t}" for t in range(16)], *[f"wi{t}" for t in range(16)], "wrn", "win")
    pair_copy(3, 0).start()
    s_v[...] = jnp.zeros(s_v.shape, F32)
    for i in range(S // 128):
        start(f"z{i}", s_v, acc_v.at[i * 128:(i + 1) * 128])
    for j in range(1, 5):
        for t in range(4):
            pair_copy(t, j).start()

    def mid_quarter(g2, carry):
        mid_group(g2, range(8))
        return carry

    lax.fori_loop(0, 4, mid_quarter, 0)
    mid_nyquist()

    wait("c", "x")
    for t in range(3):
        pair_copy(t, 0).wait()
    unpack_weights(0)

    def inv_half(jj, carry):
        nrm = {}
        for j0 in range(4):
            i32(jj, j0)
            rows = pl.ds(pl.multiple_of(jj * 1024 + 256 * j0, 256), 256)
            proj_q(0, rows, nrm)
            proj_k(0, rows, nrm)
            proj_v(0, rows)
        publish(nrm, 0, (jj,))
        return carry

    lax.fori_loop(0, 2, inv_half, 0)
    for a in range(8):
        c = pltpu.make_async_copy(xb_v.at[a], out_h.at[:, M + a * 128:M + (a + 1) * 128],
                                  bsems.at[a])
        c.start()
        pending.append(c)

    pair_copy(3, 0).wait()
    wait(*[f"z{i}" for i in range(S // 128)])
    for j in range(5, H // 2):
        for t in range(4):
            pair_copy(t, j).start()

    def body(h, carry):
        @pl.when((h & 1) == 1)
        def _():
            for t in range(4):
                pair_copy(t, (h + 1) >> 1).wait()

        unpack_weights(h + 1)
        head(h)
        return carry

    lax.fori_loop(0, H - 1, body, 0)
    head(H - 1, last=True)
    for c in pending:
        c.wait()
    for i in range(nq):
        for t in range(NSPLIT):
            out_copy(i, t).wait()


@jax.jit
def pallas_concat_heads__compressed_kv_cla__spectral_gfnet__prompt_kernel(
    A_x: jax.Array,
    A_c_kv: jax.Array,
    A_w_q: jax.Array,
    A_w_uk: jax.Array,
    A_w_uv: jax.Array,
    A_w_o: jax.Array,
    B_x: jax.Array,
    B_w_r: jax.Array,
    B_w_i: jax.Array,
):
    vm = pltpu.VMEM
    scratch = [
        vm((S, M), BF16), vm((S, C), BF16),
        vm((H // 2, M, D), U32), vm((H // 2, C, D), U32), vm((H // 2, C, D), U32),
        vm((H * D, M), BF16),
        vm((M, D), BF16), vm((C, D), BF16), vm((C, D), BF16),
        vm((8, S, 128), BF16),
        vm((16, 512, 128), BF16), vm((16, 512, 128), BF16),
        vm((1, S), BF16), vm((1, S), BF16),
        vm(_L_NP.shape, BF16), vm(_GF_NP.shape, BF16),
        vm((S, 1024), BF16),
        vm((16, KR, 256), F32), vm((16, KR, 256), BF16),
        vm((S, M), F32),
        vm((2, S, D), BF16), vm((2, S, D), BF16), vm((2, S, D), BF16),
        vm((128, M), F32),
        pltpu.SMEM((8,), F32),
        pltpu.SemaphoreType.DMA((64,)),
        pltpu.SemaphoreType.DMA((16,)),
        pltpu.SemaphoreType.DMA((4, H // 2)),
        pltpu.SemaphoreType.DMA((8,)),
    ]
    anyspec = pl.BlockSpec(memory_space=pl.ANY)
    out = pl.pallas_call(
        _kernel,
        out_shape=jax.ShapeDtypeStruct((S, M + DB), BF16),
        in_specs=[anyspec] * 11,
        out_specs=anyspec,
        scratch_shapes=scratch,
        compiler_params=pltpu.CompilerParams(vmem_limit_bytes=122 * 1024 * 1024),
        name="mla_gfnet_fused",
    )(
        A_x.reshape(S, M), A_c_kv.reshape(S, C), A_w_q, A_w_uk, A_w_uv,
        A_w_o.reshape(H * D, M),
        B_x.reshape(S, DB), B_w_r.T, B_w_i.T,
        jnp.asarray(_L_NP), jnp.asarray(_GF_NP),
    )
    return out.reshape(1, S, M + DB)
```

```python
import functools
import math

import numpy as np
import jax
import jax.numpy as jnp
from jax import lax
import jax.experimental.pallas as pl
import jax.experimental.pallas.tpu as pltpu

S = 2048
M = 1024
H = 32
D = 128
C = 512
DB = 1024
KR = 528

F32 = jnp.float32
BF16 = jnp.bfloat16
U32 = jnp.uint32
NT = (((1,), (1,)), ((), ()))
NEG = -1e30


def _np_bf16(a):
    return np.asarray(a, np.float32).astype(jnp.bfloat16)


def _make_consts():
    th = 2.0 * np.pi / DB
    b = np.arange(128)[None, :]
    k2 = np.arange(64)[:, None]
    lf = []
    for k1 in (1, 2, 3):
        g = np.exp(-1j * th * b * (k1 + 8 * k2))
        gp = np.exp(-1j * th * b * (8 - k1 + 8 * k2))
        lf.append(np.block([[g.real, -g.imag], [g.imag, g.real],
                            [gp.real, gp.imag], [gp.imag, -gp.real]]))
    g0 = np.exp(-1j * th * b * (8 * k2))
    g4 = np.exp(-1j * th * b * (4 + 8 * k2))
    l0 = np.concatenate([g0.real, g0.imag, np.cos(th * b * 512), np.zeros((127, 128))], 0)
    l4 = np.concatenate([g4.real, g4.imag, np.zeros((128, 128))], 0)
    lf.append(np.concatenate([l0, l4], 1))
    sc = 1.0 / (S * DB)
    bb = np.arange(128)[:, None]
    kk = np.arange(64)[None, :]
    li = []
    for k1 in (1, 2, 3):
        ph, pp = th * bb * (k1 + 8 * kk), th * bb * (8 - k1 + 8 * kk)
        c, s_, cp, sp = np.cos(ph), np.sin(ph), np.cos(pp), np.sin(pp)
        li.append(2 * sc * np.block([[c, -s_, cp, -sp], [s_, c, -sp, -cp]]))
    ph = th * bb * (8 * kk)
    c0, s0 = 2 * np.cos(ph), -2 * np.sin(ph)
    c0[:, 0] = 1.0
    s0[:, 0] = np.cos(th * bb[:, 0] * 512)
    i0 = sc * np.concatenate([c0, s0], 1)
    ph = th * bb * (4 + 8 * kk)
    i4 = sc * np.concatenate([2 * np.cos(ph), -2 * np.sin(ph)], 1)
    li.append(np.concatenate([np.concatenate([i0, i4], 1), np.zeros((128, 256))], 0))
    lmat = np.concatenate(lf + li, axis=0)
    p = np.arange(128)[None, :]
    kp = np.arange(128)[:, None]
    gf = []
    for q in range(16):
        g = np.exp(-2j * np.pi * (16 * p + q) * kp / S)
        gf.append(np.block([[g.real.T, g.imag.T], [-g.imag.T, g.real.T]]))
    return _np_bf16(lmat), _np_bf16(np.concatenate(gf, 0))


_L_NP, _GF_NP = _make_consts()


_dot = functools.partial(jnp.dot, preferred_element_type=F32)
_dot_nt = functools.partial(lax.dot_general, dimension_numbers=NT, preferred_element_type=F32)


def _t(x):
    return None if x is None else (1, x)


def _tneg(a):
    return None if a is None else (-a[0], a[1])


def _tadd(a, b):
    if a is None:
        return b
    if b is None:
        return a
    if a[0] == b[0]:
        return (a[0], a[1] + b[1])
    return (1, a[1] - b[1]) if a[0] > 0 else (1, b[1] - a[1])


def _tsub(a, b):
    return _tadd(a, _tneg(b))


def _tscale(a, c):
    return None if a is None else (1, a[1] * (c * a[0]))


def _tmul(a, v):
    return None if a is None else (a[0], a[1] * v)


def _tval(a):
    return a[1] if a[0] > 0 else -a[1]


def _twiddle(z, e, n, sign):
    re, im = z
    if e == 0:
        return re, im
    if 4 * e == n:
        return (_tneg(im), re) if sign > 0 else (im, _tneg(re))
    c = math.cos(2.0 * math.pi * e / n)
    s = sign * math.sin(2.0 * math.pi * e / n)
    if 8 * e % n == 0:
        r = abs(c)
        rc = re if c > 0 else _tneg(re)
        rs = re if s > 0 else _tneg(re)
        ic = im if c > 0 else _tneg(im)
        is_ = im if s > 0 else _tneg(im)
        return _tscale(_tsub(rc, is_), r), _tscale(_tadd(rs, ic), r)
    return (_tsub(_tscale(re, c), _tscale(im, s)), _tadd(_tscale(re, s), _tscale(im, c)))


def _fft(zs, sign):
    n = len(zs)
    if n == 1:
        return [zs[0]]
    ev = _fft(zs[0::2], sign)
    od = _fft(zs[1::2], sign)
    out = [None] * n
    for k in range(n // 2):
        t = _twiddle(od[k], k, n, sign)
        out[k] = (_tadd(ev[k][0], t[0]), _tadd(ev[k][1], t[1]))
        out[k + n // 2] = (_tsub(ev[k][0], t[0]), _tsub(ev[k][1], t[1]))
    return out


def _irfft8(t0, t4, t1, t2, t3):
    r = math.sqrt(0.5)
    a0, a1 = t0 + t4, t0 - t4
    e0, e2 = a0 + t2[0], a0 - t2[0]
    e1, e3 = a1 - t2[1], a1 + t2[1]
    o0 = t1[0] + t3[0]
    o2 = t3[1] - t1[1]
    u, v = t1[0] - t3[0], t1[1] + t3[1]
    o1, o3 = (u - v) * r, (-u - v) * r
    return [e0 + o0, e1 + o1, e2 + o2, e3 + o3, e0 - o0, e1 - o1, e2 - o2, e3 - o3]


def _lo_half(w):
    return pltpu.bitcast(w << 16, F32)


def _hi_half(w):
    return pltpu.bitcast(w & jnp.uint32(0xFFFF0000), F32)


def _pack_words(lo, hi):
    lo = pltpu.bitcast(lo.astype(BF16).astype(F32), U32)
    hi = pltpu.bitcast(hi.astype(BF16).astype(F32), U32)
    return (lo >> 16) | hi


def _interleave(gens):
    live = list(gens)
    while live:
        nxt = []
        for g in live:
            try:
                next(g)
                nxt.append(g)
            except StopIteration:
                pass
        live = nxt


def _drain(g):
    for _ in g:
        pass


BQ = 512
KW = 4
NSPLIT = 4
LAG_OUT = 16
F_LAG = 2
F_FILL = 1.0
SCORE_LIMIT = 60.0


def _kernel(x_h, c_h, wq_h, wk_h, wv_h, wo_h, xb_h, wr_h, wi_h, l_h, gf_h,
            out_h,
            x_v, c_v, wq_raw, wk_raw, wv_raw, wo_v, ws_q, ws_k, ws_v,
            xb_v, wr_v, wi_v, wrn_v, win_v, l_v, gf_v,
            u_v, y_v, z_v,
            acc_v, q_v, k_v, v_v, s_v, nrm_s,
            sems, osems, wsems, bsems):
    cp = {}
    nsem = [0]

    def start(name, src, dst, priority=0):
        c = pltpu.make_async_copy(src, dst, sems.at[nsem[0]])
        nsem[0] += 1
        c.start(priority=priority)
        cp[name] = c

    def wait(*names):
        for nm in names:
            cp[nm].wait()

    wq32, wk32, wv32 = wq_h.bitcast(U32), wk_h.bitcast(U32), wv_h.bitcast(U32)

    def pair_copy(t, j):
        src, dst = ((wq32, wq_raw), (wk32, wk_raw), (wv32, wv_raw))[t]
        return pltpu.make_async_copy(src.at[:, j, :], dst.at[j], wsems.at[t, j])

    xb32 = xb_v.bitcast(U32)
    wr32 = wr_v.bitcast(U32)
    wi32 = wi_v.bitcast(U32)

    def word_rows(a, jj):
        return xb32.at[a, pl.ds(pl.multiple_of(4 * jj, 4), 1020)]

    def f1(jj, j0):
        views = [word_rows(a, jj) for a in range(8)]
        for g in range(8):
            words = [v[pl.ds(128 * g + j0, 16, stride=8), :] for v in views]
            for e in range(2):
                half = _lo_half if e == 0 else _hi_half
                o = _fft([(_t(half(w)), None) for w in words], -1)
                r0 = pl.multiple_of((8 * jj + 2 * j0 + e) * 128 + 16 * g, 16)
                parts = [o[0][0], o[4][0], o[1][0], o[1][1], o[2][0], o[2][1], o[3][0], o[3][1]]
                for t in range(8):
                    u_v[pl.ds(r0, 16), t * 128:(t + 1) * 128] = _tval(parts[t]).astype(BF16)

    def f23(q):
        rows = pl.ds(pl.multiple_of(q * 128, 128), 128)
        o = [_dot_nt(l_v[256 * i:256 * (i + 1), :], u_v[rows, 256 * (i + 1):256 * (i + 2)])
             .astype(BF16) for i in range(3)]
        o0 = _dot_nt(l_v[768:912, 0:128], u_v[rows, 0:128]).astype(BF16)
        o4 = _dot_nt(l_v[768:896, 128:256], u_v[rows, 128:256]).astype(BF16)

        def blk(k1, part):
            if k1 == 0:
                return o0[64 * part:64 * part + 64]
            if k1 == 4:
                return o4[64 * part:64 * part + 64]
            if k1 < 4:
                return o[k1 - 1][64 * part:64 * part + 64]
            return o[7 - k1][128 + 64 * part:128 + 64 * part + 64]

        re = jnp.concatenate([blk(k1, 0) for k1 in range(8)] + [o0[128:144]], axis=0)
        im = jnp.concatenate([blk(k1, 1) for k1 in range(8)] + [jnp.zeros((16, 128), BF16)],
                             axis=0)
        y_v[q] = _dot(jnp.concatenate([re, im], axis=1),
                      gf_v[pl.ds(pl.multiple_of(q * 256, 256), 256), :])

    def mid(rows, filt):
        xf = _fft([(_t(y_v[q, rows, 0:128]), _t(y_v[q, rows, 128:256])) for q in range(16)], -1)
        zs = []
        for kq in range(16):
            fr, fi = filt(kq)
            re, im = xf[kq]
            zs.append((_tsub(_tmul(re, fr), _tmul(im, fi)), _tadd(_tmul(re, fi), _tmul(im, fr))))
        us = _fft(zs, +1)
        for q in range(16):
            z_v[q, rows, 0:128] = _tval(us[q][0]).astype(BF16)
            z_v[q, rows, 128:256] = _tval(us[q][1]).astype(BF16)

    def mid_group(g2, k1s):
        base = pl.multiple_of(64 * g2, 64)
        for k1 in k1s:
            half = _lo_half if k1 % 2 == 0 else _hi_half
            sl = pl.ds(k1 // 2, 16, stride=4)

            def filt(kq):
                return (half(wr32.at[kq, pl.ds(base, 64)][sl, :]),
                        half(wi32.at[kq, pl.ds(base, 64)][sl, :]))

            mid(pl.ds(pl.multiple_of(64 * k1 + 16 * g2, 16), 16), filt)

    def mid_nyquist():
        def filt(kq):
            cs = slice(kq * 128, (kq + 1) * 128)
            return (jnp.broadcast_to(wrn_v[:, cs].astype(F32), (16, 128)),
                    jnp.broadcast_to(win_v[:, cs].astype(F32), (16, 128)))

        mid(slice(512, KR), filt)

    srow = lax.broadcasted_iota(jnp.int32, (64, 128), 0)

    def i32(jj, j0):
        ys = []
        for e in range(2):
            q = 8 * jj + 2 * j0 + e
            z = _dot_nt(z_v[q], gf_v[pl.ds(pl.multiple_of(q * 256, 256), 256), :])
            zr, zi = z[:, 0:128], z[:, 128:256]
            zi0 = jnp.where(srow == 0, jnp.broadcast_to(zr[512:513], (64, 128)), zi[0:64])
            rhs0 = jnp.concatenate([zr[0:64], zi0], axis=0).astype(BF16)
            t0 = _dot(l_v[1792:1920, 0:128], rhs0)
            rhs4 = jnp.concatenate([zr[256:320], zi[256:320]], axis=0).astype(BF16)
            t4 = _dot(l_v[1792:1920, 128:256], rhs4)
            ts = []
            for k1 in (1, 2, 3):
                kc = 8 - k1
                rhs = jnp.concatenate([zr[64 * k1:64 * k1 + 64], zi[64 * k1:64 * k1 + 64],
                                       zr[64 * kc:64 * kc + 64], zi[64 * kc:64 * kc + 64]],
                                      axis=0).astype(BF16)
                o = _dot(l_v[1024 + 256 * (k1 - 1):1024 + 256 * k1, :], rhs)
                ts.append((o[0:128], o[128:256]))
            ys.append(_irfft8(t0, t4, *ts))
        for a in range(8):
            word_rows(a, jj)[pl.ds(j0, 128, stride=8), :] = _pack_words(ys[0][a], ys[1][a]).T

    nq = S // BQ
    nsub = BQ // 128
    row = lax.broadcasted_iota(jnp.int32, (128, 128), 0)
    col = lax.broadcasted_iota(jnp.int32, (128, 128), 1)
    tri = col <= row
    qscale = (D ** -0.5) * math.log2(math.e)

    def mx(a, b):
        return b if a is None else jnp.maximum(a, b)

    def addn(a, b):
        return b if a is None else a + b

    class St:
        pass

    def unpack_weights(h):
        j = h >> 1
        sh = jnp.asarray(16 * (1 - (h & 1))).astype(U32)
        for raw, w in ((wq_raw, ws_q), (wk_raw, ws_k), (wv_raw, ws_v)):
            w[...] = _hi_half(raw[j] << sh).astype(BF16)

    def track(nrm, name, a):
        n2 = jnp.max(jnp.sum(a * a, axis=1, keepdims=True), axis=0, keepdims=True)
        nrm[name] = mx(nrm.get(name), n2)

    def publish(nrm, slot, chunks):
        for w, name in enumerate(("q", "k")):
            val = jnp.max(nrm[name])
            for ch in chunks:
                nrm_s[4 * slot + 2 * ch + w] = val

    def proj_q(slot, rows, nrm):
        q = _dot(x_v[rows, :], ws_q[...]) * qscale
        track(nrm, "q", q)
        q_v[slot, rows, :] = q.astype(BF16)

    def proj_k(slot, rows, nrm):
        k = _dot(c_v[rows, :], ws_k[...])
        track(nrm, "k", k)
        k_v[slot, rows, :] = k.astype(BF16)

    def proj_v(slot, rows):
        v_v[slot, rows, :] = _dot(c_v[rows, :], ws_v[...]).astype(BF16)

    def proj_steps(slot, pm=256):
        steps = []
        nrm = {}
        for i in range(S // pm):
            rows = slice(i * pm, (i + 1) * pm)
            steps.append((8 * pm // 128, functools.partial(proj_q, slot, rows, nrm)))
            steps.append((4 * pm // 128, functools.partial(proj_k, slot, rows, nrm)))
            steps.append((4 * pm // 128, functools.partial(proj_v, slot, rows)))
        steps.append((0, functools.partial(publish, nrm, slot, (0, 1))))
        return steps

    pending = []

    def out_steps(h, i, st, last, nsplit=NSPLIT):
        rows = slice(i * BQ, (i + 1) * BQ)
        w = M // nsplit

        def step(t):
            cs = slice(t * w, (t + 1) * w)
            o = acc_v[rows, cs] + _dot(st.ctx, wo_v[pl.ds(pl.multiple_of(h * D, D), D), cs])
            if last:
                u_v[rows, cs] = o.astype(BF16)
                out_copy(i, t).start()
            else:
                acc_v[rows, cs] = o

        return [(nsub * w // 128, functools.partial(step, t)) for t in range(nsplit)]

    def fast_tiles(i, st, slot):
        r0 = i * BQ
        ntf = r0 // 128
        lacc = [None] * nsub
        acc = [None] * nsub
        left = [ntf + nsub]
        tiles = []

        def done(n):
            left[0] -= n
            if left[0] == 0:
                l = jnp.sum(jnp.concatenate(lacc, axis=0), axis=1, keepdims=True)
                st.ctx = (jnp.concatenate(acc, axis=0) / l).astype(BF16)

        def add_tile(t, c0, w):
            box = []

            def qk_exp():
                s = _dot_nt(q_v[slot, r0 + t * 128:r0 + BQ, :], k_v[slot, c0:c0 + w * 128, :])
                if c0 >= r0:
                    s0 = jnp.where(tri, s[:128], NEG)
                    s = jnp.concatenate([s0, s[128:]], axis=0) if t < nsub - 1 else s0
                p = jnp.exp2(s)
                for u in range(t, nsub):
                    lacc[u] = addn(lacc[u], functools.reduce(jnp.add, [
                        p[(u - t) * 128:(u - t + 1) * 128, j * 128:(j + 1) * 128]
                        for j in range(w)]))
                box.append(p.astype(BF16))

            def pv():
                o = _dot(box.pop(), v_v[slot, c0:c0 + w * 128, :])
                for u in range(t, nsub):
                    acc[u] = addn(acc[u], o[(u - t) * 128:(u - t + 1) * 128])
                done(w)

            tiles.append((w * (nsub - t), qk_exp, pv))

        kt = 0
        while kt < ntf:
            w = min(KW, ntf - kt)
            add_tile(0, kt * 128, w)
            kt += w
        for t in range(nsub):
            add_tile(t, r0 + t * 128, 1)
        return tiles

    def head_fast(h, slot, proj, last=False):
        sts = [St() for _ in range(nq)]
        order = list(range(nq))[::-1]
        tiles, ends = [], {}
        for i in order:
            tiles += fast_tiles(i, sts[i], slot)
            ends[len(tiles) - 1] = i
        proj = list(proj)
        outs = []
        t = [0.0]
        attn = 2 * sum(c for c, _, _ in tiles)
        fill = sum(c for c, _ in proj) + nq * nsub * (M // 128)
        debt = [0.0]

        def filler(force=False):
            while debt[0] > 0 or force:
                if outs and (outs[0][0] <= t[0] or not proj):
                    _, c, fn = outs.pop(0)
                elif proj:
                    c, fn = proj.pop(0)
                else:
                    return
                fn()
                t[0] += c
                debt[0] -= c

        n = len(tiles)
        for k in range(n + F_LAG):
            c = 0
            if k < n:
                tiles[k][1]()
                c += tiles[k][0]
            if k >= F_LAG:
                tiles[k - F_LAG][2]()
                c += tiles[k - F_LAG][0]
            t[0] += c
            if k - F_LAG in ends:
                i = ends[k - F_LAG]
                outs += [(t[0] + LAG_OUT, cc, fn) for cc, fn in out_steps(h, i, sts[i], last)]
            debt[0] += c * fill / attn * F_FILL
            filler()
        filler(force=True)

    def head_safe(h, slot, last=False):
        rr = lax.broadcasted_iota(jnp.int32, (256, 256), 0)
        cc = lax.broadcasted_iota(jnp.int32, (256, 256), 1)

        def q_block(qi, carry):
            rows = pl.ds(pl.multiple_of(qi * 256, 256), 256)
            q = q_v[slot, rows, :]

            def kv_block(kt, mla):
                m, l, acc = mla
                cols = pl.ds(pl.multiple_of(kt * 256, 256), 256)
                s = _dot_nt(q, k_v[slot, cols, :])
                s = jnp.where(cc + (kt - qi) * 256 <= rr, s, NEG)
                m_new = jnp.maximum(m, jnp.max(s, axis=1, keepdims=True))
                alpha = jnp.exp2(m - m_new)
                p = jnp.exp2(s - m_new)
                l = alpha * l + jnp.sum(p, axis=1, keepdims=True)
                acc = alpha * acc + _dot(p.astype(BF16), v_v[slot, cols, :])
                return m_new, l, acc

            init = (jnp.full((256, 1), NEG, F32), jnp.zeros((256, 1), F32),
                    jnp.zeros((256, D), F32))
            _, l, acc = lax.fori_loop(0, qi + 1, kv_block, init)
            ctx = (acc / l).astype(BF16)
            o = acc_v[rows, :] + _dot(ctx, wo_v[pl.ds(pl.multiple_of(h * D, D), D), :])
            if last:
                u_v[rows, :] = o.astype(BF16)
            else:
                acc_v[rows, :] = o
            return carry

        lax.fori_loop(0, S // 256, q_block, 0)

    def proj_safe(slot):
        def chunk(ch, carry):
            nrm = {}
            for i in range(2):
                rows = pl.ds(pl.multiple_of(ch * 1024 + i * 512, 512), 512)
                proj_q(slot, rows, nrm)
                proj_k(slot, rows, nrm)
                proj_v(slot, rows)
            publish(nrm, slot, (ch,))
            return carry

        lax.fori_loop(0, 2, chunk, 0)

    def out_copy(i, t):
        w = M // NSPLIT
        rows, cs = slice(i * BQ, (i + 1) * BQ), slice(t * w, (t + 1) * w)
        return pltpu.make_async_copy(u_v.at[rows, cs], out_h.at[rows, cs],
                                     osems.at[i * NSPLIT + t])

    def head(h, last=False):
        slot = h & 1
        q2 = jnp.maximum(nrm_s[4 * slot], nrm_s[4 * slot + 2])
        k2 = jnp.maximum(nrm_s[4 * slot + 1], nrm_s[4 * slot + 3])
        small = q2 * k2 <= SCORE_LIMIT ** 2

        @pl.when(small)
        def _():
            head_fast(h, slot, [] if last else proj_steps(1 - slot), last)

        @pl.when(jnp.logical_not(small))
        def _():
            head_safe(h, slot, last)
            if last:
                for i in range(nq):
                    for t in range(NSPLIT):
                        out_copy(i, t).start()
            else:
                proj_safe(1 - slot)

    for a in range(8):
        start(f"xb{a}", xb_h.at[:, a * 128:(a + 1) * 128], xb_v.at[a])
    start("l", l_h, l_v)
    start("gf", gf_h, gf_v)
    for t in range(16):
        start(f"wr{t}", wr_h.at[0:512, t * 128:(t + 1) * 128], wr_v.at[t])
        start(f"wi{t}", wi_h.at[0:512, t * 128:(t + 1) * 128], wi_v.at[t])
    start("wrn", wr_h.at[512:513, :], wrn_v)
    start("win", wi_h.at[512:513, :], win_v)
    start("c", c_h, c_v)
    start("x", x_h, x_v)
    for t in range(3):
        pair_copy(t, 0).start()
    start("wo", wo_h, wo_v)
    s_v[...] = jnp.zeros(s_v.shape, F32)
    for i in range(S // 512):
        start(f"z{i}", s_v, acc_v.at[i * 512:(i + 1) * 512], priority=1)
    wait(*[f"xb{a}" for a in range(8)], "l", "gf")

    def fwd_half(jj, carry):
        for i in range(7):
            for t in range(3):
                pair_copy(t, 7 * jj + i + 1).start()
        f1(jj, 0)
        for j0 in range(4):
            if j0 + 1 < 4:
                f1(jj, j0 + 1)
            f23(8 * jj + 2 * j0)
            f23(8 * jj + 2 * j0 + 1)
        return carry

    lax.fori_loop(0, 2, fwd_half, 0)

    for t in range(3):
        pair_copy(t, H // 2 - 1).start()
    wait(*[f"wr{t}" for t in range(16)], *[f"wi{t}" for t in range(16)], "wrn", "win")
    def mid_quarter(g2, carry):
        mid_group(g2, range(8))
        return carry

    lax.fori_loop(0, 4, mid_quarter, 0)
    mid_nyquist()

    wait("c", "x")
    for t in range(3):
        pair_copy(t, 0).wait()
    unpack_weights(0)

    def inv_half(jj, carry):
        nrm = {}
        for j0 in range(4):
            i32(jj, j0)
            rows = pl.ds(pl.multiple_of(jj * 1024 + 256 * j0, 256), 256)
            proj_q(0, rows, nrm)
            proj_k(0, rows, nrm)
            proj_v(0, rows)
        publish(nrm, 0, (jj,))
        return carry

    lax.fori_loop(0, 2, inv_half, 0)
    for a in range(8):
        c = pltpu.make_async_copy(xb_v.at[a], out_h.at[:, M + a * 128:M + (a + 1) * 128],
                                  bsems.at[a])
        c.start()
        pending.append(c)

    wait("wo", *[f"z{i}" for i in range(S // 512)])
    def body(h, carry):
        @pl.when((h & 1) == 1)
        def _():
            for t in range(3):
                pair_copy(t, (h + 1) >> 1).wait()

        unpack_weights(h + 1)
        head(h)
        return carry

    lax.fori_loop(0, H - 1, body, 0)
    head(H - 1, last=True)
    for c in pending:
        c.wait()
    for i in range(nq):
        for t in range(NSPLIT):
            out_copy(i, t).wait()


@jax.jit
def pallas_concat_heads__compressed_kv_cla__spectral_gfnet__prompt_kernel(
    A_x: jax.Array,
    A_c_kv: jax.Array,
    A_w_q: jax.Array,
    A_w_uk: jax.Array,
    A_w_uv: jax.Array,
    A_w_o: jax.Array,
    B_x: jax.Array,
    B_w_r: jax.Array,
    B_w_i: jax.Array,
):
    vm = pltpu.VMEM
    scratch = [
        vm((S, M), BF16), vm((S, C), BF16),
        vm((H // 2, M, D), U32), vm((H // 2, C, D), U32), vm((H // 2, C, D), U32),
        vm((H * D, M), BF16),
        vm((M, D), BF16), vm((C, D), BF16), vm((C, D), BF16),
        vm((8, S, 128), BF16),
        vm((16, 512, 128), BF16), vm((16, 512, 128), BF16),
        vm((1, S), BF16), vm((1, S), BF16),
        vm(_L_NP.shape, BF16), vm(_GF_NP.shape, BF16),
        vm((S, 1024), BF16),
        vm((16, KR, 256), F32), vm((16, KR, 256), BF16),
        vm((S, M), F32),
        vm((2, S, D), BF16), vm((2, S, D), BF16), vm((2, S, D), BF16),
        vm((512, M), F32),
        pltpu.SMEM((8,), F32),
        pltpu.SemaphoreType.DMA((64,)),
        pltpu.SemaphoreType.DMA((16,)),
        pltpu.SemaphoreType.DMA((3, H // 2)),
        pltpu.SemaphoreType.DMA((8,)),
    ]
    anyspec = pl.BlockSpec(memory_space=pl.ANY)
    out = pl.pallas_call(
        _kernel,
        out_shape=jax.ShapeDtypeStruct((S, M + DB), BF16),
        in_specs=[anyspec] * 11,
        out_specs=anyspec,
        scratch_shapes=scratch,
        compiler_params=pltpu.CompilerParams(vmem_limit_bytes=122 * 1024 * 1024),
        name="mla_gfnet_fused",
    )(
        A_x.reshape(S, M), A_c_kv.reshape(S, C), A_w_q, A_w_uk, A_w_uv,
        A_w_o.reshape(H * D, M),
        B_x.reshape(S, DB), B_w_r.T, B_w_i.T,
        jnp.asarray(_L_NP), jnp.asarray(_GF_NP),
    )
    return out.reshape(1, S, M + DB)
```

```python
import functools
import math

import numpy as np
import jax
import jax.numpy as jnp
from jax import lax
import jax.experimental.pallas as pl
import jax.experimental.pallas.tpu as pltpu

S = 2048
M = 1024
H = 32
D = 128
C = 512
DB = 1024
KR = 528

F32 = jnp.float32
BF16 = jnp.bfloat16
U32 = jnp.uint32
NT = (((1,), (1,)), ((), ()))
NEG = -1e30


def _np_bf16(a):
    return np.asarray(a, np.float32).astype(jnp.bfloat16)


def _make_consts():
    th = 2.0 * np.pi / DB
    b = np.arange(128)[None, :]
    k2 = np.arange(64)[:, None]
    lf = []
    for k1 in (1, 2, 3):
        g = np.exp(-1j * th * b * (k1 + 8 * k2))
        gp = np.exp(-1j * th * b * (8 - k1 + 8 * k2))
        lf.append(np.block([[g.real, -g.imag], [g.imag, g.real],
                            [gp.real, gp.imag], [gp.imag, -gp.real]]))
    g0 = np.exp(-1j * th * b * (8 * k2))
    g4 = np.exp(-1j * th * b * (4 + 8 * k2))
    l0 = np.concatenate([g0.real, g0.imag, np.cos(th * b * 512), np.zeros((127, 128))], 0)
    l4 = np.concatenate([g4.real, g4.imag, np.zeros((128, 128))], 0)
    lf.append(np.concatenate([l0, l4], 1))
    sc = 1.0 / (S * DB)
    bb = np.arange(128)[:, None]
    kk = np.arange(64)[None, :]
    li = []
    for k1 in (1, 2, 3):
        ph, pp = th * bb * (k1 + 8 * kk), th * bb * (8 - k1 + 8 * kk)
        c, s_, cp, sp = np.cos(ph), np.sin(ph), np.cos(pp), np.sin(pp)
        li.append(2 * sc * np.block([[c, -s_, cp, -sp], [s_, c, -sp, -cp]]))
    ph = th * bb * (8 * kk)
    c0, s0 = 2 * np.cos(ph), -2 * np.sin(ph)
    c0[:, 0] = 1.0
    s0[:, 0] = np.cos(th * bb[:, 0] * 512)
    i0 = sc * np.concatenate([c0, s0], 1)
    ph = th * bb * (4 + 8 * kk)
    i4 = sc * np.concatenate([2 * np.cos(ph), -2 * np.sin(ph)], 1)
    li.append(np.concatenate([np.concatenate([i0, i4], 1), np.zeros((128, 256))], 0))
    lmat = np.concatenate(lf + li, axis=0)
    p = np.arange(128)[None, :]
    kp = np.arange(128)[:, None]
    gf = []
    for q in range(16):
        g = np.exp(-2j * np.pi * (16 * p + q) * kp / S)
        gf.append(np.block([[g.real.T, g.imag.T], [-g.imag.T, g.real.T]]))
    return _np_bf16(lmat), _np_bf16(np.concatenate(gf, 0))


_L_NP, _GF_NP = _make_consts()


_dot = functools.partial(jnp.dot, preferred_element_type=F32)
_dot_nt = functools.partial(lax.dot_general, dimension_numbers=NT, preferred_element_type=F32)


def _t(x):
    return None if x is None else (1, x)


def _tneg(a):
    return None if a is None else (-a[0], a[1])


def _tadd(a, b):
    if a is None:
        return b
    if b is None:
        return a
    if a[0] == b[0]:
        return (a[0], a[1] + b[1])
    return (1, a[1] - b[1]) if a[0] > 0 else (1, b[1] - a[1])


def _tsub(a, b):
    return _tadd(a, _tneg(b))


def _tscale(a, c):
    return None if a is None else (1, a[1] * (c * a[0]))


def _tmul(a, v):
    return None if a is None else (a[0], a[1] * v)


def _tval(a):
    return a[1] if a[0] > 0 else -a[1]


def _twiddle(z, e, n, sign):
    re, im = z
    if e == 0:
        return re, im
    if 4 * e == n:
        return (_tneg(im), re) if sign > 0 else (im, _tneg(re))
    c = math.cos(2.0 * math.pi * e / n)
    s = sign * math.sin(2.0 * math.pi * e / n)
    if 8 * e % n == 0:
        r = abs(c)
        rc = re if c > 0 else _tneg(re)
        rs = re if s > 0 else _tneg(re)
        ic = im if c > 0 else _tneg(im)
        is_ = im if s > 0 else _tneg(im)
        return _tscale(_tsub(rc, is_), r), _tscale(_tadd(rs, ic), r)
    return (_tsub(_tscale(re, c), _tscale(im, s)), _tadd(_tscale(re, s), _tscale(im, c)))


def _fft(zs, sign):
    n = len(zs)
    if n == 1:
        return [zs[0]]
    ev = _fft(zs[0::2], sign)
    od = _fft(zs[1::2], sign)
    out = [None] * n
    for k in range(n // 2):
        t = _twiddle(od[k], k, n, sign)
        out[k] = (_tadd(ev[k][0], t[0]), _tadd(ev[k][1], t[1]))
        out[k + n // 2] = (_tsub(ev[k][0], t[0]), _tsub(ev[k][1], t[1]))
    return out


def _irfft8(t0, t4, t1, t2, t3):
    r = math.sqrt(0.5)
    a0, a1 = t0 + t4, t0 - t4
    e0, e2 = a0 + t2[0], a0 - t2[0]
    e1, e3 = a1 - t2[1], a1 + t2[1]
    o0 = t1[0] + t3[0]
    o2 = t3[1] - t1[1]
    u, v = t1[0] - t3[0], t1[1] + t3[1]
    o1, o3 = (u - v) * r, (-u - v) * r
    return [e0 + o0, e1 + o1, e2 + o2, e3 + o3, e0 - o0, e1 - o1, e2 - o2, e3 - o3]


def _lo_half(w):
    return pltpu.bitcast(w << 16, F32)


def _hi_half(w):
    return pltpu.bitcast(w & jnp.uint32(0xFFFF0000), F32)


def _pack_words(lo, hi):
    lo = pltpu.bitcast(lo.astype(BF16).astype(F32), U32)
    hi = pltpu.bitcast(hi.astype(BF16).astype(F32), U32)
    return (lo >> 16) | hi


def _interleave(gens):
    live = list(gens)
    while live:
        nxt = []
        for g in live:
            try:
                next(g)
                nxt.append(g)
            except StopIteration:
                pass
        live = nxt


def _drain(g):
    for _ in g:
        pass


BQ = 512
KW = 2
NSPLIT = 4
PM = 512
LAG_OUT = 16
F_LAG = 1
F_FILL = 1.0
SCORE_LIMIT = 60.0


def _kernel(x_h, c_h, wq_h, wk_h, wv_h, wo_h, xb_h, wr_h, wi_h, l_h, gf_h,
            out_h,
            x_v, c_v, xs_v, cs_v, wq_raw, wk_raw, wv_raw, wo_v, ws_q, ws_k, ws_v,
            xb_v, wr_v, wi_v, wrn_v, win_v, l_v, gf_v,
            u_v, y_v, z_v,
            acc_v, q_v, k_v, v_v, s_v, nrm_s,
            sems, osems, wsems, bsems):
    cp = {}
    nsem = [0]

    def start(name, src, dst, priority=0):
        c = pltpu.make_async_copy(src, dst, sems.at[nsem[0]])
        nsem[0] += 1
        c.start(priority=priority)
        cp[name] = c

    def wait(*names):
        for nm in names:
            cp[nm].wait()

    wq32, wk32, wv32 = wq_h.bitcast(U32), wk_h.bitcast(U32), wv_h.bitcast(U32)

    def pair_copy(t, j):
        src, dst = ((wq32, wq_raw), (wk32, wk_raw), (wv32, wv_raw))[t]
        return pltpu.make_async_copy(src.at[:, j, :], dst.at[j], wsems.at[t, j])

    xb32 = xb_v.bitcast(U32)
    wr32 = wr_v.bitcast(U32)
    wi32 = wi_v.bitcast(U32)

    def word_rows(a, jj):
        return xb32.at[a, pl.ds(pl.multiple_of(4 * jj, 4), 1020)]

    def f1(jj, j0):
        views = [word_rows(a, jj) for a in range(8)]
        for g in range(8):
            words = [v[pl.ds(128 * g + j0, 16, stride=8), :] for v in views]
            for e in range(2):
                half = _lo_half if e == 0 else _hi_half
                o = _fft([(_t(half(w)), None) for w in words], -1)
                r0 = pl.multiple_of((8 * jj + 2 * j0 + e) * 128 + 16 * g, 16)
                parts = [o[0][0], o[4][0], o[1][0], o[1][1], o[2][0], o[2][1], o[3][0], o[3][1]]
                for t in range(8):
                    u_v[pl.ds(r0, 16), t * 128:(t + 1) * 128] = _tval(parts[t]).astype(BF16)

    def f23(q):
        rows = pl.ds(pl.multiple_of(q * 128, 128), 128)
        o = [_dot_nt(l_v[256 * i:256 * (i + 1), :], u_v[rows, 256 * (i + 1):256 * (i + 2)])
             .astype(BF16) for i in range(3)]
        o0 = _dot_nt(l_v[768:912, 0:128], u_v[rows, 0:128]).astype(BF16)
        o4 = _dot_nt(l_v[768:896, 128:256], u_v[rows, 128:256]).astype(BF16)

        def blk(k1, part):
            if k1 == 0:
                return o0[64 * part:64 * part + 64]
            if k1 == 4:
                return o4[64 * part:64 * part + 64]
            if k1 < 4:
                return o[k1 - 1][64 * part:64 * part + 64]
            return o[7 - k1][128 + 64 * part:128 + 64 * part + 64]

        re = jnp.concatenate([blk(k1, 0) for k1 in range(8)] + [o0[128:144]], axis=0)
        im = jnp.concatenate([blk(k1, 1) for k1 in range(8)] + [jnp.zeros((16, 128), BF16)],
                             axis=0)
        y_v[q] = _dot(jnp.concatenate([re, im], axis=1),
                      gf_v[pl.ds(pl.multiple_of(q * 256, 256), 256), :])

    def mid(rows, filt):
        xf = _fft([(_t(y_v[q, rows, 0:128]), _t(y_v[q, rows, 128:256])) for q in range(16)], -1)
        zs = []
        for kq in range(16):
            fr, fi = filt(kq)
            re, im = xf[kq]
            zs.append((_tsub(_tmul(re, fr), _tmul(im, fi)), _tadd(_tmul(re, fi), _tmul(im, fr))))
        us = _fft(zs, +1)
        for q in range(16):
            z_v[q, rows, 0:128] = _tval(us[q][0]).astype(BF16)
            z_v[q, rows, 128:256] = _tval(us[q][1]).astype(BF16)

    def mid_group(g2, k1s):
        base = pl.multiple_of(64 * g2, 64)
        for k1 in k1s:
            half = _lo_half if k1 % 2 == 0 else _hi_half
            sl = pl.ds(k1 // 2, 16, stride=4)

            def filt(kq):
                return (half(wr32.at[kq, pl.ds(base, 64)][sl, :]),
                        half(wi32.at[kq, pl.ds(base, 64)][sl, :]))

            mid(pl.ds(pl.multiple_of(64 * k1 + 16 * g2, 16), 16), filt)

    def mid_nyquist():
        def filt(kq):
            cs = slice(kq * 128, (kq + 1) * 128)
            return (jnp.broadcast_to(wrn_v[:, cs].astype(F32), (16, 128)),
                    jnp.broadcast_to(win_v[:, cs].astype(F32), (16, 128)))

        mid(slice(512, KR), filt)

    srow = lax.broadcasted_iota(jnp.int32, (64, 128), 0)

    def i32(jj, j0):
        ys = []
        for e in range(2):
            q = 8 * jj + 2 * j0 + e
            z = _dot_nt(z_v[q], gf_v[pl.ds(pl.multiple_of(q * 256, 256), 256), :])
            zr, zi = z[:, 0:128], z[:, 128:256]
            zi0 = jnp.where(srow == 0, jnp.broadcast_to(zr[512:513], (64, 128)), zi[0:64])
            rhs0 = jnp.concatenate([zr[0:64], zi0], axis=0).astype(BF16)
            t0 = _dot(l_v[1792:1920, 0:128], rhs0)
            rhs4 = jnp.concatenate([zr[256:320], zi[256:320]], axis=0).astype(BF16)
            t4 = _dot(l_v[1792:1920, 128:256], rhs4)
            ts = []
            for k1 in (1, 2, 3):
                kc = 8 - k1
                rhs = jnp.concatenate([zr[64 * k1:64 * k1 + 64], zi[64 * k1:64 * k1 + 64],
                                       zr[64 * kc:64 * kc + 64], zi[64 * kc:64 * kc + 64]],
                                      axis=0).astype(BF16)
                o = _dot(l_v[1024 + 256 * (k1 - 1):1024 + 256 * k1, :], rhs)
                ts.append((o[0:128], o[128:256]))
            ys.append(_irfft8(t0, t4, *ts))
        for a in range(8):
            word_rows(a, jj)[pl.ds(j0, 128, stride=8), :] = _pack_words(ys[0][a], ys[1][a]).T

    nq = S // BQ
    nsub = BQ // 128
    row = lax.broadcasted_iota(jnp.int32, (128, 128), 0)
    col = lax.broadcasted_iota(jnp.int32, (128, 128), 1)
    tri = col <= row
    qscale = (D ** -0.5) * math.log2(math.e)

    def mx(a, b):
        return b if a is None else jnp.maximum(a, b)

    def addn(a, b):
        return b if a is None else a + b

    class St:
        pass

    def split_inputs(src, dst):
        n = src.shape[1] // 2

        def chunk(i, carry):
            top = pl.ds(pl.multiple_of(i * 128, 128), 128)
            bot = pl.ds(pl.multiple_of(S // 2 + i * 128, 128), 128)
            a11, a12 = src[top, 0:n].astype(F32), src[top, n:].astype(F32)
            a21, a22 = src[bot, 0:n].astype(F32), src[bot, n:].astype(F32)
            for t, v in enumerate((a11 + a22, a21 + a22, a11 + a12, a21 - a11, a12 - a22)):
                dst[t, top, :] = v.astype(BF16)
            return carry

        lax.fori_loop(0, S // 256, chunk, 0)

    def unpack_weights(j):
        for raw, w in ((wq_raw, ws_q), (wk_raw, ws_k), (wv_raw, ws_v)):
            n = w.shape[1]
            up, dn = raw[j, 0:n, :], raw[j, n:, :]
            b11, b12, b21, b22 = _lo_half(up), _hi_half(up), _lo_half(dn), _hi_half(dn)
            for t, v in enumerate((b11 + b22, b11, b12 - b22, b21 - b11, b22,
                                   b11 + b12, b21 + b22)):
                w[t] = v.astype(BF16)

    def track(nrm, name, a):
        n2 = jnp.max(jnp.sum(a * a, axis=1, keepdims=True), axis=0, keepdims=True)
        nrm[name] = mx(nrm.get(name), n2)

    def publish(nrm, base, e):
        for t in range(2):
            for w, name in enumerate(("q", "k")):
                nrm_s[4 * (base + t) + 2 * e + w] = jnp.max(nrm[name, t])

    def proj(name, src, sums, w, dst, scale, base, r0, nrm):
        n = w.shape[1]
        top = pl.ds(pl.multiple_of(r0, PM), PM)
        bot = pl.ds(pl.multiple_of(S // 2 + r0, PM), PM)
        m1 = _dot(sums[0, top, :], w[0])
        m2 = _dot(sums[1, top, :], w[1])
        m3 = _dot(src[top, 0:n], w[2])
        m4 = _dot(src[bot, n:], w[3])
        m5 = _dot(sums[2, top, :], w[4])
        m6 = _dot(sums[3, top, :], w[5])
        m7 = _dot(sums[4, top, :], w[6])
        outs = ((0, top, (m1 + m4) + (m7 - m5)), (1, top, m3 + m5),
                (0, bot, m2 + m4), (1, bot, (m1 - m2) + (m3 + m6)))
        for t, rows, val in outs:
            if scale is not None:
                val = val * scale
            if name is not None:
                track(nrm, (name, t), val)
            dst[base + t, rows, :] = val.astype(BF16)

    def proj_steps(base, e):
        steps, nrm = [], {}
        for i in range(S // 4 // PM):
            r0 = e * (S // 4) + i * PM
            steps.append((7 * 4 * PM // 128,
                          functools.partial(proj, "q", x_v, xs_v, ws_q, q_v, qscale, base, r0, nrm)))
            steps.append((7 * 2 * PM // 128,
                          functools.partial(proj, "k", c_v, cs_v, ws_k, k_v, None, base, r0, nrm)))
            steps.append((7 * 2 * PM // 128,
                          functools.partial(proj, None, c_v, cs_v, ws_v, v_v, None, base, r0, nrm)))
        steps.append((0, functools.partial(publish, nrm, base, e)))
        return steps

    pending = []

    def out_steps(h, i, st, last, nsplit=NSPLIT):
        rows = slice(i * BQ, (i + 1) * BQ)
        w = M // nsplit

        def step(t):
            cs = slice(t * w, (t + 1) * w)
            o = acc_v[rows, cs] + _dot(st.ctx, wo_v[pl.ds(pl.multiple_of(h * D, D), D), cs])
            acc_v[rows, cs] = o
            if last:
                u_v[rows, cs] = o.astype(BF16)
                out_copy(i, t).start()

        return [(nsub * w // 128, functools.partial(step, t)) for t in range(nsplit)]

    def fast_tiles(i, st, slot):
        r0 = i * BQ
        ntf = r0 // 128
        lacc = [None] * nsub
        acc = [None] * nsub
        left = [ntf + nsub]
        tiles = []

        def done(n):
            left[0] -= n
            if left[0] == 0:
                l = jnp.sum(jnp.concatenate(lacc, axis=0), axis=1, keepdims=True)
                st.ctx = (jnp.concatenate(acc, axis=0) / l).astype(BF16)

        def add_tile(t, c0, w):
            box = []

            def qk_exp():
                s = _dot_nt(q_v[slot, r0 + t * 128:r0 + BQ, :], k_v[slot, c0:c0 + w * 128, :])
                if c0 >= r0:
                    s0 = jnp.where(tri, s[:128], NEG)
                    s = jnp.concatenate([s0, s[128:]], axis=0) if t < nsub - 1 else s0
                p = jnp.exp2(s)
                for u in range(t, nsub):
                    lacc[u] = addn(lacc[u], functools.reduce(jnp.add, [
                        p[(u - t) * 128:(u - t + 1) * 128, j * 128:(j + 1) * 128]
                        for j in range(w)]))
                box.append(p.astype(BF16))

            def pv():
                o = _dot(box.pop(), v_v[slot, c0:c0 + w * 128, :])
                for u in range(t, nsub):
                    acc[u] = addn(acc[u], o[(u - t) * 128:(u - t + 1) * 128])
                done(w)

            tiles.append((w * (nsub - t), qk_exp, pv))

        kt = 0
        while kt < ntf:
            w = min(KW, ntf - kt)
            add_tile(0, kt * 128, w)
            kt += w
        for t in range(nsub):
            add_tile(t, r0 + t * 128, 1)
        return tiles

    def head_fast(h, slot, proj, last=False):
        sts = [St() for _ in range(nq)]
        order = list(range(nq))[::-1]
        tiles, ends = [], {}
        for i in order:
            tiles += fast_tiles(i, sts[i], slot)
            ends[len(tiles) - 1] = i
        proj = list(proj)
        outs = []
        t = [0.0]
        attn = 2 * sum(c for c, _, _ in tiles)
        fill = sum(c for c, _ in proj) + nq * nsub * (M // 128)
        debt = [0.0]

        def filler(force=False):
            while debt[0] > 0 or force:
                if outs and (outs[0][0] <= t[0] or not proj):
                    _, c, fn = outs.pop(0)
                elif proj:
                    c, fn = proj.pop(0)
                else:
                    return
                fn()
                t[0] += c
                debt[0] -= c

        n = len(tiles)
        for k in range(n + F_LAG):
            c = 0
            if k < n:
                tiles[k][1]()
                c += tiles[k][0]
            if k >= F_LAG:
                tiles[k - F_LAG][2]()
                c += tiles[k - F_LAG][0]
            t[0] += c
            if k - F_LAG in ends:
                i = ends[k - F_LAG]
                outs += [(t[0] + LAG_OUT, cc, fn) for cc, fn in out_steps(h, i, sts[i], last)]
            debt[0] += c * fill / attn * F_FILL
            filler()
        filler(force=True)

    def head_safe(h, slot, last=False):
        rr = lax.broadcasted_iota(jnp.int32, (256, 256), 0)
        cc = lax.broadcasted_iota(jnp.int32, (256, 256), 1)

        def q_block(qi, carry):
            rows = pl.ds(pl.multiple_of(qi * 256, 256), 256)
            q = q_v[slot, rows, :]

            def kv_block(kt, mla):
                m, l, acc = mla
                cols = pl.ds(pl.multiple_of(kt * 256, 256), 256)
                s = _dot_nt(q, k_v[slot, cols, :])
                s = jnp.where(cc + (kt - qi) * 256 <= rr, s, NEG)
                m_new = jnp.maximum(m, jnp.max(s, axis=1, keepdims=True))
                alpha = jnp.exp2(m - m_new)
                p = jnp.exp2(s - m_new)
                l = alpha * l + jnp.sum(p, axis=1, keepdims=True)
                acc = alpha * acc + _dot(p.astype(BF16), v_v[slot, cols, :])
                return m_new, l, acc

            init = (jnp.full((256, 1), NEG, F32), jnp.zeros((256, 1), F32),
                    jnp.zeros((256, D), F32))
            _, l, acc = lax.fori_loop(0, qi + 1, kv_block, init)
            ctx = (acc / l).astype(BF16)
            o = acc_v[rows, :] + _dot(ctx, wo_v[pl.ds(pl.multiple_of(h * D, D), D), :])
            acc_v[rows, :] = o
            if last:
                u_v[rows, :] = o.astype(BF16)
            return carry

        lax.fori_loop(0, S // 256, q_block, 0)

    def out_copy(i, t):
        w = M // NSPLIT
        rows, cs = slice(i * BQ, (i + 1) * BQ), slice(t * w, (t + 1) * w)
        return pltpu.make_async_copy(u_v.at[rows, cs], out_h.at[rows, cs],
                                     osems.at[i * NSPLIT + t])

    def head(h, last=False):
        slot = h & 3
        q2 = jnp.maximum(nrm_s[4 * slot], nrm_s[4 * slot + 2])
        k2 = jnp.maximum(nrm_s[4 * slot + 1], nrm_s[4 * slot + 3])
        small = q2 * k2 <= SCORE_LIMIT ** 2

        def next_pair():
            if last:
                return []
            unpack_weights((h >> 1) + 1)
            return proj_steps(2 - (h & 2), h & 1)

        @pl.when(small)
        def _():
            head_fast(h, slot, next_pair(), last)

        @pl.when(jnp.logical_not(small))
        def _():
            head_safe(h, slot, last)
            for _, fn in next_pair():
                fn()
            if last:
                for i in range(nq):
                    for t in range(NSPLIT):
                        out_copy(i, t).start()

    for a in range(8):
        start(f"xb{a}", xb_h.at[:, a * 128:(a + 1) * 128], xb_v.at[a])
    start("l", l_h, l_v)
    start("gf", gf_h, gf_v)
    for t in range(16):
        start(f"wr{t}", wr_h.at[0:512, t * 128:(t + 1) * 128], wr_v.at[t])
        start(f"wi{t}", wi_h.at[0:512, t * 128:(t + 1) * 128], wi_v.at[t])
    start("wrn", wr_h.at[512:513, :], wrn_v)
    start("win", wi_h.at[512:513, :], win_v)
    start("c", c_h, c_v)
    start("x", x_h, x_v)
    for t in range(3):
        pair_copy(t, 0).start()
    start("wo", wo_h, wo_v)
    s_v[...] = jnp.zeros(s_v.shape, F32)
    for i in range(S // 512):
        start(f"z{i}", s_v, acc_v.at[i * 512:(i + 1) * 512], priority=1)
    wait(*[f"xb{a}" for a in range(8)], "l", "gf")

    def fwd_half(jj, carry):
        for i in range(7):
            for t in range(3):
                pair_copy(t, 7 * jj + i + 1).start()
        f1(jj, 0)
        for j0 in range(4):
            if j0 + 1 < 4:
                f1(jj, j0 + 1)
            f23(8 * jj + 2 * j0)
            f23(8 * jj + 2 * j0 + 1)
        return carry

    lax.fori_loop(0, 2, fwd_half, 0)

    for t in range(3):
        pair_copy(t, H // 2 - 1).start()
    wait(*[f"wr{t}" for t in range(16)], *[f"wi{t}" for t in range(16)], "wrn", "win")
    def mid_quarter(g2, carry):
        mid_group(g2, range(8))
        return carry

    lax.fori_loop(0, 4, mid_quarter, 0)
    mid_nyquist()

    wait("c", "x")
    for t in range(3):
        pair_copy(t, 0).wait()
    split_inputs(x_v, xs_v)
    split_inputs(c_v, cs_v)
    unpack_weights(0)

    def inv_half(jj, carry):
        merge = proj_steps(0, jj)
        for j0 in range(4):
            i32(jj, j0)
            for _, fn in merge[len(merge) * j0 // 4:len(merge) * (j0 + 1) // 4]:
                fn()
        return carry

    lax.fori_loop(0, 2, inv_half, 0)
    for a in range(8):
        c = pltpu.make_async_copy(xb_v.at[a], out_h.at[:, M + a * 128:M + (a + 1) * 128],
                                  bsems.at[a])
        c.start()
        pending.append(c)

    wait("wo", *[f"z{i}" for i in range(S // 512)])
    def body(h, carry):
        @pl.when((h & 1) == 0)
        def _():
            for t in range(3):
                pair_copy(t, (h >> 1) + 1).wait()

        head(h)
        return carry

    lax.fori_loop(0, H - 2, body, 0)
    def tail(h, carry):
        @pl.when(h == H - 1)
        def _():
            for i in range(nq):
                for t in range(NSPLIT):
                    out_copy(i, t).wait()

        head(h, last=True)
        return carry

    lax.fori_loop(H - 2, H, tail, 0)
    for c in pending:
        c.wait()
    for i in range(nq):
        for t in range(NSPLIT):
            out_copy(i, t).wait()


@jax.jit
def pallas_concat_heads__compressed_kv_cla__spectral_gfnet__prompt_kernel(
    A_x: jax.Array,
    A_c_kv: jax.Array,
    A_w_q: jax.Array,
    A_w_uk: jax.Array,
    A_w_uv: jax.Array,
    A_w_o: jax.Array,
    B_x: jax.Array,
    B_w_r: jax.Array,
    B_w_i: jax.Array,
):
    vm = pltpu.VMEM
    scratch = [
        vm((S, M), BF16), vm((S, C), BF16),
        vm((5, S // 2, M // 2), BF16), vm((5, S // 2, C // 2), BF16),
        vm((H // 2, M, D), U32), vm((H // 2, C, D), U32), vm((H // 2, C, D), U32),
        vm((H * D, M), BF16),
        vm((7, M // 2, D), BF16), vm((7, C // 2, D), BF16), vm((7, C // 2, D), BF16),
        vm((8, S, 128), BF16),
        vm((16, 512, 128), BF16), vm((16, 512, 128), BF16),
        vm((1, S), BF16), vm((1, S), BF16),
        vm(_L_NP.shape, BF16), vm(_GF_NP.shape, BF16),
        vm((S, 1024), BF16),
        vm((16, KR, 256), F32), vm((16, KR, 256), BF16),
        vm((S, M), F32),
        vm((4, S, D), BF16), vm((4, S, D), BF16), vm((4, S, D), BF16),
        vm((512, M), F32),
        pltpu.SMEM((16,), F32),
        pltpu.SemaphoreType.DMA((64,)),
        pltpu.SemaphoreType.DMA((16,)),
        pltpu.SemaphoreType.DMA((3, H // 2)),
        pltpu.SemaphoreType.DMA((8,)),
    ]
    anyspec = pl.BlockSpec(memory_space=pl.ANY)
    out = pl.pallas_call(
        _kernel,
        out_shape=jax.ShapeDtypeStruct((S, M + DB), BF16),
        in_specs=[anyspec] * 11,
        out_specs=anyspec,
        scratch_shapes=scratch,
        compiler_params=pltpu.CompilerParams(vmem_limit_bytes=122 * 1024 * 1024),
        name="mla_gfnet_fused",
    )(
        A_x.reshape(S, M), A_c_kv.reshape(S, C), A_w_q, A_w_uk, A_w_uv,
        A_w_o.reshape(H * D, M),
        B_x.reshape(S, DB), B_w_r.T, B_w_i.T,
        jnp.asarray(_L_NP), jnp.asarray(_GF_NP),
    )
    return out.reshape(1, S, M + DB)
```

```python
import functools
import math

import numpy as np
import jax
import jax.numpy as jnp
from jax import lax
import jax.experimental.pallas as pl
import jax.experimental.pallas.tpu as pltpu

S = 2048
M = 1024
H = 32
D = 128
C = 512
DB = 1024
KR = 528

F32 = jnp.float32
BF16 = jnp.bfloat16
U32 = jnp.uint32
NT = (((1,), (1,)), ((), ()))
NEG = -1e30


def _np_bf16(a):
    return np.asarray(a, np.float32).astype(jnp.bfloat16)


def _make_consts():
    th = 2.0 * np.pi / DB
    b = np.arange(128)[None, :]
    k2 = np.arange(64)[:, None]
    lf = []
    for k1 in (1, 2, 3):
        g = np.exp(-1j * th * b * (k1 + 8 * k2))
        gp = np.exp(-1j * th * b * (8 - k1 + 8 * k2))
        lf.append(np.block([[g.real, -g.imag], [g.imag, g.real],
                            [gp.real, gp.imag], [gp.imag, -gp.real]]))
    g0 = np.exp(-1j * th * b * (8 * k2))
    g4 = np.exp(-1j * th * b * (4 + 8 * k2))
    l0 = np.concatenate([g0.real, g0.imag, np.cos(th * b * 512), np.zeros((127, 128))], 0)
    l4 = np.concatenate([g4.real, g4.imag, np.zeros((128, 128))], 0)
    lf.append(np.concatenate([l0, l4], 1))
    sc = 1.0 / (S * DB)
    bb = np.arange(128)[:, None]
    kk = np.arange(64)[None, :]
    li = []
    for k1 in (1, 2, 3):
        ph, pp = th * bb * (k1 + 8 * kk), th * bb * (8 - k1 + 8 * kk)
        c, s_, cp, sp = np.cos(ph), np.sin(ph), np.cos(pp), np.sin(pp)
        li.append(2 * sc * np.block([[c, -s_, cp, -sp], [s_, c, -sp, -cp]]))
    ph = th * bb * (8 * kk)
    c0, s0 = 2 * np.cos(ph), -2 * np.sin(ph)
    c0[:, 0] = 1.0
    s0[:, 0] = np.cos(th * bb[:, 0] * 512)
    i0 = sc * np.concatenate([c0, s0], 1)
    ph = th * bb * (4 + 8 * kk)
    i4 = sc * np.concatenate([2 * np.cos(ph), -2 * np.sin(ph)], 1)
    li.append(np.concatenate([np.concatenate([i0, i4], 1), np.zeros((128, 256))], 0))
    lmat = np.concatenate(lf + li, axis=0)
    p = np.arange(128)[None, :]
    kp = np.arange(128)[:, None]
    gf = []
    for q in range(16):
        g = np.exp(-2j * np.pi * (16 * p + q) * kp / S)
        gf.append(np.block([[g.real.T, g.imag.T], [-g.imag.T, g.real.T]]))
    return _np_bf16(lmat), _np_bf16(np.concatenate(gf, 0))


_L_NP, _GF_NP = _make_consts()


_dot = functools.partial(jnp.dot, preferred_element_type=F32)
_dot_nt = functools.partial(lax.dot_general, dimension_numbers=NT, preferred_element_type=F32)


def _t(x):
    return None if x is None else (1, x)


def _tneg(a):
    return None if a is None else (-a[0], a[1])


def _tadd(a, b):
    if a is None:
        return b
    if b is None:
        return a
    if a[0] == b[0]:
        return (a[0], a[1] + b[1])
    return (1, a[1] - b[1]) if a[0] > 0 else (1, b[1] - a[1])


def _tsub(a, b):
    return _tadd(a, _tneg(b))


def _tscale(a, c):
    return None if a is None else (1, a[1] * (c * a[0]))


def _tmul(a, v):
    return None if a is None else (a[0], a[1] * v)


def _tval(a):
    return a[1] if a[0] > 0 else -a[1]


def _twiddle(z, e, n, sign):
    re, im = z
    if e == 0:
        return re, im
    if 4 * e == n:
        return (_tneg(im), re) if sign > 0 else (im, _tneg(re))
    c = math.cos(2.0 * math.pi * e / n)
    s = sign * math.sin(2.0 * math.pi * e / n)
    if 8 * e % n == 0:
        r = abs(c)
        rc = re if c > 0 else _tneg(re)
        rs = re if s > 0 else _tneg(re)
        ic = im if c > 0 else _tneg(im)
        is_ = im if s > 0 else _tneg(im)
        return _tscale(_tsub(rc, is_), r), _tscale(_tadd(rs, ic), r)
    return (_tsub(_tscale(re, c), _tscale(im, s)), _tadd(_tscale(re, s), _tscale(im, c)))


def _fft(zs, sign):
    n = len(zs)
    if n == 1:
        return [zs[0]]
    ev = _fft(zs[0::2], sign)
    od = _fft(zs[1::2], sign)
    out = [None] * n
    for k in range(n // 2):
        t = _twiddle(od[k], k, n, sign)
        out[k] = (_tadd(ev[k][0], t[0]), _tadd(ev[k][1], t[1]))
        out[k + n // 2] = (_tsub(ev[k][0], t[0]), _tsub(ev[k][1], t[1]))
    return out


def _irfft8(t0, t4, t1, t2, t3):
    r = math.sqrt(0.5)
    a0, a1 = t0 + t4, t0 - t4
    e0, e2 = a0 + t2[0], a0 - t2[0]
    e1, e3 = a1 - t2[1], a1 + t2[1]
    o0 = t1[0] + t3[0]
    o2 = t3[1] - t1[1]
    u, v = t1[0] - t3[0], t1[1] + t3[1]
    o1, o3 = (u - v) * r, (-u - v) * r
    return [e0 + o0, e1 + o1, e2 + o2, e3 + o3, e0 - o0, e1 - o1, e2 - o2, e3 - o3]


def _lo_half(w):
    return pltpu.bitcast(w << 16, F32)


def _hi_half(w):
    return pltpu.bitcast(w & jnp.uint32(0xFFFF0000), F32)


def _pack_words(lo, hi):
    lo = pltpu.bitcast(lo.astype(BF16).astype(F32), U32)
    hi = pltpu.bitcast(hi.astype(BF16).astype(F32), U32)
    return (lo >> 16) | hi


def _interleave(gens):
    live = list(gens)
    while live:
        nxt = []
        for g in live:
            try:
                next(g)
                nxt.append(g)
            except StopIteration:
                pass
        live = nxt


def _drain(g):
    for _ in g:
        pass


BQ = 512
KW = 2
NSPLIT = 4
PM = 512
LAG_OUT = 16
F_LAG = 1
F_FILL = 1.0
SCORE_LIMIT = 60.0


def _kernel(x_h, c_h, wq_h, wk_h, wv_h, wo_h, xb_h, wr_h, wi_h, l_h, gf_h,
            out_h,
            x_v, c_v, xs_v, cs_v, wq_raw, wk_raw, wv_raw, wo_v, ws_q, ws_k, ws_v,
            xb_v, wr_v, wi_v, wrn_v, win_v, l_v, gf_v,
            u_v, y_v, z_v,
            acc_v, q_v, k_v, v_v, s_v, nrm_v, bound_s,
            sems, osems, wsems, bsems):
    cp = {}
    nsem = [0]

    def start(name, src, dst, priority=0):
        c = pltpu.make_async_copy(src, dst, sems.at[nsem[0]])
        nsem[0] += 1
        c.start(priority=priority)
        cp[name] = c

    def wait(*names):
        for nm in names:
            cp[nm].wait()

    wq32, wk32, wv32 = wq_h.bitcast(U32), wk_h.bitcast(U32), wv_h.bitcast(U32)

    def pair_copy(t, j):
        src, dst = ((wq32, wq_raw), (wk32, wk_raw), (wv32, wv_raw))[t]
        return pltpu.make_async_copy(src.at[:, j, :], dst.at[j], wsems.at[t, j])

    xb32 = xb_v.bitcast(U32)
    wr32 = wr_v.bitcast(U32)
    wi32 = wi_v.bitcast(U32)

    def word_rows(a, jj):
        return xb32.at[a, pl.ds(pl.multiple_of(4 * jj, 4), 1020)]

    def f1(jj, j0):
        views = [word_rows(a, jj) for a in range(8)]
        for g in range(8):
            words = [v[pl.ds(128 * g + j0, 16, stride=8), :] for v in views]
            for e in range(2):
                half = _lo_half if e == 0 else _hi_half
                o = _fft([(_t(half(w)), None) for w in words], -1)
                r0 = pl.multiple_of((8 * jj + 2 * j0 + e) * 128 + 16 * g, 16)
                parts = [o[0][0], o[4][0], o[1][0], o[1][1], o[2][0], o[2][1], o[3][0], o[3][1]]
                for t in range(8):
                    u_v[pl.ds(r0, 16), t * 128:(t + 1) * 128] = _tval(parts[t]).astype(BF16)

    def f23(q):
        rows = pl.ds(pl.multiple_of(q * 128, 128), 128)
        o = [_dot_nt(l_v[256 * i:256 * (i + 1), :], u_v[rows, 256 * (i + 1):256 * (i + 2)])
             .astype(BF16) for i in range(3)]
        o0 = _dot_nt(l_v[768:912, 0:128], u_v[rows, 0:128]).astype(BF16)
        o4 = _dot_nt(l_v[768:896, 128:256], u_v[rows, 128:256]).astype(BF16)

        def blk(k1, part):
            if k1 == 0:
                return o0[64 * part:64 * part + 64]
            if k1 == 4:
                return o4[64 * part:64 * part + 64]
            if k1 < 4:
                return o[k1 - 1][64 * part:64 * part + 64]
            return o[7 - k1][128 + 64 * part:128 + 64 * part + 64]

        re = jnp.concatenate([blk(k1, 0) for k1 in range(8)] + [o0[128:144]], axis=0)
        im = jnp.concatenate([blk(k1, 1) for k1 in range(8)] + [jnp.zeros((16, 128), BF16)],
                             axis=0)
        y_v[q] = _dot(jnp.concatenate([re, im], axis=1),
                      gf_v[pl.ds(pl.multiple_of(q * 256, 256), 256), :])

    def mid(rows, filt):
        xf = _fft([(_t(y_v[q, rows, 0:128]), _t(y_v[q, rows, 128:256])) for q in range(16)], -1)
        zs = []
        for kq in range(16):
            fr, fi = filt(kq)
            re, im = xf[kq]
            zs.append((_tsub(_tmul(re, fr), _tmul(im, fi)), _tadd(_tmul(re, fi), _tmul(im, fr))))
        us = _fft(zs, +1)
        for q in range(16):
            z_v[q, rows, 0:128] = _tval(us[q][0]).astype(BF16)
            z_v[q, rows, 128:256] = _tval(us[q][1]).astype(BF16)

    def mid_group(g2, k1s):
        base = pl.multiple_of(64 * g2, 64)
        for k1 in k1s:
            half = _lo_half if k1 % 2 == 0 else _hi_half
            sl = pl.ds(k1 // 2, 16, stride=4)

            def filt(kq):
                return (half(wr32.at[kq, pl.ds(base, 64)][sl, :]),
                        half(wi32.at[kq, pl.ds(base, 64)][sl, :]))

            mid(pl.ds(pl.multiple_of(64 * k1 + 16 * g2, 16), 16), filt)

    def mid_nyquist():
        def filt(kq):
            cs = slice(kq * 128, (kq + 1) * 128)
            return (jnp.broadcast_to(wrn_v[:, cs].astype(F32), (16, 128)),
                    jnp.broadcast_to(win_v[:, cs].astype(F32), (16, 128)))

        mid(slice(512, KR), filt)

    srow = lax.broadcasted_iota(jnp.int32, (64, 128), 0)

    def i32(jj, j0):
        ys = []
        for e in range(2):
            q = 8 * jj + 2 * j0 + e
            z = _dot_nt(z_v[q], gf_v[pl.ds(pl.multiple_of(q * 256, 256), 256), :])
            zr, zi = z[:, 0:128], z[:, 128:256]
            zi0 = jnp.where(srow == 0, jnp.broadcast_to(zr[512:513], (64, 128)), zi[0:64])
            rhs0 = jnp.concatenate([zr[0:64], zi0], axis=0).astype(BF16)
            t0 = _dot(l_v[1792:1920, 0:128], rhs0)
            rhs4 = jnp.concatenate([zr[256:320], zi[256:320]], axis=0).astype(BF16)
            t4 = _dot(l_v[1792:1920, 128:256], rhs4)
            ts = []
            for k1 in (1, 2, 3):
                kc = 8 - k1
                rhs = jnp.concatenate([zr[64 * k1:64 * k1 + 64], zi[64 * k1:64 * k1 + 64],
                                       zr[64 * kc:64 * kc + 64], zi[64 * kc:64 * kc + 64]],
                                      axis=0).astype(BF16)
                o = _dot(l_v[1024 + 256 * (k1 - 1):1024 + 256 * k1, :], rhs)
                ts.append((o[0:128], o[128:256]))
            ys.append(_irfft8(t0, t4, *ts))
        for a in range(8):
            word_rows(a, jj)[pl.ds(j0, 128, stride=8), :] = _pack_words(ys[0][a], ys[1][a]).T

    nq = S // BQ
    nsub = BQ // 128
    row = lax.broadcasted_iota(jnp.int32, (128, 128), 0)
    col = lax.broadcasted_iota(jnp.int32, (128, 128), 1)
    tri = col <= row
    qscale = (D ** -0.5) * math.log2(math.e)

    def mx(a, b):
        return b if a is None else jnp.maximum(a, b)

    def addn(a, b):
        return b if a is None else a + b

    class St:
        pass

    def split_inputs(src, dst):
        n = src.shape[1] // 2

        def chunk(i, carry):
            top = pl.ds(pl.multiple_of(i * 128, 128), 128)
            bot = pl.ds(pl.multiple_of(S // 2 + i * 128, 128), 128)
            a11, a12 = src[top, 0:n].astype(F32), src[top, n:].astype(F32)
            a21, a22 = src[bot, 0:n].astype(F32), src[bot, n:].astype(F32)
            for t, v in enumerate((a11 + a22, a21 + a22, a11 + a12, a21 - a11, a12 - a22)):
                dst[t, top, :] = v.astype(BF16)
            return carry

        lax.fori_loop(0, S // 256, chunk, 0)

    def unpack_weights(j):
        def unpack(raw, w, r0):
            n = w.shape[1]
            rows = pl.ds(pl.multiple_of(r0, 64), 64)
            up, dn = raw[j, rows, :], raw[j, pl.ds(pl.multiple_of(n + r0, 64), 64), :]
            b11, b12, b21, b22 = _lo_half(up), _hi_half(up), _lo_half(dn), _hi_half(dn)
            for t, v in enumerate((b11 + b22, b11, b12 - b22, b21 - b11, b22,
                                   b11 + b12, b21 + b22)):
                w[t, rows, :] = v.astype(BF16)

        def chunk(i, carry):
            unpack(wq_raw, ws_q, i * 128)
            unpack(wq_raw, ws_q, i * 128 + 64)
            unpack(wk_raw, ws_k, i * 64)
            unpack(wv_raw, ws_v, i * 64)
            return carry

        lax.fori_loop(0, 4, chunk, 0)

    def track(nrm, name, a):
        n2 = jnp.max(jnp.sum(a * a, axis=1, keepdims=True), axis=0, keepdims=True)
        nrm[name] = mx(nrm.get(name), n2)

    def publish(nrm, base, e):
        for t in range(2):
            for w, name in enumerate(("q", "k")):
                old = jnp.where(e == 0, 0.0, nrm_v[base + t, w])
                nrm_v[base + t, w] = jnp.maximum(old, jnp.broadcast_to(nrm[name, t], (8, 128)))

    def set_bound(h):
        bound_s[0] = jnp.max(nrm_v[h & 3, 0] * nrm_v[h & 3, 1])

    def proj(name, src, sums, w, dst, scale, base, r0, nrm):
        n = w.shape[1]
        top = pl.ds(pl.multiple_of(r0, PM), PM)
        bot = pl.ds(pl.multiple_of(S // 2 + r0, PM), PM)
        m1 = _dot(sums[0, top, :], w[0])
        m2 = _dot(sums[1, top, :], w[1])
        m3 = _dot(src[top, 0:n], w[2])
        m4 = _dot(src[bot, n:], w[3])
        m5 = _dot(sums[2, top, :], w[4])
        m6 = _dot(sums[3, top, :], w[5])
        m7 = _dot(sums[4, top, :], w[6])
        outs = ((0, top, (m1 + m4) + (m7 - m5)), (1, top, m3 + m5),
                (0, bot, m2 + m4), (1, bot, (m1 - m2) + (m3 + m6)))
        for t, rows, val in outs:
            if scale is not None:
                val = val * scale
            if name is not None:
                track(nrm, (name, t), val)
            dst[base + t, rows, :] = val.astype(BF16)

    def proj_steps(base, e):
        steps, nrm = [], {}
        for i in range(S // 4 // PM):
            r0 = e * (S // 4) + i * PM
            steps.append((7 * 4 * PM // 128,
                          functools.partial(proj, "q", x_v, xs_v, ws_q, q_v, qscale, base, r0, nrm)))
            steps.append((7 * 2 * PM // 128,
                          functools.partial(proj, "k", c_v, cs_v, ws_k, k_v, None, base, r0, nrm)))
            steps.append((7 * 2 * PM // 128,
                          functools.partial(proj, None, c_v, cs_v, ws_v, v_v, None, base, r0, nrm)))
        steps.append((0, functools.partial(publish, nrm, base, e)))
        return steps

    pending = []

    def out_steps(h, i, st, last, nsplit=NSPLIT):
        rows = slice(i * BQ, (i + 1) * BQ)
        w = M // nsplit

        def step(t):
            cs = slice(t * w, (t + 1) * w)
            o = acc_v[rows, cs] + _dot(st.ctx, wo_v[pl.ds(pl.multiple_of(h * D, D), D), cs])
            acc_v[rows, cs] = o
            if last:
                u_v[rows, cs] = o.astype(BF16)
                out_copy(i, t).start()

        return [(nsub * w // 128, functools.partial(step, t)) for t in range(nsplit)]

    def fast_tiles(i, st, slot):
        r0 = i * BQ
        ntf = r0 // 128
        lacc = [None] * nsub
        acc = [None] * nsub
        left = [ntf + nsub]
        tiles = []

        def done(n):
            left[0] -= n
            if left[0] == 0:
                l = jnp.sum(jnp.concatenate(lacc, axis=0), axis=1, keepdims=True)
                st.ctx = (jnp.concatenate(acc, axis=0) / l).astype(BF16)

        def add_tile(t, c0, w):
            box = []

            def qk_exp():
                s = _dot_nt(q_v[slot, r0 + t * 128:r0 + BQ, :], k_v[slot, c0:c0 + w * 128, :])
                if c0 >= r0:
                    s0 = jnp.where(tri, s[:128], NEG)
                    s = jnp.concatenate([s0, s[128:]], axis=0) if t < nsub - 1 else s0
                p = jnp.exp2(s)
                for u in range(t, nsub):
                    lacc[u] = addn(lacc[u], functools.reduce(jnp.add, [
                        p[(u - t) * 128:(u - t + 1) * 128, j * 128:(j + 1) * 128]
                        for j in range(w)]))
                box.append(p.astype(BF16))

            def pv():
                o = _dot(box.pop(), v_v[slot, c0:c0 + w * 128, :])
                for u in range(t, nsub):
                    acc[u] = addn(acc[u], o[(u - t) * 128:(u - t + 1) * 128])
                done(w)

            tiles.append((w * (nsub - t), qk_exp, pv))

        kt = 0
        while kt < ntf:
            w = min(KW, ntf - kt)
            add_tile(0, kt * 128, w)
            kt += w
        for t in range(nsub):
            add_tile(t, r0 + t * 128, 1)
        return tiles

    def head_fast(h, slot, proj, last=False):
        sts = [St() for _ in range(nq)]
        order = list(range(nq))[::-1]
        tiles, ends = [], {}
        for i in order:
            tiles += fast_tiles(i, sts[i], slot)
            ends[len(tiles) - 1] = i
        proj = list(proj)
        outs = []
        t = [0.0]
        attn = 2 * sum(c for c, _, _ in tiles)
        fill = sum(c for c, _ in proj) + nq * nsub * (M // 128)
        debt = [0.0]

        def filler(force=False):
            while debt[0] > 0 or force:
                if outs and (outs[0][0] <= t[0] or not proj):
                    _, c, fn = outs.pop(0)
                elif proj:
                    c, fn = proj.pop(0)
                else:
                    return
                fn()
                t[0] += c
                debt[0] -= c

        n = len(tiles)
        for k in range(n + F_LAG):
            c = 0
            if k < n:
                tiles[k][1]()
                c += tiles[k][0]
            if k >= F_LAG:
                tiles[k - F_LAG][2]()
                c += tiles[k - F_LAG][0]
            t[0] += c
            if k - F_LAG in ends:
                i = ends[k - F_LAG]
                outs += [(t[0] + LAG_OUT, cc, fn) for cc, fn in out_steps(h, i, sts[i], last)]
            debt[0] += c * fill / attn * F_FILL
            filler()
        filler(force=True)

    def head_safe(h, slot, last=False):
        rr = lax.broadcasted_iota(jnp.int32, (256, 256), 0)
        cc = lax.broadcasted_iota(jnp.int32, (256, 256), 1)

        def q_block(qi, carry):
            rows = pl.ds(pl.multiple_of(qi * 256, 256), 256)
            q = q_v[slot, rows, :]

            def kv_block(kt, mla):
                m, l, acc = mla
                cols = pl.ds(pl.multiple_of(kt * 256, 256), 256)
                s = _dot_nt(q, k_v[slot, cols, :])
                s = jnp.where(cc + (kt - qi) * 256 <= rr, s, NEG)
                m_new = jnp.maximum(m, jnp.max(s, axis=1, keepdims=True))
                alpha = jnp.exp2(m - m_new)
                p = jnp.exp2(s - m_new)
                l = alpha * l + jnp.sum(p, axis=1, keepdims=True)
                acc = alpha * acc + _dot(p.astype(BF16), v_v[slot, cols, :])
                return m_new, l, acc

            init = (jnp.full((256, 1), NEG, F32), jnp.zeros((256, 1), F32),
                    jnp.zeros((256, D), F32))
            _, l, acc = lax.fori_loop(0, qi + 1, kv_block, init)
            ctx = (acc / l).astype(BF16)
            o = acc_v[rows, :] + _dot(ctx, wo_v[pl.ds(pl.multiple_of(h * D, D), D), :])
            acc_v[rows, :] = o
            if last:
                u_v[rows, :] = o.astype(BF16)
            return carry

        lax.fori_loop(0, S // 256, q_block, 0)

    def out_copy(i, t):
        w = M // NSPLIT
        rows, cs = slice(i * BQ, (i + 1) * BQ), slice(t * w, (t + 1) * w)
        return pltpu.make_async_copy(u_v.at[rows, cs], out_h.at[rows, cs],
                                     osems.at[i * NSPLIT + t])

    def head(h, last=False):
        slot = h & 3
        small = bound_s[0] <= SCORE_LIMIT ** 2

        def next_pair():
            if last:
                return []
            return proj_steps(2 - (h & 2), h & 1)

        @pl.when(small)
        def _():
            head_fast(h, slot, next_pair(), last)
            set_bound(h + 1)

        @pl.when(jnp.logical_not(small))
        def _():
            head_safe(h, slot, last)
            for _, fn in next_pair():
                fn()
            set_bound(h + 1)
            if last:
                for i in range(nq):
                    for t in range(NSPLIT):
                        out_copy(i, t).start()

    for a in range(8):
        start(f"xb{a}", xb_h.at[:, a * 128:(a + 1) * 128], xb_v.at[a])
    start("l", l_h, l_v)
    start("gf", gf_h, gf_v)
    for t in range(16):
        start(f"wr{t}", wr_h.at[0:512, t * 128:(t + 1) * 128], wr_v.at[t])
        start(f"wi{t}", wi_h.at[0:512, t * 128:(t + 1) * 128], wi_v.at[t])
    start("wrn", wr_h.at[512:513, :], wrn_v)
    start("win", wi_h.at[512:513, :], win_v)
    start("c", c_h, c_v)
    start("x", x_h, x_v)
    for t in range(3):
        pair_copy(t, 0).start()
    start("wo", wo_h, wo_v)
    s_v[...] = jnp.zeros(s_v.shape, F32)
    for i in range(S // 512):
        start(f"z{i}", s_v, acc_v.at[i * 512:(i + 1) * 512], priority=1)
    wait(*[f"xb{a}" for a in range(8)], "l", "gf")

    def fwd_half(jj, carry):
        for i in range(7):
            for t in range(3):
                pair_copy(t, 7 * jj + i + 1).start()
        f1(jj, 0)
        for j0 in range(4):
            if j0 + 1 < 4:
                f1(jj, j0 + 1)
            f23(8 * jj + 2 * j0)
            f23(8 * jj + 2 * j0 + 1)
        return carry

    lax.fori_loop(0, 2, fwd_half, 0)

    for t in range(3):
        pair_copy(t, H // 2 - 1).start()
    wait(*[f"wr{t}" for t in range(16)], *[f"wi{t}" for t in range(16)], "wrn", "win")
    def mid_quarter(g2, carry):
        mid_group(g2, range(8))
        return carry

    lax.fori_loop(0, 4, mid_quarter, 0)
    mid_nyquist()

    wait("c", "x")
    for t in range(3):
        pair_copy(t, 0).wait()
    split_inputs(x_v, xs_v)
    split_inputs(c_v, cs_v)
    unpack_weights(0)

    def inv_half(jj, carry):
        merge = proj_steps(0, jj)
        for j0 in range(4):
            i32(jj, j0)
            for _, fn in merge[len(merge) * j0 // 4:len(merge) * (j0 + 1) // 4]:
                fn()
        return carry

    lax.fori_loop(0, 2, inv_half, 0)
    for a in range(8):
        c = pltpu.make_async_copy(xb_v.at[a], out_h.at[:, M + a * 128:M + (a + 1) * 128],
                                  bsems.at[a])
        c.start()
        pending.append(c)

    wait("wo", *[f"z{i}" for i in range(S // 512)])
    set_bound(0)
    def body(h, carry):
        @pl.when((h & 1) == 0)
        def _():
            for t in range(3):
                pair_copy(t, (h >> 1) + 1).wait()
            unpack_weights((h >> 1) + 1)

        head(h)
        return carry

    lax.fori_loop(0, H - 2, body, 0)
    def tail(h, carry):
        @pl.when(h == H - 1)
        def _():
            for i in range(nq):
                for t in range(NSPLIT):
                    out_copy(i, t).wait()

        head(h, last=True)
        return carry

    lax.fori_loop(H - 2, H, tail, 0)
    for c in pending:
        c.wait()
    for i in range(nq):
        for t in range(NSPLIT):
            out_copy(i, t).wait()


@jax.jit
def pallas_concat_heads__compressed_kv_cla__spectral_gfnet__prompt_kernel(
    A_x: jax.Array,
    A_c_kv: jax.Array,
    A_w_q: jax.Array,
    A_w_uk: jax.Array,
    A_w_uv: jax.Array,
    A_w_o: jax.Array,
    B_x: jax.Array,
    B_w_r: jax.Array,
    B_w_i: jax.Array,
):
    vm = pltpu.VMEM
    scratch = [
        vm((S, M), BF16), vm((S, C), BF16),
        vm((5, S // 2, M // 2), BF16), vm((5, S // 2, C // 2), BF16),
        vm((H // 2, M, D), U32), vm((H // 2, C, D), U32), vm((H // 2, C, D), U32),
        vm((H * D, M), BF16),
        vm((7, M // 2, D), BF16), vm((7, C // 2, D), BF16), vm((7, C // 2, D), BF16),
        vm((8, S, 128), BF16),
        vm((16, 512, 128), BF16), vm((16, 512, 128), BF16),
        vm((1, S), BF16), vm((1, S), BF16),
        vm(_L_NP.shape, BF16), vm(_GF_NP.shape, BF16),
        vm((S, 1024), BF16),
        vm((16, KR, 256), F32), vm((16, KR, 256), BF16),
        vm((S, M), F32),
        vm((4, S, D), BF16), vm((4, S, D), BF16), vm((4, S, D), BF16),
        vm((512, M), F32),
        vm((4, 2, 8, 128), F32), pltpu.SMEM((1,), F32),
        pltpu.SemaphoreType.DMA((64,)),
        pltpu.SemaphoreType.DMA((16,)),
        pltpu.SemaphoreType.DMA((3, H // 2)),
        pltpu.SemaphoreType.DMA((8,)),
    ]
    anyspec = pl.BlockSpec(memory_space=pl.ANY)
    out = pl.pallas_call(
        _kernel,
        out_shape=jax.ShapeDtypeStruct((S, M + DB), BF16),
        in_specs=[anyspec] * 11,
        out_specs=anyspec,
        scratch_shapes=scratch,
        compiler_params=pltpu.CompilerParams(vmem_limit_bytes=122 * 1024 * 1024),
        name="mla_gfnet_fused",
    )(
        A_x.reshape(S, M), A_c_kv.reshape(S, C), A_w_q, A_w_uk, A_w_uv,
        A_w_o.reshape(H * D, M),
        B_x.reshape(S, DB), B_w_r.T, B_w_i.T,
        jnp.asarray(_L_NP), jnp.asarray(_GF_NP),
    )
    return out.reshape(1, S, M + DB)
```

```python
import functools
import math

import numpy as np
import jax
import jax.numpy as jnp
from jax import lax
import jax.experimental.pallas as pl
import jax.experimental.pallas.tpu as pltpu

S = 2048
M = 1024
H = 32
D = 128
C = 512
DB = 1024
KR = 528

F32 = jnp.float32
BF16 = jnp.bfloat16
U32 = jnp.uint32
NT = (((1,), (1,)), ((), ()))
NEG = -1e30


def _np_bf16(a):
    return np.asarray(a, np.float32).astype(jnp.bfloat16)


def _make_consts():
    th = 2.0 * np.pi / DB
    b = np.arange(128)[None, :]
    k2 = np.arange(64)[:, None]
    lf = []
    for k1 in (1, 2, 3):
        g = np.exp(-1j * th * b * (k1 + 8 * k2))
        gp = np.exp(-1j * th * b * (8 - k1 + 8 * k2))
        lf.append(np.block([[g.real, -g.imag], [g.imag, g.real],
                            [gp.real, gp.imag], [gp.imag, -gp.real]]))
    g0 = np.exp(-1j * th * b * (8 * k2))
    g4 = np.exp(-1j * th * b * (4 + 8 * k2))
    l0 = np.concatenate([g0.real, g0.imag, np.cos(th * b * 512), np.zeros((127, 128))], 0)
    l4 = np.concatenate([g4.real, g4.imag, np.zeros((128, 128))], 0)
    lf.append(np.concatenate([l0, l4], 1))
    sc = 1.0 / (S * DB)
    bb = np.arange(128)[:, None]
    kk = np.arange(64)[None, :]
    li = []
    for k1 in (1, 2, 3):
        ph, pp = th * bb * (k1 + 8 * kk), th * bb * (8 - k1 + 8 * kk)
        c, s_, cp, sp = np.cos(ph), np.sin(ph), np.cos(pp), np.sin(pp)
        li.append(2 * sc * np.block([[c, -s_, cp, -sp], [s_, c, -sp, -cp]]))
    ph = th * bb * (8 * kk)
    c0, s0 = 2 * np.cos(ph), -2 * np.sin(ph)
    c0[:, 0] = 1.0
    s0[:, 0] = np.cos(th * bb[:, 0] * 512)
    i0 = sc * np.concatenate([c0, s0], 1)
    ph = th * bb * (4 + 8 * kk)
    i4 = sc * np.concatenate([2 * np.cos(ph), -2 * np.sin(ph)], 1)
    li.append(np.concatenate([np.concatenate([i0, i4], 1), np.zeros((128, 256))], 0))
    lmat = np.concatenate(lf + li, axis=0)
    p = np.arange(128)[None, :]
    kp = np.arange(128)[:, None]
    gf = []
    for q in range(16):
        g = np.exp(-2j * np.pi * (16 * p + q) * kp / S)
        gf.append(np.block([[g.real.T, g.imag.T], [-g.imag.T, g.real.T]]))
    return _np_bf16(lmat), _np_bf16(np.concatenate(gf, 0))


_L_NP, _GF_NP = _make_consts()


_dot = functools.partial(jnp.dot, preferred_element_type=F32)
_dot_nt = functools.partial(lax.dot_general, dimension_numbers=NT, preferred_element_type=F32)


def _t(x):
    return None if x is None else (1, x)


def _tneg(a):
    return None if a is None else (-a[0], a[1])


def _tadd(a, b):
    if a is None:
        return b
    if b is None:
        return a
    if a[0] == b[0]:
        return (a[0], a[1] + b[1])
    return (1, a[1] - b[1]) if a[0] > 0 else (1, b[1] - a[1])


def _tsub(a, b):
    return _tadd(a, _tneg(b))


def _tscale(a, c):
    return None if a is None else (1, a[1] * (c * a[0]))


def _tmul(a, v):
    return None if a is None else (a[0], a[1] * v)


def _tval(a):
    return a[1] if a[0] > 0 else -a[1]


def _twiddle(z, e, n, sign):
    re, im = z
    if e == 0:
        return re, im
    if 4 * e == n:
        return (_tneg(im), re) if sign > 0 else (im, _tneg(re))
    c = math.cos(2.0 * math.pi * e / n)
    s = sign * math.sin(2.0 * math.pi * e / n)
    if 8 * e % n == 0:
        r = abs(c)
        rc = re if c > 0 else _tneg(re)
        rs = re if s > 0 else _tneg(re)
        ic = im if c > 0 else _tneg(im)
        is_ = im if s > 0 else _tneg(im)
        return _tscale(_tsub(rc, is_), r), _tscale(_tadd(rs, ic), r)
    return (_tsub(_tscale(re, c), _tscale(im, s)), _tadd(_tscale(re, s), _tscale(im, c)))


def _fft(zs, sign):
    n = len(zs)
    if n == 1:
        return [zs[0]]
    ev = _fft(zs[0::2], sign)
    od = _fft(zs[1::2], sign)
    out = [None] * n
    for k in range(n // 2):
        t = _twiddle(od[k], k, n, sign)
        out[k] = (_tadd(ev[k][0], t[0]), _tadd(ev[k][1], t[1]))
        out[k + n // 2] = (_tsub(ev[k][0], t[0]), _tsub(ev[k][1], t[1]))
    return out


def _irfft8(t0, t4, t1, t2, t3):
    r = math.sqrt(0.5)
    a0, a1 = t0 + t4, t0 - t4
    e0, e2 = a0 + t2[0], a0 - t2[0]
    e1, e3 = a1 - t2[1], a1 + t2[1]
    o0 = t1[0] + t3[0]
    o2 = t3[1] - t1[1]
    u, v = t1[0] - t3[0], t1[1] + t3[1]
    o1, o3 = (u - v) * r, (-u - v) * r
    return [e0 + o0, e1 + o1, e2 + o2, e3 + o3, e0 - o0, e1 - o1, e2 - o2, e3 - o3]


def _lo_half(w):
    return pltpu.bitcast(w << 16, F32)


def _hi_half(w):
    return pltpu.bitcast(w & jnp.uint32(0xFFFF0000), F32)


def _pack_words(lo, hi):
    lo = pltpu.bitcast(lo.astype(BF16).astype(F32), U32)
    hi = pltpu.bitcast(hi.astype(BF16).astype(F32), U32)
    return (lo >> 16) | hi


def _interleave(gens):
    live = list(gens)
    while live:
        nxt = []
        for g in live:
            try:
                next(g)
                nxt.append(g)
            except StopIteration:
                pass
        live = nxt


def _drain(g):
    for _ in g:
        pass


BQ = 512
KW = 2
NSPLIT = 4
PM = 512
LAG_OUT = 16
F_LAG = 1
F_FILL = 1.0
SCORE_LIMIT = 60.0


def _kernel(x_h, c_h, wq_h, wk_h, wv_h, wo_h, xb_h, wr_h, wi_h, l_h, gf_h,
            out_h,
            x_v, c_v, xs_v, cs_v, wq_raw, wk_raw, wv_raw, wo_v, ws_q, ws_k, ws_v,
            xb_v, wr_v, wi_v, wrn_v, win_v, l_v, gf_v,
            u_v, y_v, z_v,
            acc_v, q_v, k_v, v_v, s_v, nrm_v, bound_s,
            sems, osems, wsems, bsems):
    cp = {}
    nsem = [0]

    def start(name, src, dst, priority=0):
        c = pltpu.make_async_copy(src, dst, sems.at[nsem[0]])
        nsem[0] += 1
        c.start(priority=priority)
        cp[name] = c

    def wait(*names):
        for nm in names:
            cp[nm].wait()

    wq32, wk32, wv32 = wq_h.bitcast(U32), wk_h.bitcast(U32), wv_h.bitcast(U32)

    def pair_copy(t, j):
        src, dst = ((wq32, wq_raw), (wk32, wk_raw), (wv32, wv_raw))[t]
        return pltpu.make_async_copy(src.at[:, j, :], dst.at[j], wsems.at[t, j])

    xb32 = xb_v.bitcast(U32)
    wr32 = wr_v.bitcast(U32)
    wi32 = wi_v.bitcast(U32)

    def word_rows(a, jj):
        return xb32.at[a, pl.ds(pl.multiple_of(4 * jj, 4), 1020)]

    def f1(jj, j0):
        views = [word_rows(a, jj) for a in range(8)]
        for g in range(8):
            words = [v[pl.ds(128 * g + j0, 16, stride=8), :] for v in views]
            for e in range(2):
                half = _lo_half if e == 0 else _hi_half
                o = _fft([(_t(half(w)), None) for w in words], -1)
                r0 = pl.multiple_of((8 * jj + 2 * j0 + e) * 128 + 16 * g, 16)
                parts = [o[0][0], o[4][0], o[1][0], o[1][1], o[2][0], o[2][1], o[3][0], o[3][1]]
                for t in range(8):
                    u_v[pl.ds(r0, 16), t * 128:(t + 1) * 128] = _tval(parts[t]).astype(BF16)

    def f23(q):
        rows = pl.ds(pl.multiple_of(q * 128, 128), 128)
        o = [_dot_nt(l_v[256 * i:256 * (i + 1), :], u_v[rows, 256 * (i + 1):256 * (i + 2)])
             .astype(BF16) for i in range(3)]
        o0 = _dot_nt(l_v[768:912, 0:128], u_v[rows, 0:128]).astype(BF16)
        o4 = _dot_nt(l_v[768:896, 128:256], u_v[rows, 128:256]).astype(BF16)

        def blk(k1, part):
            if k1 == 0:
                return o0[64 * part:64 * part + 64]
            if k1 == 4:
                return o4[64 * part:64 * part + 64]
            if k1 < 4:
                return o[k1 - 1][64 * part:64 * part + 64]
            return o[7 - k1][128 + 64 * part:128 + 64 * part + 64]

        re = jnp.concatenate([blk(k1, 0) for k1 in range(8)] + [o0[128:144]], axis=0)
        im = jnp.concatenate([blk(k1, 1) for k1 in range(8)] + [jnp.zeros((16, 128), BF16)],
                             axis=0)
        y_v[q] = _dot(jnp.concatenate([re, im], axis=1),
                      gf_v[pl.ds(pl.multiple_of(q * 256, 256), 256), :])

    def mid(rows, filt):
        xf = _fft([(_t(y_v[q, rows, 0:128]), _t(y_v[q, rows, 128:256])) for q in range(16)], -1)
        zs = []
        for kq in range(16):
            fr, fi = filt(kq)
            re, im = xf[kq]
            zs.append((_tsub(_tmul(re, fr), _tmul(im, fi)), _tadd(_tmul(re, fi), _tmul(im, fr))))
        us = _fft(zs, +1)
        for q in range(16):
            z_v[q, rows, 0:128] = _tval(us[q][0]).astype(BF16)
            z_v[q, rows, 128:256] = _tval(us[q][1]).astype(BF16)

    def mid_group(g2, k1s):
        base = pl.multiple_of(64 * g2, 64)
        for k1 in k1s:
            half = _lo_half if k1 % 2 == 0 else _hi_half
            sl = pl.ds(k1 // 2, 16, stride=4)

            def filt(kq):
                return (half(wr32.at[kq, pl.ds(base, 64)][sl, :]),
                        half(wi32.at[kq, pl.ds(base, 64)][sl, :]))

            mid(pl.ds(pl.multiple_of(64 * k1 + 16 * g2, 16), 16), filt)

    def mid_nyquist():
        def filt(kq):
            cs = slice(kq * 128, (kq + 1) * 128)
            return (jnp.broadcast_to(wrn_v[:, cs].astype(F32), (16, 128)),
                    jnp.broadcast_to(win_v[:, cs].astype(F32), (16, 128)))

        mid(slice(512, KR), filt)

    srow = lax.broadcasted_iota(jnp.int32, (64, 128), 0)

    def i32(jj, j0):
        ys = []
        for e in range(2):
            q = 8 * jj + 2 * j0 + e
            z = _dot_nt(z_v[q], gf_v[pl.ds(pl.multiple_of(q * 256, 256), 256), :])
            zr, zi = z[:, 0:128], z[:, 128:256]
            zi0 = jnp.where(srow == 0, jnp.broadcast_to(zr[512:513], (64, 128)), zi[0:64])
            rhs0 = jnp.concatenate([zr[0:64], zi0], axis=0).astype(BF16)
            t0 = _dot(l_v[1792:1920, 0:128], rhs0)
            rhs4 = jnp.concatenate([zr[256:320], zi[256:320]], axis=0).astype(BF16)
            t4 = _dot(l_v[1792:1920, 128:256], rhs4)
            ts = []
            for k1 in (1, 2, 3):
                kc = 8 - k1
                rhs = jnp.concatenate([zr[64 * k1:64 * k1 + 64], zi[64 * k1:64 * k1 + 64],
                                       zr[64 * kc:64 * kc + 64], zi[64 * kc:64 * kc + 64]],
                                      axis=0).astype(BF16)
                o = _dot(l_v[1024 + 256 * (k1 - 1):1024 + 256 * k1, :], rhs)
                ts.append((o[0:128], o[128:256]))
            ys.append(_irfft8(t0, t4, *ts))
        for a in range(8):
            word_rows(a, jj)[pl.ds(j0, 128, stride=8), :] = _pack_words(ys[0][a], ys[1][a]).T

    nq = S // BQ
    nsub = BQ // 128
    row = lax.broadcasted_iota(jnp.int32, (128, 128), 0)
    col = lax.broadcasted_iota(jnp.int32, (128, 128), 1)
    tri = col <= row
    qscale = (D ** -0.5) * math.log2(math.e)

    def mx(a, b):
        return b if a is None else jnp.maximum(a, b)

    def addn(a, b):
        return b if a is None else a + b

    class St:
        pass

    def split_inputs(src, dst):
        n = src.shape[1] // 2

        def chunk(i, carry):
            top = pl.ds(pl.multiple_of(i * 128, 128), 128)
            bot = pl.ds(pl.multiple_of(S // 2 + i * 128, 128), 128)
            a11, a12 = src[top, 0:n].astype(F32), src[top, n:].astype(F32)
            a21, a22 = src[bot, 0:n].astype(F32), src[bot, n:].astype(F32)
            for t, v in enumerate((a11 + a22, a21 + a22, a11 + a12, a21 - a11, a12 - a22)):
                dst[t, top, :] = v.astype(BF16)
            return carry

        lax.fori_loop(0, S // 256, chunk, 0)

    def unpack_weights(j):
        def unpack(raw, w, r0):
            n = w.shape[1]
            rows = pl.ds(pl.multiple_of(r0, 64), 64)
            up, dn = raw[j, rows, :], raw[j, pl.ds(pl.multiple_of(n + r0, 64), 64), :]
            b11, b12, b21, b22 = _lo_half(up), _hi_half(up), _lo_half(dn), _hi_half(dn)
            for t, v in enumerate((b11 + b22, b11, b12 - b22, b21 - b11, b22,
                                   b11 + b12, b21 + b22)):
                w[t, rows, :] = v.astype(BF16)

        def chunk(i, carry):
            unpack(wq_raw, ws_q, i * 128)
            unpack(wq_raw, ws_q, i * 128 + 64)
            unpack(wk_raw, ws_k, i * 64)
            unpack(wv_raw, ws_v, i * 64)
            return carry

        lax.fori_loop(0, 4, chunk, 0)

    def track(nrm, name, a):
        n2 = jnp.max(jnp.sum(a * a, axis=1, keepdims=True), axis=0, keepdims=True)
        nrm[name] = mx(nrm.get(name), n2)

    def publish(nrm, base, first):
        for t in range(2):
            for w, name in enumerate(("q", "k")):
                old = jnp.where(first, 0.0, nrm_v[base + t, w])
                nrm_v[base + t, w] = jnp.maximum(old, jnp.broadcast_to(nrm[name, t], (8, 128)))

    def set_bound(h):
        bound_s[0] = jnp.max(nrm_v[h & 3, 0] * nrm_v[h & 3, 1])

    def proj(name, src, sums, w, dst, scale, base, r0, nrm, pm=PM):
        n = w.shape[1]
        top = pl.ds(pl.multiple_of(r0, pm), pm)
        bot = pl.ds(pl.multiple_of(S // 2 + r0, pm), pm)
        m1 = _dot(sums[0, top, :], w[0])
        m2 = _dot(sums[1, top, :], w[1])
        m3 = _dot(src[top, 0:n], w[2])
        m4 = _dot(src[bot, n:], w[3])
        m5 = _dot(sums[2, top, :], w[4])
        m6 = _dot(sums[3, top, :], w[5])
        m7 = _dot(sums[4, top, :], w[6])
        outs = ((0, top, (m1 + m4) + (m7 - m5)), (1, top, m3 + m5),
                (0, bot, m2 + m4), (1, bot, (m1 - m2) + (m3 + m6)))
        for t, rows, val in outs:
            if scale is not None:
                val = val * scale
            if name is not None:
                track(nrm, (name, t), val)
            dst[base + t, rows, :] = val.astype(BF16)

    def proj_steps(base, e):
        steps, nrm = [], {}
        for i in range(S // 4 // PM):
            r0 = e * (S // 4) + i * PM
            steps.append((7 * 4 * PM // 128,
                          functools.partial(proj, "q", x_v, xs_v, ws_q, q_v, qscale, base, r0, nrm)))
            steps.append((7 * 2 * PM // 128,
                          functools.partial(proj, "k", c_v, cs_v, ws_k, k_v, None, base, r0, nrm)))
            steps.append((7 * 2 * PM // 128,
                          functools.partial(proj, None, c_v, cs_v, ws_v, v_v, None, base, r0, nrm)))
        steps.append((0, functools.partial(publish, nrm, base, e == 0)))
        return steps

    pending = []

    def out_steps(h, i, st, last, nsplit=NSPLIT):
        rows = slice(i * BQ, (i + 1) * BQ)
        w = M // nsplit

        def step(t):
            cs = slice(t * w, (t + 1) * w)
            o = acc_v[rows, cs] + _dot(st.ctx, wo_v[pl.ds(pl.multiple_of(h * D, D), D), cs])
            acc_v[rows, cs] = o
            if last:
                u_v[rows, cs] = o.astype(BF16)
                if out_copies(i)[t] is not None:
                    out_copies(i)[t].start()

        return [(nsub * w // 128, functools.partial(step, t)) for t in range(nsplit)]

    def fast_tiles(i, st, slot):
        r0 = i * BQ
        ntf = r0 // 128
        lacc = [None] * nsub
        acc = [None] * nsub
        left = [ntf + nsub]
        tiles = []

        def done(n):
            left[0] -= n
            if left[0] == 0:
                l = jnp.sum(jnp.concatenate(lacc, axis=0), axis=1, keepdims=True)
                st.ctx = (jnp.concatenate(acc, axis=0) / l).astype(BF16)

        def add_tile(t, c0, w):
            box = []

            def qk_exp():
                s = _dot_nt(q_v[slot, r0 + t * 128:r0 + BQ, :], k_v[slot, c0:c0 + w * 128, :])
                if c0 >= r0:
                    s0 = jnp.where(tri, s[:128], NEG)
                    s = jnp.concatenate([s0, s[128:]], axis=0) if t < nsub - 1 else s0
                p = jnp.exp2(s)
                for u in range(t, nsub):
                    lacc[u] = addn(lacc[u], functools.reduce(jnp.add, [
                        p[(u - t) * 128:(u - t + 1) * 128, j * 128:(j + 1) * 128]
                        for j in range(w)]))
                box.append(p.astype(BF16))

            def pv():
                o = _dot(box.pop(), v_v[slot, c0:c0 + w * 128, :])
                for u in range(t, nsub):
                    acc[u] = addn(acc[u], o[(u - t) * 128:(u - t + 1) * 128])
                done(w)

            tiles.append((w * (nsub - t), qk_exp, pv))

        kt = 0
        while kt < ntf:
            w = min(KW, ntf - kt)
            add_tile(0, kt * 128, w)
            kt += w
        for t in range(nsub):
            add_tile(t, r0 + t * 128, 1)
        return tiles

    def head_fast(h, slot, proj, last=False):
        sts = [St() for _ in range(nq)]
        order = list(range(nq))[::-1]
        tiles, ends = [], {}
        for i in order:
            tiles += fast_tiles(i, sts[i], slot)
            ends[len(tiles) - 1] = i
        proj = list(proj)
        outs = []
        t = [0.0]
        attn = 2 * sum(c for c, _, _ in tiles)
        fill = sum(c for c, _ in proj) + nq * nsub * (M // 128)
        debt = [0.0]

        def filler(force=False):
            while debt[0] > 0 or force:
                if outs and (outs[0][0] <= t[0] or not proj):
                    _, c, fn = outs.pop(0)
                elif proj:
                    c, fn = proj.pop(0)
                else:
                    return
                fn()
                t[0] += c
                debt[0] -= c

        n = len(tiles)
        for k in range(n + F_LAG):
            c = 0
            if k < n:
                tiles[k][1]()
                c += tiles[k][0]
            if k >= F_LAG:
                tiles[k - F_LAG][2]()
                c += tiles[k - F_LAG][0]
            t[0] += c
            if k - F_LAG in ends:
                i = ends[k - F_LAG]
                outs += [(t[0] + LAG_OUT, cc, fn) for cc, fn in out_steps(h, i, sts[i], last)]
            debt[0] += c * fill / attn * F_FILL
            filler()
        filler(force=True)

    def head_safe(h, slot, last=False):
        rr = lax.broadcasted_iota(jnp.int32, (256, 256), 0)
        cc = lax.broadcasted_iota(jnp.int32, (256, 256), 1)

        def q_block(qi, carry):
            rows = pl.ds(pl.multiple_of(qi * 256, 256), 256)
            q = q_v[slot, rows, :]

            def kv_block(kt, mla):
                m, l, acc = mla
                cols = pl.ds(pl.multiple_of(kt * 256, 256), 256)
                s = _dot_nt(q, k_v[slot, cols, :])
                s = jnp.where(cc + (kt - qi) * 256 <= rr, s, NEG)
                m_new = jnp.maximum(m, jnp.max(s, axis=1, keepdims=True))
                alpha = jnp.exp2(m - m_new)
                p = jnp.exp2(s - m_new)
                l = alpha * l + jnp.sum(p, axis=1, keepdims=True)
                acc = alpha * acc + _dot(p.astype(BF16), v_v[slot, cols, :])
                return m_new, l, acc

            init = (jnp.full((256, 1), NEG, F32), jnp.zeros((256, 1), F32),
                    jnp.zeros((256, D), F32))
            _, l, acc = lax.fori_loop(0, qi + 1, kv_block, init)
            ctx = (acc / l).astype(BF16)
            o = acc_v[rows, :] + _dot(ctx, wo_v[pl.ds(pl.multiple_of(h * D, D), D), :])
            acc_v[rows, :] = o
            if last:
                u_v[rows, :] = o.astype(BF16)
            return carry

        lax.fori_loop(0, S // 256, q_block, 0)

    def out_copies(i):
        rows, w = slice(i * BQ, (i + 1) * BQ), M // NSPLIT
        if i > 0:
            return [None] * (NSPLIT - 1) + [pltpu.make_async_copy(
                u_v.at[rows], out_h.at[rows, 0:M], osems.at[NSPLIT + i])]
        return [pltpu.make_async_copy(u_v.at[rows, t * w:(t + 1) * w],
                                      out_h.at[rows, t * w:(t + 1) * w], osems.at[t])
                for t in range(NSPLIT)]

    def all_out_copies():
        return [c for i in range(nq) for c in out_copies(i) if c is not None]

    def head(h, last=False):
        slot = h & 3
        small = bound_s[0] <= SCORE_LIMIT ** 2

        @pl.when(small)
        def _():
            head_fast(h, slot, [] if last else proj_steps(2 - (h & 2), h & 1), last)
            set_bound(h + 1)

        @pl.when(jnp.logical_not(small))
        def _():
            head_safe(h, slot, last)
            if not last:
                def rows(i, carry):
                    base, r0, nrm = 2 - (h & 2), (h & 1) * (S // 4) + i * 128, {}
                    proj("q", x_v, xs_v, ws_q, q_v, qscale, base, r0, nrm, 128)
                    proj("k", c_v, cs_v, ws_k, k_v, None, base, r0, nrm, 128)
                    proj(None, c_v, cs_v, ws_v, v_v, None, base, r0, nrm, 128)
                    publish(nrm, base, r0 == 0)
                    return carry

                lax.fori_loop(0, S // 4 // 128, rows, 0)
            set_bound(h + 1)
            if last:
                for c in all_out_copies():
                    c.start()

    for a in range(8):
        start(f"xb{a}", xb_h.at[:, a * 128:(a + 1) * 128], xb_v.at[a])
    start("l", l_h, l_v)
    start("gf", gf_h, gf_v)
    for t in range(16):
        start(f"wr{t}", wr_h.at[0:512, t * 128:(t + 1) * 128], wr_v.at[t])
        start(f"wi{t}", wi_h.at[0:512, t * 128:(t + 1) * 128], wi_v.at[t])
    start("wrn", wr_h.at[512:513, :], wrn_v)
    start("win", wi_h.at[512:513, :], win_v)
    start("c", c_h, c_v)
    start("x", x_h, x_v)
    for t in range(3):
        pair_copy(t, 0).start()
    start("wo", wo_h, wo_v)
    s_v[...] = jnp.zeros(s_v.shape, F32)
    for i in range(S // 512):
        start(f"z{i}", s_v, acc_v.at[i * 512:(i + 1) * 512], priority=1)
    wait(*[f"xb{a}" for a in range(8)])

    def fft8(jj, carry):
        for j0 in range(4):
            f1(jj, j0)
        return carry

    lax.fori_loop(0, 2, fft8, 0)
    wait("l", "gf")

    def fwd_quarter(i, carry):
        for t in range(3):
            for u in range(3):
                pair_copy(t, 4 * i + 1 + u).start()
        for q in range(4):
            f23(4 * i + q)
        return carry

    lax.fori_loop(0, 4, fwd_quarter, 0)
    for i in range(3):
        for t in range(3):
            pair_copy(t, 4 * i + 4).start()
    wait(*[f"wr{t}" for t in range(16)], *[f"wi{t}" for t in range(16)], "wrn", "win")
    def mid_quarter(g2, carry):
        mid_group(g2, range(8))
        return carry

    lax.fori_loop(0, 4, mid_quarter, 0)
    mid_nyquist()

    wait("c", "x")
    for t in range(3):
        pair_copy(t, 0).wait()
    split_inputs(x_v, xs_v)
    split_inputs(c_v, cs_v)
    unpack_weights(0)

    def inv_half(jj, carry):
        merge = proj_steps(0, jj)
        for j0 in range(4):
            i32(jj, j0)
            for _, fn in merge[len(merge) * j0 // 4:len(merge) * (j0 + 1) // 4]:
                fn()
        return carry

    lax.fori_loop(0, 2, inv_half, 0)
    for a in range(8):
        c = pltpu.make_async_copy(xb_v.at[a], out_h.at[:, M + a * 128:M + (a + 1) * 128],
                                  bsems.at[a])
        c.start()
        pending.append(c)

    wait("wo", *[f"z{i}" for i in range(S // 512)])
    set_bound(0)
    def body(h, carry):
        @pl.when((h & 1) == 0)
        def _():
            for t in range(3):
                pair_copy(t, (h >> 1) + 1).wait()
            unpack_weights((h >> 1) + 1)

        head(h)
        return carry

    lax.fori_loop(0, H - 2, body, 0)
    def tail(h, carry):
        @pl.when(h == H - 1)
        def _():
            for c in all_out_copies():
                c.wait()

        head(h, last=True)
        return carry

    lax.fori_loop(H - 2, H, tail, 0)
    for c in pending:
        c.wait()
    for c in all_out_copies():
        c.wait()


@jax.jit
def pallas_concat_heads__compressed_kv_cla__spectral_gfnet__prompt_kernel(
    A_x: jax.Array,
    A_c_kv: jax.Array,
    A_w_q: jax.Array,
    A_w_uk: jax.Array,
    A_w_uv: jax.Array,
    A_w_o: jax.Array,
    B_x: jax.Array,
    B_w_r: jax.Array,
    B_w_i: jax.Array,
):
    vm = pltpu.VMEM
    scratch = [
        vm((S, M), BF16), vm((S, C), BF16),
        vm((5, S // 2, M // 2), BF16), vm((5, S // 2, C // 2), BF16),
        vm((H // 2, M, D), U32), vm((H // 2, C, D), U32), vm((H // 2, C, D), U32),
        vm((H * D, M), BF16),
        vm((7, M // 2, D), BF16), vm((7, C // 2, D), BF16), vm((7, C // 2, D), BF16),
        vm((8, S, 128), BF16),
        vm((16, 512, 128), BF16), vm((16, 512, 128), BF16),
        vm((1, S), BF16), vm((1, S), BF16),
        vm(_L_NP.shape, BF16), vm(_GF_NP.shape, BF16),
        vm((S, 1024), BF16),
        vm((16, KR, 256), F32), vm((16, KR, 256), BF16),
        vm((S, M), F32),
        vm((4, S, D), BF16), vm((4, S, D), BF16), vm((4, S, D), BF16),
        vm((512, M), F32),
        vm((4, 2, 8, 128), F32), pltpu.SMEM((1,), F32),
        pltpu.SemaphoreType.DMA((64,)),
        pltpu.SemaphoreType.DMA((16,)),
        pltpu.SemaphoreType.DMA((3, H // 2)),
        pltpu.SemaphoreType.DMA((8,)),
    ]
    anyspec = pl.BlockSpec(memory_space=pl.ANY)
    out = pl.pallas_call(
        _kernel,
        out_shape=jax.ShapeDtypeStruct((S, M + DB), BF16),
        in_specs=[anyspec] * 11,
        out_specs=anyspec,
        scratch_shapes=scratch,
        compiler_params=pltpu.CompilerParams(vmem_limit_bytes=122 * 1024 * 1024),
        name="mla_gfnet_fused",
    )(
        A_x.reshape(S, M), A_c_kv.reshape(S, C), A_w_q, A_w_uk, A_w_uv,
        A_w_o.reshape(H * D, M),
        B_x.reshape(S, DB), B_w_r.T, B_w_i.T,
        jnp.asarray(_L_NP), jnp.asarray(_GF_NP),
    )
    return out.reshape(1, S, M + DB)
```

```python
import functools
import math

import numpy as np
import jax
import jax.numpy as jnp
from jax import lax
import jax.experimental.pallas as pl
import jax.experimental.pallas.tpu as pltpu

S = 2048
M = 1024
H = 32
D = 128
C = 512
DB = 1024
KR = 528

F32 = jnp.float32
BF16 = jnp.bfloat16
U32 = jnp.uint32
NT = (((1,), (1,)), ((), ()))
NEG = -1e30


def _np_bf16(a):
    return np.asarray(a, np.float32).astype(jnp.bfloat16)


def _make_consts():
    th = 2.0 * np.pi / DB
    b = np.arange(128)[None, :]
    k2 = np.arange(64)[:, None]
    lf = []
    for k1 in (1, 2, 3):
        g = np.exp(-1j * th * b * (k1 + 8 * k2))
        gp = np.exp(-1j * th * b * (8 - k1 + 8 * k2))
        lf.append(np.block([[g.real, -g.imag], [g.imag, g.real],
                            [gp.real, gp.imag], [gp.imag, -gp.real]]))
    g0 = np.exp(-1j * th * b * (8 * k2))
    g4 = np.exp(-1j * th * b * (4 + 8 * k2))
    l0 = np.concatenate([g0.real, g0.imag, np.cos(th * b * 512), np.zeros((127, 128))], 0)
    l4 = np.concatenate([g4.real, g4.imag, np.zeros((128, 128))], 0)
    lf.append(np.concatenate([l0, l4], 1))
    sc = 1.0 / (S * DB)
    bb = np.arange(128)[:, None]
    kk = np.arange(64)[None, :]
    li = []
    for k1 in (1, 2, 3):
        ph, pp = th * bb * (k1 + 8 * kk), th * bb * (8 - k1 + 8 * kk)
        c, s_, cp, sp = np.cos(ph), np.sin(ph), np.cos(pp), np.sin(pp)
        li.append(2 * sc * np.block([[c, -s_, cp, -sp], [s_, c, -sp, -cp]]))
    ph = th * bb * (8 * kk)
    c0, s0 = 2 * np.cos(ph), -2 * np.sin(ph)
    c0[:, 0] = 1.0
    s0[:, 0] = np.cos(th * bb[:, 0] * 512)
    i0 = sc * np.concatenate([c0, s0], 1)
    ph = th * bb * (4 + 8 * kk)
    i4 = sc * np.concatenate([2 * np.cos(ph), -2 * np.sin(ph)], 1)
    li.append(np.concatenate([np.concatenate([i0, i4], 1), np.zeros((128, 256))], 0))
    lmat = np.concatenate(lf + li, axis=0)
    p = np.arange(128)[None, :]
    kp = np.arange(128)[:, None]
    gf = []
    for q in range(16):
        g = np.exp(-2j * np.pi * (16 * p + q) * kp / S)
        gf.append(np.block([[g.real.T, g.imag.T], [-g.imag.T, g.real.T]]))
    return _np_bf16(lmat), _np_bf16(np.concatenate(gf, 0))


_L_NP, _GF_NP = _make_consts()


_dot = functools.partial(jnp.dot, preferred_element_type=F32)
_dot_nt = functools.partial(lax.dot_general, dimension_numbers=NT, preferred_element_type=F32)


def _t(x):
    return None if x is None else (1, x)


def _tneg(a):
    return None if a is None else (-a[0], a[1])


def _tadd(a, b):
    if a is None:
        return b
    if b is None:
        return a
    if a[0] == b[0]:
        return (a[0], a[1] + b[1])
    return (1, a[1] - b[1]) if a[0] > 0 else (1, b[1] - a[1])


def _tsub(a, b):
    return _tadd(a, _tneg(b))


def _tscale(a, c):
    return None if a is None else (1, a[1] * (c * a[0]))


def _tmul(a, v):
    return None if a is None else (a[0], a[1] * v)


def _tval(a):
    return a[1] if a[0] > 0 else -a[1]


def _twiddle(z, e, n, sign):
    re, im = z
    if e == 0:
        return re, im
    if 4 * e == n:
        return (_tneg(im), re) if sign > 0 else (im, _tneg(re))
    c = math.cos(2.0 * math.pi * e / n)
    s = sign * math.sin(2.0 * math.pi * e / n)
    if 8 * e % n == 0:
        r = abs(c)
        rc = re if c > 0 else _tneg(re)
        rs = re if s > 0 else _tneg(re)
        ic = im if c > 0 else _tneg(im)
        is_ = im if s > 0 else _tneg(im)
        return _tscale(_tsub(rc, is_), r), _tscale(_tadd(rs, ic), r)
    return (_tsub(_tscale(re, c), _tscale(im, s)), _tadd(_tscale(re, s), _tscale(im, c)))


def _fft(zs, sign):
    n = len(zs)
    if n == 1:
        return [zs[0]]
    ev = _fft(zs[0::2], sign)
    od = _fft(zs[1::2], sign)
    out = [None] * n
    for k in range(n // 2):
        t = _twiddle(od[k], k, n, sign)
        out[k] = (_tadd(ev[k][0], t[0]), _tadd(ev[k][1], t[1]))
        out[k + n // 2] = (_tsub(ev[k][0], t[0]), _tsub(ev[k][1], t[1]))
    return out


def _irfft8(t0, t4, t1, t2, t3):
    r = math.sqrt(0.5)
    a0, a1 = t0 + t4, t0 - t4
    e0, e2 = a0 + t2[0], a0 - t2[0]
    e1, e3 = a1 - t2[1], a1 + t2[1]
    o0 = t1[0] + t3[0]
    o2 = t3[1] - t1[1]
    u, v = t1[0] - t3[0], t1[1] + t3[1]
    o1, o3 = (u - v) * r, (-u - v) * r
    return [e0 + o0, e1 + o1, e2 + o2, e3 + o3, e0 - o0, e1 - o1, e2 - o2, e3 - o3]


def _lo_half(w):
    return pltpu.bitcast(w << 16, F32)


def _hi_half(w):
    return pltpu.bitcast(w & jnp.uint32(0xFFFF0000), F32)


def _pack_words(lo, hi):
    lo = pltpu.bitcast(lo.astype(BF16).astype(F32), U32)
    hi = pltpu.bitcast(hi.astype(BF16).astype(F32), U32)
    return (lo >> 16) | hi


def _interleave(gens):
    live = list(gens)
    while live:
        nxt = []
        for g in live:
            try:
                next(g)
                nxt.append(g)
            except StopIteration:
                pass
        live = nxt


def _drain(g):
    for _ in g:
        pass


BQ = 512
KW = 2
NSPLIT = 4
PM = 512
PM0 = 128
LAG_OUT = 16
F_LAG = 1
F_FILL = 1.0
SCORE_LIMIT = 60.0


def _kernel(x_h, c_h, wq_h, wk_h, wv_h, wo_h, xb_h, wr_h, wi_h, l_h, gf_h,
            out_h,
            x_v, c_v, xs_v, cs_v, wq_raw, wk_raw, wv_raw, wo_v, ws_q, ws_k, ws_v,
            xb_v, wr_v, wi_v, wrn_v, win_v, l_v, gf_v,
            u_v, y_v, z_v,
            acc_v, q_v, k_v, v_v, s_v, nrm_v, bound_s,
            sems, osems, wsems, bsems, gsems):
    cp = {}
    nsem = [0]

    def start(name, src, dst, priority=0):
        c = pltpu.make_async_copy(src, dst, sems.at[nsem[0]])
        nsem[0] += 1
        c.start(priority=priority)
        cp[name] = c

    def wait(*names):
        for nm in names:
            cp[nm].wait()

    wq32, wk32, wv32 = wq_h.bitcast(U32), wk_h.bitcast(U32), wv_h.bitcast(U32)

    def pair_copy(t, j):
        src, dst = ((wq32, wq_raw), (wk32, wk_raw), (wv32, wv_raw))[t]
        return pltpu.make_async_copy(src.at[:, j, :], dst.at[j], wsems.at[t, j])

    xb32 = xb_v.bitcast(U32)
    wr32 = wr_v.bitcast(U32)
    wi32 = wi_v.bitcast(U32)

    def word_rows(a, jj):
        return xb32.at[a, pl.ds(pl.multiple_of(4 * jj, 4), 1020)]

    def f1(jj, j0):
        views = [word_rows(a, jj) for a in range(8)]
        for g in range(8):
            words = [v[pl.ds(128 * g + j0, 16, stride=8), :] for v in views]
            for e in range(2):
                half = _lo_half if e == 0 else _hi_half
                o = _fft([(_t(half(w)), None) for w in words], -1)
                r0 = pl.multiple_of((8 * jj + 2 * j0 + e) * 128 + 16 * g, 16)
                parts = [o[0][0], o[4][0], o[1][0], o[1][1], o[2][0], o[2][1], o[3][0], o[3][1]]
                for t in range(8):
                    u_v[pl.ds(r0, 16), t * 128:(t + 1) * 128] = _tval(parts[t]).astype(BF16)

    def f23(q):
        rows = pl.ds(pl.multiple_of(q * 128, 128), 128)
        o = [_dot_nt(l_v[256 * i:256 * (i + 1), :], u_v[rows, 256 * (i + 1):256 * (i + 2)])
             .astype(BF16) for i in range(3)]
        o0 = _dot_nt(l_v[768:912, 0:128], u_v[rows, 0:128]).astype(BF16)
        o4 = _dot_nt(l_v[768:896, 128:256], u_v[rows, 128:256]).astype(BF16)

        def blk(k1, part):
            if k1 == 0:
                return o0[64 * part:64 * part + 64]
            if k1 == 4:
                return o4[64 * part:64 * part + 64]
            if k1 < 4:
                return o[k1 - 1][64 * part:64 * part + 64]
            return o[7 - k1][128 + 64 * part:128 + 64 * part + 64]

        re = jnp.concatenate([blk(k1, 0) for k1 in range(8)] + [o0[128:144]], axis=0)
        im = jnp.concatenate([blk(k1, 1) for k1 in range(8)] + [jnp.zeros((16, 128), BF16)],
                             axis=0)
        y_v[q] = _dot(jnp.concatenate([re, im], axis=1),
                      gf_v[pl.ds(pl.multiple_of(q * 256, 256), 256), :])

    def mid(rows, filt):
        xf = _fft([(_t(y_v[q, rows, 0:128]), _t(y_v[q, rows, 128:256])) for q in range(16)], -1)
        zs = []
        for kq in range(16):
            fr, fi = filt(kq)
            re, im = xf[kq]
            zs.append((_tsub(_tmul(re, fr), _tmul(im, fi)), _tadd(_tmul(re, fi), _tmul(im, fr))))
        us = _fft(zs, +1)
        for q in range(16):
            z_v[q, rows, 0:128] = _tval(us[q][0]).astype(BF16)
            z_v[q, rows, 128:256] = _tval(us[q][1]).astype(BF16)

    def mid_group(g2, k1s):
        base = pl.multiple_of(64 * g2, 64)
        for k1 in k1s:
            half = _lo_half if k1 % 2 == 0 else _hi_half
            sl = pl.ds(k1 // 2, 16, stride=4)

            def filt(kq):
                return (half(wr32.at[kq, pl.ds(base, 64)][sl, :]),
                        half(wi32.at[kq, pl.ds(base, 64)][sl, :]))

            mid(pl.ds(pl.multiple_of(64 * k1 + 16 * g2, 16), 16), filt)

    def mid_nyquist():
        def filt(kq):
            cs = slice(kq * 128, (kq + 1) * 128)
            return (jnp.broadcast_to(wrn_v[:, cs].astype(F32), (16, 128)),
                    jnp.broadcast_to(win_v[:, cs].astype(F32), (16, 128)))

        mid(slice(512, KR), filt)

    srow = lax.broadcasted_iota(jnp.int32, (64, 128), 0)

    def i32(jj, j0, between):
        ys, zs = [], []
        for e in range(2):
            q = 8 * jj + 2 * j0 + e
            zs.append(_dot_nt(z_v[q], gf_v[pl.ds(pl.multiple_of(q * 256, 256), 256), :]))
        between()
        for z in zs:
            zr, zi = z[:, 0:128], z[:, 128:256]
            zi0 = jnp.where(srow == 0, jnp.broadcast_to(zr[512:513], (64, 128)), zi[0:64])
            rhs0 = jnp.concatenate([zr[0:64], zi0], axis=0).astype(BF16)
            t0 = _dot(l_v[1792:1920, 0:128], rhs0)
            rhs4 = jnp.concatenate([zr[256:320], zi[256:320]], axis=0).astype(BF16)
            t4 = _dot(l_v[1792:1920, 128:256], rhs4)
            ts = []
            for k1 in (1, 2, 3):
                kc = 8 - k1
                rhs = jnp.concatenate([zr[64 * k1:64 * k1 + 64], zi[64 * k1:64 * k1 + 64],
                                       zr[64 * kc:64 * kc + 64], zi[64 * kc:64 * kc + 64]],
                                      axis=0).astype(BF16)
                o = _dot(l_v[1024 + 256 * (k1 - 1):1024 + 256 * k1, :], rhs)
                ts.append((o[0:128], o[128:256]))
            ys.append(_irfft8(t0, t4, *ts))
        for a in range(8):
            word_rows(a, jj)[pl.ds(j0, 128, stride=8), :] = _pack_words(ys[0][a], ys[1][a]).T

    nq = S // BQ
    nsub = BQ // 128
    row = lax.broadcasted_iota(jnp.int32, (128, 128), 0)
    col = lax.broadcasted_iota(jnp.int32, (128, 128), 1)
    tri = col <= row
    qscale = (D ** -0.5) * math.log2(math.e)

    def mx(a, b):
        return b if a is None else jnp.maximum(a, b)

    def addn(a, b):
        return b if a is None else a + b

    class St:
        pass

    def split_inputs(src, dst):
        n = src.shape[1] // 2

        def chunk(i, carry):
            top = pl.ds(pl.multiple_of(i * 128, 128), 128)
            bot = pl.ds(pl.multiple_of(S // 2 + i * 128, 128), 128)
            a11, a12 = src[top, 0:n].astype(F32), src[top, n:].astype(F32)
            a21, a22 = src[bot, 0:n].astype(F32), src[bot, n:].astype(F32)
            for t, v in enumerate((a11 + a22, a21 + a22, a11 + a12, a21 - a11, a12 - a22)):
                dst[t, top, :] = v.astype(BF16)
            return carry

        lax.fori_loop(0, S // 256, chunk, 0)

    def unpack_weights(j):
        def unpack(raw, w, r0):
            n = w.shape[1]
            rows = pl.ds(pl.multiple_of(r0, 64), 64)
            up, dn = raw[j, rows, :], raw[j, pl.ds(pl.multiple_of(n + r0, 64), 64), :]
            b11, b12, b21, b22 = _lo_half(up), _hi_half(up), _lo_half(dn), _hi_half(dn)
            for t, v in enumerate((b11 + b22, b11, b12 - b22, b21 - b11, b22,
                                   b11 + b12, b21 + b22)):
                w[t, rows, :] = v.astype(BF16)

        def chunk(i, carry):
            unpack(wq_raw, ws_q, i * 128)
            unpack(wq_raw, ws_q, i * 128 + 64)
            unpack(wk_raw, ws_k, i * 64)
            unpack(wv_raw, ws_v, i * 64)
            return carry

        lax.fori_loop(0, 4, chunk, 0)

    def track(nrm, name, a):
        n2 = jnp.max(jnp.sum(a * a, axis=1, keepdims=True), axis=0, keepdims=True)
        nrm[name] = mx(nrm.get(name), n2)

    def publish(nrm, base, first):
        for t in range(2):
            for w, name in enumerate(("q", "k")):
                old = jnp.where(first, 0.0, nrm_v[base + t, w])
                nrm_v[base + t, w] = jnp.maximum(old, jnp.broadcast_to(nrm[name, t], (8, 128)))

    def set_bound(h):
        bound_s[0] = jnp.max(nrm_v[h & 3, 0] * nrm_v[h & 3, 1])

    def proj(name, src, sums, w, dst, scale, base, r0, nrm, pm=PM):
        n = w.shape[1]
        top = pl.ds(pl.multiple_of(r0, pm), pm)
        bot = pl.ds(pl.multiple_of(S // 2 + r0, pm), pm)
        m1 = _dot(sums[0, top, :], w[0])
        m2 = _dot(sums[1, top, :], w[1])
        m3 = _dot(src[top, 0:n], w[2])
        m4 = _dot(src[bot, n:], w[3])
        m5 = _dot(sums[2, top, :], w[4])
        m6 = _dot(sums[3, top, :], w[5])
        m7 = _dot(sums[4, top, :], w[6])
        outs = ((0, top, (m1 + m4) + (m7 - m5)), (1, top, m3 + m5),
                (0, bot, m2 + m4), (1, bot, (m1 - m2) + (m3 + m6)))
        for t, rows, val in outs:
            if scale is not None:
                val = val * scale
            if name is not None:
                track(nrm, (name, t), val)
            dst[base + t, rows, :] = val.astype(BF16)

    def proj_steps(base, e, pm=PM):
        steps, nrm = [], {}
        for i in range(S // 4 // pm):
            r0 = e * (S // 4) + i * pm
            for cost, args in ((4, ("q", x_v, xs_v, ws_q, q_v, qscale)),
                               (2, ("k", c_v, cs_v, ws_k, k_v, None)),
                               (2, (None, c_v, cs_v, ws_v, v_v, None))):
                steps.append((7 * cost * pm // 128,
                              functools.partial(proj, *args, base, r0, nrm, pm)))
        steps.append((0, functools.partial(publish, nrm, base, e == 0)))
        return steps

    pending = []

    def out_steps(h, i, st, last, nsplit=NSPLIT):
        rows = slice(i * BQ, (i + 1) * BQ)
        w = M // nsplit

        def step(t):
            cs = slice(t * w, (t + 1) * w)
            o = acc_v[rows, cs] + _dot(st.ctx, wo_v[pl.ds(pl.multiple_of(h * D, D), D), cs])
            acc_v[rows, cs] = o
            if last:
                u_v[rows, cs] = o.astype(BF16)
                if out_copies(i)[t] is not None:
                    out_copies(i)[t].start()

        return [(nsub * w // 128, functools.partial(step, t)) for t in range(nsplit)]

    def fast_tiles(i, st, slot):
        r0 = i * BQ
        ntf = r0 // 128
        lacc = [None] * nsub
        acc = [None] * nsub
        left = [ntf + nsub]
        tiles = []

        def done(n):
            left[0] -= n
            if left[0] == 0:
                l = jnp.sum(jnp.concatenate(lacc, axis=0), axis=1, keepdims=True)
                st.ctx = (jnp.concatenate(acc, axis=0) / l).astype(BF16)

        def add_tile(t, c0, w):
            box = []

            def qk_exp():
                s = _dot_nt(q_v[slot, r0 + t * 128:r0 + BQ, :], k_v[slot, c0:c0 + w * 128, :])
                if c0 >= r0:
                    s0 = jnp.where(tri, s[:128], NEG)
                    s = jnp.concatenate([s0, s[128:]], axis=0) if t < nsub - 1 else s0
                p = jnp.exp2(s)
                for u in range(t, nsub):
                    lacc[u] = addn(lacc[u], functools.reduce(jnp.add, [
                        p[(u - t) * 128:(u - t + 1) * 128, j * 128:(j + 1) * 128]
                        for j in range(w)]))
                box.append(p.astype(BF16))

            def pv():
                o = _dot(box.pop(), v_v[slot, c0:c0 + w * 128, :])
                for u in range(t, nsub):
                    acc[u] = addn(acc[u], o[(u - t) * 128:(u - t + 1) * 128])
                done(w)

            tiles.append((w * (nsub - t), qk_exp, pv))

        kt = 0
        while kt < ntf:
            w = min(KW, ntf - kt)
            add_tile(0, kt * 128, w)
            kt += w
        for t in range(nsub):
            add_tile(t, r0 + t * 128, 1)
        return tiles

    def head_fast(h, slot, proj, last=False):
        sts = [St() for _ in range(nq)]
        order = list(range(nq))[::-1]
        tiles, ends = [], {}
        for i in order:
            tiles += fast_tiles(i, sts[i], slot)
            ends[len(tiles) - 1] = i
        proj = list(proj)
        outs = []
        t = [0.0]
        attn = 2 * sum(c for c, _, _ in tiles)
        fill = sum(c for c, _ in proj) + nq * nsub * (M // 128)
        debt = [0.0]

        def filler(force=False):
            while debt[0] > 0 or force:
                if outs and (outs[0][0] <= t[0] or not proj):
                    _, c, fn = outs.pop(0)
                elif proj:
                    c, fn = proj.pop(0)
                else:
                    return
                fn()
                t[0] += c
                debt[0] -= c

        n = len(tiles)
        for k in range(n + F_LAG):
            c = 0
            if k < n:
                tiles[k][1]()
                c += tiles[k][0]
            if k >= F_LAG:
                tiles[k - F_LAG][2]()
                c += tiles[k - F_LAG][0]
            t[0] += c
            if k - F_LAG in ends:
                i = ends[k - F_LAG]
                outs += [(t[0] + LAG_OUT, cc, fn) for cc, fn in out_steps(h, i, sts[i], last)]
            debt[0] += c * fill / attn * F_FILL
            filler()
        filler(force=True)

    def head_safe(h, slot, last=False):
        rr = lax.broadcasted_iota(jnp.int32, (256, 256), 0)
        cc = lax.broadcasted_iota(jnp.int32, (256, 256), 1)

        def q_block(qi, carry):
            rows = pl.ds(pl.multiple_of(qi * 256, 256), 256)
            q = q_v[slot, rows, :]

            def kv_block(kt, mla):
                m, l, acc = mla
                cols = pl.ds(pl.multiple_of(kt * 256, 256), 256)
                s = _dot_nt(q, k_v[slot, cols, :])
                s = jnp.where(cc + (kt - qi) * 256 <= rr, s, NEG)
                m_new = jnp.maximum(m, jnp.max(s, axis=1, keepdims=True))
                alpha = jnp.exp2(m - m_new)
                p = jnp.exp2(s - m_new)
                l = alpha * l + jnp.sum(p, axis=1, keepdims=True)
                acc = alpha * acc + _dot(p.astype(BF16), v_v[slot, cols, :])
                return m_new, l, acc

            init = (jnp.full((256, 1), NEG, F32), jnp.zeros((256, 1), F32),
                    jnp.zeros((256, D), F32))
            _, l, acc = lax.fori_loop(0, qi + 1, kv_block, init)
            ctx = (acc / l).astype(BF16)
            o = acc_v[rows, :] + _dot(ctx, wo_v[pl.ds(pl.multiple_of(h * D, D), D), :])
            acc_v[rows, :] = o
            if last:
                u_v[rows, :] = o.astype(BF16)
            return carry

        lax.fori_loop(0, S // 256, q_block, 0)

    def out_copies(i):
        rows, w = slice(i * BQ, (i + 1) * BQ), M // NSPLIT
        if i > 0:
            return [None] * (NSPLIT - 1) + [pltpu.make_async_copy(
                u_v.at[rows], out_h.at[rows, 0:M], osems.at[NSPLIT + i])]
        return [pltpu.make_async_copy(u_v.at[rows, t * w:(t + 1) * w],
                                      out_h.at[rows, t * w:(t + 1) * w], osems.at[t])
                for t in range(NSPLIT)]

    def all_out_copies():
        return [c for i in range(nq) for c in out_copies(i) if c is not None]

    def head(h, last=False):
        slot = h & 3
        small = bound_s[0] <= SCORE_LIMIT ** 2

        @pl.when(small)
        def _():
            head_fast(h, slot, [] if last else proj_steps(2 - (h & 2), h & 1), last)
            set_bound(h + 1)

        @pl.when(jnp.logical_not(small))
        def _():
            head_safe(h, slot, last)
            if not last:
                def rows(i, carry):
                    base, r0, nrm = 2 - (h & 2), (h & 1) * (S // 4) + i * 128, {}
                    proj("q", x_v, xs_v, ws_q, q_v, qscale, base, r0, nrm, 128)
                    proj("k", c_v, cs_v, ws_k, k_v, None, base, r0, nrm, 128)
                    proj(None, c_v, cs_v, ws_v, v_v, None, base, r0, nrm, 128)
                    publish(nrm, base, r0 == 0)
                    return carry

                lax.fori_loop(0, S // 4 // 128, rows, 0)
            set_bound(h + 1)
            if last:
                for c in all_out_copies():
                    c.start()

    for a in range(8):
        start(f"xb{a}", xb_h.at[:, a * 128:(a + 1) * 128], xb_v.at[a])
    start("l", l_h, l_v)

    def gf_copy(i):
        rows = pl.ds(pl.multiple_of(i * 1024, 1024), 1024)
        return pltpu.make_async_copy(gf_h.at[rows], gf_v.at[rows], gsems.at[i])

    for i in range(4):
        gf_copy(i).start()
    for t in range(16):
        start(f"wr{t}", wr_h.at[0:512, t * 128:(t + 1) * 128], wr_v.at[t])
        start(f"wi{t}", wi_h.at[0:512, t * 128:(t + 1) * 128], wi_v.at[t])
    start("wrn", wr_h.at[512:513, :], wrn_v)
    start("win", wi_h.at[512:513, :], win_v)
    start("c", c_h, c_v)
    start("x", x_h, x_v)
    for t in range(3):
        pair_copy(t, 0).start()
    start("wo", wo_h, wo_v)
    s_v[...] = jnp.zeros(s_v.shape, F32)
    for i in range(S // 512):
        start(f"z{i}", s_v, acc_v.at[i * 512:(i + 1) * 512], priority=1)
    wait(*[f"xb{a}" for a in range(8)])

    def fft8(jj, carry):
        for j0 in range(4):
            f1(jj, j0)
        return carry

    lax.fori_loop(0, 2, fft8, 0)
    wait("l")

    def fwd_quarter(i, carry):
        gf_copy(i).wait()
        for t in range(3):
            for u in range(3):
                pair_copy(t, 4 * i + 1 + u).start()
        for q in range(4):
            f23(4 * i + q)
        return carry

    lax.fori_loop(0, 4, fwd_quarter, 0)
    for i in range(3):
        for t in range(3):
            pair_copy(t, 4 * i + 4).start()
    wait(*[f"wr{t}" for t in range(16)], *[f"wi{t}" for t in range(16)], "wrn", "win")
    def mid_quarter(g2, carry):
        mid_group(g2, range(8))
        return carry

    lax.fori_loop(0, 4, mid_quarter, 0)
    mid_nyquist()

    wait("c", "x")
    for t in range(3):
        pair_copy(t, 0).wait()
    split_inputs(x_v, xs_v)
    split_inputs(c_v, cs_v)
    unpack_weights(0)

    def inv_half(jj, carry):
        merge = proj_steps(0, jj, PM0)
        for j0 in range(4):
            part = merge[len(merge) * j0 // 4:len(merge) * (j0 + 1) // 4]
            i32(jj, j0, lambda: [fn() for _, fn in part])
        return carry

    lax.fori_loop(0, 2, inv_half, 0)
    for a in range(8):
        c = pltpu.make_async_copy(xb_v.at[a], out_h.at[:, M + a * 128:M + (a + 1) * 128],
                                  bsems.at[a])
        c.start()
        pending.append(c)

    wait("wo", *[f"z{i}" for i in range(S // 512)])
    set_bound(0)
    def body(h, carry):
        @pl.when((h & 1) == 0)
        def _():
            for t in range(3):
                pair_copy(t, (h >> 1) + 1).wait()
            unpack_weights((h >> 1) + 1)

        head(h)
        return carry

    lax.fori_loop(0, H - 2, body, 0)
    def tail(h, carry):
        @pl.when(h == H - 1)
        def _():
            for c in all_out_copies():
                c.wait()

        head(h, last=True)
        return carry

    lax.fori_loop(H - 2, H, tail, 0)
    for c in pending:
        c.wait()
    for c in all_out_copies():
        c.wait()


@jax.jit
def pallas_concat_heads__compressed_kv_cla__spectral_gfnet__prompt_kernel(
    A_x: jax.Array,
    A_c_kv: jax.Array,
    A_w_q: jax.Array,
    A_w_uk: jax.Array,
    A_w_uv: jax.Array,
    A_w_o: jax.Array,
    B_x: jax.Array,
    B_w_r: jax.Array,
    B_w_i: jax.Array,
):
    vm = pltpu.VMEM
    scratch = [
        vm((S, M), BF16), vm((S, C), BF16),
        vm((5, S // 2, M // 2), BF16), vm((5, S // 2, C // 2), BF16),
        vm((H // 2, M, D), U32), vm((H // 2, C, D), U32), vm((H // 2, C, D), U32),
        vm((H * D, M), BF16),
        vm((7, M // 2, D), BF16), vm((7, C // 2, D), BF16), vm((7, C // 2, D), BF16),
        vm((8, S, 128), BF16),
        vm((16, 512, 128), BF16), vm((16, 512, 128), BF16),
        vm((1, S), BF16), vm((1, S), BF16),
        vm(_L_NP.shape, BF16), vm(_GF_NP.shape, BF16),
        vm((S, 1024), BF16),
        vm((16, KR, 256), F32), vm((16, KR, 256), BF16),
        vm((S, M), F32),
        vm((4, S, D), BF16), vm((4, S, D), BF16), vm((4, S, D), BF16),
        vm((512, M), F32),
        vm((4, 2, 8, 128), F32), pltpu.SMEM((1,), F32),
        pltpu.SemaphoreType.DMA((64,)),
        pltpu.SemaphoreType.DMA((16,)),
        pltpu.SemaphoreType.DMA((3, H // 2)),
        pltpu.SemaphoreType.DMA((8,)),
        pltpu.SemaphoreType.DMA((4,)),
    ]
    anyspec = pl.BlockSpec(memory_space=pl.ANY)
    out = pl.pallas_call(
        _kernel,
        out_shape=jax.ShapeDtypeStruct((S, M + DB), BF16),
        in_specs=[anyspec] * 11,
        out_specs=anyspec,
        scratch_shapes=scratch,
        compiler_params=pltpu.CompilerParams(vmem_limit_bytes=122 * 1024 * 1024),
        name="mla_gfnet_fused",
    )(
        A_x.reshape(S, M), A_c_kv.reshape(S, C), A_w_q, A_w_uk, A_w_uv,
        A_w_o.reshape(H * D, M),
        B_x.reshape(S, DB), B_w_r.T, B_w_i.T,
        jnp.asarray(_L_NP), jnp.asarray(_GF_NP),
    )
    return out.reshape(1, S, M + DB)
```

```python
import functools
import math

import numpy as np
import jax
import jax.numpy as jnp
from jax import lax
import jax.experimental.pallas as pl
import jax.experimental.pallas.tpu as pltpu

S = 2048
M = 1024
H = 32
D = 128
C = 512
DB = 1024
KR = 528

F32 = jnp.float32
BF16 = jnp.bfloat16
U32 = jnp.uint32
NT = (((1,), (1,)), ((), ()))
NEG = -1e30


def _np_bf16(a):
    return np.asarray(a, np.float32).astype(jnp.bfloat16)


def _make_consts():
    th = 2.0 * np.pi / DB
    b = np.arange(128)[None, :]
    k2 = np.arange(64)[:, None]
    lf = []
    for k1 in (1, 2, 3):
        g = np.exp(-1j * th * b * (k1 + 8 * k2))
        gp = np.exp(-1j * th * b * (8 - k1 + 8 * k2))
        lf.append(np.block([[g.real, -g.imag], [g.imag, g.real],
                            [gp.real, gp.imag], [gp.imag, -gp.real]]))
    g0 = np.exp(-1j * th * b * (8 * k2))
    g4 = np.exp(-1j * th * b * (4 + 8 * k2))
    l0 = np.concatenate([g0.real, g0.imag, np.cos(th * b * 512), np.zeros((127, 128))], 0)
    l4 = np.concatenate([g4.real, g4.imag, np.zeros((128, 128))], 0)
    lf.append(np.concatenate([l0, l4], 1))
    sc = 1.0 / (S * DB)
    bb = np.arange(128)[:, None]
    kk = np.arange(64)[None, :]
    li = []
    for k1 in (1, 2, 3):
        ph, pp = th * bb * (k1 + 8 * kk), th * bb * (8 - k1 + 8 * kk)
        c, s_, cp, sp = np.cos(ph), np.sin(ph), np.cos(pp), np.sin(pp)
        li.append(2 * sc * np.block([[c, -s_, cp, -sp], [s_, c, -sp, -cp]]))
    ph = th * bb * (8 * kk)
    c0, s0 = 2 * np.cos(ph), -2 * np.sin(ph)
    c0[:, 0] = 1.0
    s0[:, 0] = np.cos(th * bb[:, 0] * 512)
    i0 = sc * np.concatenate([c0, s0], 1)
    ph = th * bb * (4 + 8 * kk)
    i4 = sc * np.concatenate([2 * np.cos(ph), -2 * np.sin(ph)], 1)
    li.append(np.concatenate([np.concatenate([i0, i4], 1), np.zeros((128, 256))], 0))
    lmat = np.concatenate(lf + li, axis=0)
    p = np.arange(128)[None, :]
    kp = np.arange(128)[:, None]
    gf = []
    for q in range(16):
        g = np.exp(-2j * np.pi * (16 * p + q) * kp / S)
        gf.append(np.block([[g.real.T, g.imag.T], [-g.imag.T, g.real.T]]))
    return _np_bf16(lmat), _np_bf16(np.concatenate(gf, 0))


_L_NP, _GF_NP = _make_consts()


_dot = functools.partial(jnp.dot, preferred_element_type=F32)
_dot_nt = functools.partial(lax.dot_general, dimension_numbers=NT, preferred_element_type=F32)


def _t(x):
    return None if x is None else (1, x)


def _tneg(a):
    return None if a is None else (-a[0], a[1])


def _tadd(a, b):
    if a is None:
        return b
    if b is None:
        return a
    if a[0] == b[0]:
        return (a[0], a[1] + b[1])
    return (1, a[1] - b[1]) if a[0] > 0 else (1, b[1] - a[1])


def _tsub(a, b):
    return _tadd(a, _tneg(b))


def _tscale(a, c):
    return None if a is None else (1, a[1] * (c * a[0]))


def _tmul(a, v):
    return None if a is None else (a[0], a[1] * v)


def _tval(a):
    return a[1] if a[0] > 0 else -a[1]


def _twiddle(z, e, n, sign):
    re, im = z
    if e == 0:
        return re, im
    if 4 * e == n:
        return (_tneg(im), re) if sign > 0 else (im, _tneg(re))
    c = math.cos(2.0 * math.pi * e / n)
    s = sign * math.sin(2.0 * math.pi * e / n)
    if 8 * e % n == 0:
        r = abs(c)
        rc = re if c > 0 else _tneg(re)
        rs = re if s > 0 else _tneg(re)
        ic = im if c > 0 else _tneg(im)
        is_ = im if s > 0 else _tneg(im)
        return _tscale(_tsub(rc, is_), r), _tscale(_tadd(rs, ic), r)
    return (_tsub(_tscale(re, c), _tscale(im, s)), _tadd(_tscale(re, s), _tscale(im, c)))


def _fft(zs, sign):
    n = len(zs)
    if n == 1:
        return [zs[0]]
    ev = _fft(zs[0::2], sign)
    od = _fft(zs[1::2], sign)
    out = [None] * n
    for k in range(n // 2):
        t = _twiddle(od[k], k, n, sign)
        out[k] = (_tadd(ev[k][0], t[0]), _tadd(ev[k][1], t[1]))
        out[k + n // 2] = (_tsub(ev[k][0], t[0]), _tsub(ev[k][1], t[1]))
    return out


def _irfft8(t0, t4, t1, t2, t3):
    r = math.sqrt(0.5)
    a0, a1 = t0 + t4, t0 - t4
    e0, e2 = a0 + t2[0], a0 - t2[0]
    e1, e3 = a1 - t2[1], a1 + t2[1]
    o0 = t1[0] + t3[0]
    o2 = t3[1] - t1[1]
    u, v = t1[0] - t3[0], t1[1] + t3[1]
    o1, o3 = (u - v) * r, (-u - v) * r
    return [e0 + o0, e1 + o1, e2 + o2, e3 + o3, e0 - o0, e1 - o1, e2 - o2, e3 - o3]


def _lo_half(w):
    return pltpu.bitcast(w << 16, F32)


def _hi_half(w):
    return pltpu.bitcast(w & jnp.uint32(0xFFFF0000), F32)


def _pack_words(lo, hi):
    lo = pltpu.bitcast(lo.astype(BF16).astype(F32), U32)
    hi = pltpu.bitcast(hi.astype(BF16).astype(F32), U32)
    return (lo >> 16) | hi


def _interleave(gens):
    live = list(gens)
    while live:
        nxt = []
        for g in live:
            try:
                next(g)
                nxt.append(g)
            except StopIteration:
                pass
        live = nxt


def _drain(g):
    for _ in g:
        pass


BQ = 512
KW = 2
NSPLIT = 4
PM = 512
PM0 = 128
LAG_OUT = 16
F_LAG = 1
F_FILL = 1.0
SCORE_LIMIT = 60.0


def _kernel(x_h, c_h, wq_h, wk_h, wv_h, wo_h, xb_h, wr_h, wi_h, l_h, gf_h,
            out_h,
            x_v, c_v, xs_v, cs_v, wq_raw, wk_raw, wv_raw, wo_v, ws_q, ws_k, ws_v,
            xb_v, wr_v, wi_v, wrn_v, win_v, l_v, gf_v,
            u_v, y_v, z_v,
            acc_v, q_v, k_v, v_v, s_v, nrm_v, bound_s,
            sems, osems, wsems, bsems):
    cp = {}
    nsem = [0]

    def start(name, src, dst, priority=0):
        c = pltpu.make_async_copy(src, dst, sems.at[nsem[0]])
        nsem[0] += 1
        c.start(priority=priority)
        cp[name] = c

    def wait(*names):
        for nm in names:
            cp[nm].wait()

    wq32, wk32, wv32 = wq_h.bitcast(U32), wk_h.bitcast(U32), wv_h.bitcast(U32)

    def pair_copy(t, j):
        src, dst = ((wq32, wq_raw), (wk32, wk_raw), (wv32, wv_raw))[t]
        return pltpu.make_async_copy(src.at[:, j, :], dst.at[j], wsems.at[t, j])

    xb32 = xb_v.bitcast(U32)
    wr32 = wr_v.bitcast(U32)
    wi32 = wi_v.bitcast(U32)

    def word_rows(a, jj):
        return xb32.at[a, pl.ds(pl.multiple_of(4 * jj, 4), 1020)]

    def f1(jj, j0):
        views = [word_rows(a, jj) for a in range(8)]
        for g in range(8):
            words = [v[pl.ds(128 * g + j0, 16, stride=8), :] for v in views]
            for e in range(2):
                half = _lo_half if e == 0 else _hi_half
                o = _fft([(_t(half(w)), None) for w in words], -1)
                r0 = pl.multiple_of((8 * jj + 2 * j0 + e) * 128 + 16 * g, 16)
                parts = [o[0][0], o[4][0], o[1][0], o[1][1], o[2][0], o[2][1], o[3][0], o[3][1]]
                for t in range(8):
                    u_v[pl.ds(r0, 16), t * 128:(t + 1) * 128] = _tval(parts[t]).astype(BF16)

    def f23(q):
        rows = pl.ds(pl.multiple_of(q * 128, 128), 128)
        o = [_dot_nt(l_v[256 * i:256 * (i + 1), :], u_v[rows, 256 * (i + 1):256 * (i + 2)])
             .astype(BF16) for i in range(3)]
        o0 = _dot_nt(l_v[768:912, 0:128], u_v[rows, 0:128]).astype(BF16)
        o4 = _dot_nt(l_v[768:896, 128:256], u_v[rows, 128:256]).astype(BF16)

        def blk(k1, part):
            if k1 == 0:
                return o0[64 * part:64 * part + 64]
            if k1 == 4:
                return o4[64 * part:64 * part + 64]
            if k1 < 4:
                return o[k1 - 1][64 * part:64 * part + 64]
            return o[7 - k1][128 + 64 * part:128 + 64 * part + 64]

        re = jnp.concatenate([blk(k1, 0) for k1 in range(8)] + [o0[128:144]], axis=0)
        im = jnp.concatenate([blk(k1, 1) for k1 in range(8)] + [jnp.zeros((16, 128), BF16)],
                             axis=0)
        y_v[q] = _dot(jnp.concatenate([re, im], axis=1),
                      gf_v[pl.ds(pl.multiple_of(q * 256, 256), 256), :])

    def mid(rows, filt):
        xf = _fft([(_t(y_v[q, rows, 0:128]), _t(y_v[q, rows, 128:256])) for q in range(16)], -1)
        zs = []
        for kq in range(16):
            fr, fi = filt(kq)
            re, im = xf[kq]
            zs.append((_tsub(_tmul(re, fr), _tmul(im, fi)), _tadd(_tmul(re, fi), _tmul(im, fr))))
        us = _fft(zs, +1)
        for q in range(16):
            z_v[q, rows, 0:128] = _tval(us[q][0]).astype(BF16)
            z_v[q, rows, 128:256] = _tval(us[q][1]).astype(BF16)

    def mid_group(g2, k1s):
        base = pl.multiple_of(64 * g2, 64)
        for k1 in k1s:
            half = _lo_half if k1 % 2 == 0 else _hi_half
            sl = pl.ds(k1 // 2, 16, stride=4)

            def filt(kq):
                return (half(wr32.at[kq, pl.ds(base, 64)][sl, :]),
                        half(wi32.at[kq, pl.ds(base, 64)][sl, :]))

            mid(pl.ds(pl.multiple_of(64 * k1 + 16 * g2, 16), 16), filt)

    def mid_nyquist():
        def filt(kq):
            cs = slice(kq * 128, (kq + 1) * 128)
            return (jnp.broadcast_to(wrn_v[:, cs].astype(F32), (16, 128)),
                    jnp.broadcast_to(win_v[:, cs].astype(F32), (16, 128)))

        mid(slice(512, KR), filt)

    srow = lax.broadcasted_iota(jnp.int32, (64, 128), 0)

    def i32(jj, j0, between):
        ys, zs = [], []
        for e in range(2):
            q = 8 * jj + 2 * j0 + e
            zs.append(_dot_nt(z_v[q], gf_v[pl.ds(pl.multiple_of(q * 256, 256), 256), :]))
        between()
        for z in zs:
            zr, zi = z[:, 0:128], z[:, 128:256]
            zi0 = jnp.where(srow == 0, jnp.broadcast_to(zr[512:513], (64, 128)), zi[0:64])
            rhs0 = jnp.concatenate([zr[0:64], zi0], axis=0).astype(BF16)
            t0 = _dot(l_v[1792:1920, 0:128], rhs0)
            rhs4 = jnp.concatenate([zr[256:320], zi[256:320]], axis=0).astype(BF16)
            t4 = _dot(l_v[1792:1920, 128:256], rhs4)
            ts = []
            for k1 in (1, 2, 3):
                kc = 8 - k1
                rhs = jnp.concatenate([zr[64 * k1:64 * k1 + 64], zi[64 * k1:64 * k1 + 64],
                                       zr[64 * kc:64 * kc + 64], zi[64 * kc:64 * kc + 64]],
                                      axis=0).astype(BF16)
                o = _dot(l_v[1024 + 256 * (k1 - 1):1024 + 256 * k1, :], rhs)
                ts.append((o[0:128], o[128:256]))
            ys.append(_irfft8(t0, t4, *ts))
        for a in range(8):
            word_rows(a, jj)[pl.ds(j0, 128, stride=8), :] = _pack_words(ys[0][a], ys[1][a]).T

    nq = S // BQ
    nsub = BQ // 128
    row = lax.broadcasted_iota(jnp.int32, (128, 128), 0)
    col = lax.broadcasted_iota(jnp.int32, (128, 128), 1)
    tri = col <= row
    qscale = (D ** -0.5) * math.log2(math.e)

    def mx(a, b):
        return b if a is None else jnp.maximum(a, b)

    def addn(a, b):
        return b if a is None else a + b

    class St:
        pass

    def split_inputs(src, dst):
        n = src.shape[1] // 2

        def chunk(i, carry):
            top = pl.ds(pl.multiple_of(i * 128, 128), 128)
            bot = pl.ds(pl.multiple_of(S // 2 + i * 128, 128), 128)
            a11, a12 = src[top, 0:n].astype(F32), src[top, n:].astype(F32)
            a21, a22 = src[bot, 0:n].astype(F32), src[bot, n:].astype(F32)
            for t, v in enumerate((a11 + a22, a21 + a22, a11 + a12, a21 - a11, a12 - a22)):
                dst[t, top, :] = v.astype(BF16)
            return carry

        lax.fori_loop(0, S // 256, chunk, 0)

    def unpack_weights(j):
        def unpack(raw, w, r0):
            n = w.shape[1]
            rows = pl.ds(pl.multiple_of(r0, 64), 64)
            up, dn = raw[j, rows, :], raw[j, pl.ds(pl.multiple_of(n + r0, 64), 64), :]
            b11, b12, b21, b22 = _lo_half(up), _hi_half(up), _lo_half(dn), _hi_half(dn)
            for t, v in enumerate((b11 + b22, b11, b12 - b22, b21 - b11, b22,
                                   b11 + b12, b21 + b22)):
                w[t, rows, :] = v.astype(BF16)

        def chunk(i, carry):
            unpack(wq_raw, ws_q, i * 128)
            unpack(wq_raw, ws_q, i * 128 + 64)
            unpack(wk_raw, ws_k, i * 64)
            unpack(wv_raw, ws_v, i * 64)
            return carry

        lax.fori_loop(0, 4, chunk, 0)

    def track(nrm, name, a):
        n2 = jnp.max(jnp.sum(a * a, axis=1, keepdims=True), axis=0, keepdims=True)
        nrm[name] = mx(nrm.get(name), n2)

    def publish(nrm, base, first):
        for t in range(2):
            for w, name in enumerate(("q", "k")):
                old = jnp.where(first, 0.0, nrm_v[base + t, w])
                nrm_v[base + t, w] = jnp.maximum(old, jnp.broadcast_to(nrm[name, t], (8, 128)))

    def set_bound(h):
        bound_s[0] = jnp.max(nrm_v[h & 3, 0] * nrm_v[h & 3, 1])

    def proj(name, src, sums, w, dst, scale, base, r0, nrm, pm=PM):
        n = w.shape[1]
        top = pl.ds(pl.multiple_of(r0, pm), pm)
        bot = pl.ds(pl.multiple_of(S // 2 + r0, pm), pm)
        m1 = _dot(sums[0, top, :], w[0])
        m2 = _dot(sums[1, top, :], w[1])
        m3 = _dot(src[top, 0:n], w[2])
        m4 = _dot(src[bot, n:], w[3])
        m5 = _dot(sums[2, top, :], w[4])
        m6 = _dot(sums[3, top, :], w[5])
        m7 = _dot(sums[4, top, :], w[6])
        outs = ((0, top, (m1 + m4) + (m7 - m5)), (1, top, m3 + m5),
                (0, bot, m2 + m4), (1, bot, (m1 - m2) + (m3 + m6)))
        for t, rows, val in outs:
            if scale is not None:
                val = val * scale
            if name is not None:
                track(nrm, (name, t), val)
            dst[base + t, rows, :] = val.astype(BF16)

    def proj_steps(base, e, pm=PM):
        steps, nrm = [], {}
        for i in range(S // 4 // pm):
            r0 = e * (S // 4) + i * pm
            for cost, args in ((4, ("q", x_v, xs_v, ws_q, q_v, qscale)),
                               (2, ("k", c_v, cs_v, ws_k, k_v, None)),
                               (2, (None, c_v, cs_v, ws_v, v_v, None))):
                steps.append((7 * cost * pm // 128,
                              functools.partial(proj, *args, base, r0, nrm, pm)))
        steps.append((0, functools.partial(publish, nrm, base, e == 0)))
        return steps

    pending = []

    def out_steps(h, i, st, last, nsplit=NSPLIT):
        rows = slice(i * BQ, (i + 1) * BQ)
        w = M // nsplit

        def step(t):
            cs = slice(t * w, (t + 1) * w)
            o = acc_v[rows, cs] + _dot(st.ctx, wo_v[pl.ds(pl.multiple_of(h * D, D), D), cs])
            acc_v[rows, cs] = o
            if last:
                u_v[rows, cs] = o.astype(BF16)
                if out_copies(i)[t] is not None:
                    out_copies(i)[t].start()

        return [(nsub * w // 128, functools.partial(step, t)) for t in range(nsplit)]

    def fast_tiles(i, st, slot):
        r0 = i * BQ
        ntf = r0 // 128
        lacc = [None] * nsub
        acc = [None] * nsub
        left = [ntf + nsub]
        tiles = []

        def done(n):
            left[0] -= n
            if left[0] == 0:
                l = jnp.sum(jnp.concatenate(lacc, axis=0), axis=1, keepdims=True)
                st.ctx = (jnp.concatenate(acc, axis=0) / l).astype(BF16)

        def add_tile(t, c0, w):
            box = []

            def qk_exp():
                s = _dot_nt(q_v[slot, r0 + t * 128:r0 + BQ, :], k_v[slot, c0:c0 + w * 128, :])
                if c0 >= r0:
                    s0 = jnp.where(tri, s[:128], NEG)
                    s = jnp.concatenate([s0, s[128:]], axis=0) if t < nsub - 1 else s0
                p = jnp.exp2(s)
                for u in range(t, nsub):
                    lacc[u] = addn(lacc[u], functools.reduce(jnp.add, [
                        p[(u - t) * 128:(u - t + 1) * 128, j * 128:(j + 1) * 128]
                        for j in range(w)]))
                box.append(p.astype(BF16))

            def pv():
                o = _dot(box.pop(), v_v[slot, c0:c0 + w * 128, :])
                for u in range(t, nsub):
                    acc[u] = addn(acc[u], o[(u - t) * 128:(u - t + 1) * 128])
                done(w)

            tiles.append((w * (nsub - t), qk_exp, pv))

        kt = 0
        while kt < ntf:
            w = min(KW, ntf - kt)
            add_tile(0, kt * 128, w)
            kt += w
        for t in range(nsub):
            add_tile(t, r0 + t * 128, 1)
        return tiles

    def head_fast(h, slot, proj, last=False):
        sts = [St() for _ in range(nq)]
        order = list(range(nq))[::-1]
        tiles, ends = [], {}
        for i in order:
            tiles += fast_tiles(i, sts[i], slot)
            ends[len(tiles) - 1] = i
        proj = list(proj)
        outs = []
        t = [0.0]
        attn = 2 * sum(c for c, _, _ in tiles)
        fill = sum(c for c, _ in proj) + nq * nsub * (M // 128)
        debt = [0.0]

        def filler(force=False):
            while debt[0] > 0 or force:
                if outs and (outs[0][0] <= t[0] or not proj):
                    _, c, fn = outs.pop(0)
                elif proj:
                    c, fn = proj.pop(0)
                else:
                    return
                fn()
                t[0] += c
                debt[0] -= c

        n = len(tiles)
        for k in range(n + F_LAG):
            c = 0
            if k < n:
                tiles[k][1]()
                c += tiles[k][0]
            if k >= F_LAG:
                tiles[k - F_LAG][2]()
                c += tiles[k - F_LAG][0]
            t[0] += c
            if k - F_LAG in ends:
                i = ends[k - F_LAG]
                outs += [(t[0] + LAG_OUT, cc, fn) for cc, fn in out_steps(h, i, sts[i], last)]
            debt[0] += c * fill / attn * F_FILL
            filler()
        filler(force=True)

    def head_safe(h, slot, last=False):
        rr = lax.broadcasted_iota(jnp.int32, (256, 256), 0)
        cc = lax.broadcasted_iota(jnp.int32, (256, 256), 1)

        def q_block(qi, carry):
            rows = pl.ds(pl.multiple_of(qi * 256, 256), 256)
            q = q_v[slot, rows, :]

            def kv_block(kt, mla):
                m, l, acc = mla
                cols = pl.ds(pl.multiple_of(kt * 256, 256), 256)
                s = _dot_nt(q, k_v[slot, cols, :])
                s = jnp.where(cc + (kt - qi) * 256 <= rr, s, NEG)
                m_new = jnp.maximum(m, jnp.max(s, axis=1, keepdims=True))
                alpha = jnp.exp2(m - m_new)
                p = jnp.exp2(s - m_new)
                l = alpha * l + jnp.sum(p, axis=1, keepdims=True)
                acc = alpha * acc + _dot(p.astype(BF16), v_v[slot, cols, :])
                return m_new, l, acc

            init = (jnp.full((256, 1), NEG, F32), jnp.zeros((256, 1), F32),
                    jnp.zeros((256, D), F32))
            _, l, acc = lax.fori_loop(0, qi + 1, kv_block, init)
            ctx = (acc / l).astype(BF16)
            o = acc_v[rows, :] + _dot(ctx, wo_v[pl.ds(pl.multiple_of(h * D, D), D), :])
            acc_v[rows, :] = o
            if last:
                u_v[rows, :] = o.astype(BF16)
            return carry

        lax.fori_loop(0, S // 256, q_block, 0)

    def out_copies(i):
        rows, w = slice(i * BQ, (i + 1) * BQ), M // NSPLIT
        if i > 0:
            return [None] * (NSPLIT - 1) + [pltpu.make_async_copy(
                u_v.at[rows], out_h.at[rows, 0:M], osems.at[NSPLIT + i])]
        return [pltpu.make_async_copy(u_v.at[rows, t * w:(t + 1) * w],
                                      out_h.at[rows, t * w:(t + 1) * w], osems.at[t])
                for t in range(NSPLIT)]

    def all_out_copies():
        return [c for i in range(nq) for c in out_copies(i) if c is not None]

    def head(h, last=False):
        slot = h & 3
        small = bound_s[0] <= SCORE_LIMIT ** 2

        @pl.when(small)
        def _():
            head_fast(h, slot, [] if last else proj_steps(2 - (h & 2), h & 1), last)
            set_bound(h + 1)

        @pl.when(jnp.logical_not(small))
        def _():
            head_safe(h, slot, last)
            if not last:
                def rows(i, carry):
                    base, r0, nrm = 2 - (h & 2), (h & 1) * (S // 4) + i * 128, {}
                    proj("q", x_v, xs_v, ws_q, q_v, qscale, base, r0, nrm, 128)
                    proj("k", c_v, cs_v, ws_k, k_v, None, base, r0, nrm, 128)
                    proj(None, c_v, cs_v, ws_v, v_v, None, base, r0, nrm, 128)
                    publish(nrm, base, r0 == 0)
                    return carry

                lax.fori_loop(0, S // 4 // 128, rows, 0)
            set_bound(h + 1)
            if last:
                for c in all_out_copies():
                    c.start()

    for a in range(8):
        start(f"xb{a}", xb_h.at[:, a * 128:(a + 1) * 128], xb_v.at[a])
    start("l", l_h, l_v)
    start("gf", gf_h, gf_v)
    for t in range(16):
        start(f"wr{t}", wr_h.at[0:512, t * 128:(t + 1) * 128], wr_v.at[t])
        start(f"wi{t}", wi_h.at[0:512, t * 128:(t + 1) * 128], wi_v.at[t])
    start("wrn", wr_h.at[512:513, :], wrn_v)
    start("win", wi_h.at[512:513, :], win_v)
    start("c", c_h, c_v)
    start("x", x_h, x_v)
    for t in range(3):
        pair_copy(t, 0).start()
    start("wo", wo_h, wo_v)
    s_v[...] = jnp.zeros(s_v.shape, F32)
    for i in range(S // 512):
        start(f"z{i}", s_v, acc_v.at[i * 512:(i + 1) * 512], priority=1)
    wait(*[f"xb{a}" for a in range(8)])

    def fft8(jj, carry):
        for j0 in range(4):
            f1(jj, j0)
        return carry

    lax.fori_loop(0, 2, fft8, 0)
    wait("l", "gf")

    def fwd_quarter(i, carry):
        for t in range(3):
            for u in range(3):
                pair_copy(t, 4 * i + 1 + u).start()
        for q in range(4):
            f23(4 * i + q)
        return carry

    lax.fori_loop(0, 4, fwd_quarter, 0)
    for i in range(3):
        for t in range(3):
            pair_copy(t, 4 * i + 4).start()
    wait(*[f"wr{t}" for t in range(16)], *[f"wi{t}" for t in range(16)], "wrn", "win")
    def mid_quarter(g2, carry):
        mid_group(g2, range(8))
        return carry

    lax.fori_loop(0, 4, mid_quarter, 0)
    mid_nyquist()

    wait("c", "x")
    for t in range(3):
        pair_copy(t, 0).wait()
    split_inputs(x_v, xs_v)
    split_inputs(c_v, cs_v)
    unpack_weights(0)

    def inv_half(jj, carry):
        merge = proj_steps(0, jj, PM0)
        for j0 in range(4):
            part = merge[len(merge) * j0 // 4:len(merge) * (j0 + 1) // 4]
            i32(jj, j0, lambda: [fn() for _, fn in part])
        return carry

    lax.fori_loop(0, 2, inv_half, 0)
    for a in range(8):
        c = pltpu.make_async_copy(xb_v.at[a], out_h.at[:, M + a * 128:M + (a + 1) * 128],
                                  bsems.at[a])
        c.start()
        pending.append(c)

    wait("wo", *[f"z{i}" for i in range(S // 512)])
    set_bound(0)
    def body(h, carry):
        @pl.when((h & 1) == 0)
        def _():
            for t in range(3):
                pair_copy(t, (h >> 1) + 1).wait()
            unpack_weights((h >> 1) + 1)

        head(h)
        return carry

    lax.fori_loop(0, H - 2, body, 0)
    def tail(h, carry):
        @pl.when(h == H - 1)
        def _():
            for c in all_out_copies():
                c.wait()

        head(h, last=True)
        return carry

    lax.fori_loop(H - 2, H, tail, 0)
    for c in pending:
        c.wait()
    for c in all_out_copies():
        c.wait()


@jax.jit
def pallas_concat_heads__compressed_kv_cla__spectral_gfnet__prompt_kernel(
    A_x: jax.Array,
    A_c_kv: jax.Array,
    A_w_q: jax.Array,
    A_w_uk: jax.Array,
    A_w_uv: jax.Array,
    A_w_o: jax.Array,
    B_x: jax.Array,
    B_w_r: jax.Array,
    B_w_i: jax.Array,
):
    vm = pltpu.VMEM
    scratch = [
        vm((S, M), BF16), vm((S, C), BF16),
        vm((5, S // 2, M // 2), BF16), vm((5, S // 2, C // 2), BF16),
        vm((H // 2, M, D), U32), vm((H // 2, C, D), U32), vm((H // 2, C, D), U32),
        vm((H * D, M), BF16),
        vm((7, M // 2, D), BF16), vm((7, C // 2, D), BF16), vm((7, C // 2, D), BF16),
        vm((8, S, 128), BF16),
        vm((16, 512, 128), BF16), vm((16, 512, 128), BF16),
        vm((1, S), BF16), vm((1, S), BF16),
        vm(_L_NP.shape, BF16), vm(_GF_NP.shape, BF16),
        vm((S, 1024), BF16),
        vm((16, KR, 256), F32), vm((16, KR, 256), BF16),
        vm((S, M), F32),
        vm((4, S, D), BF16), vm((4, S, D), BF16), vm((4, S, D), BF16),
        vm((512, M), F32),
        vm((4, 2, 8, 128), F32), pltpu.SMEM((1,), F32),
        pltpu.SemaphoreType.DMA((64,)),
        pltpu.SemaphoreType.DMA((16,)),
        pltpu.SemaphoreType.DMA((3, H // 2)),
        pltpu.SemaphoreType.DMA((8,)),
    ]
    anyspec = pl.BlockSpec(memory_space=pl.ANY)
    out = pl.pallas_call(
        _kernel,
        out_shape=jax.ShapeDtypeStruct((S, M + DB), BF16),
        in_specs=[anyspec] * 11,
        out_specs=anyspec,
        scratch_shapes=scratch,
        compiler_params=pltpu.CompilerParams(vmem_limit_bytes=122 * 1024 * 1024),
        name="mla_gfnet_fused",
    )(
        A_x.reshape(S, M), A_c_kv.reshape(S, C), A_w_q, A_w_uk, A_w_uv,
        A_w_o.reshape(H * D, M),
        B_x.reshape(S, DB), B_w_r.T, B_w_i.T,
        jnp.asarray(_L_NP), jnp.asarray(_GF_NP),
    )
    return out.reshape(1, S, M + DB)
```

```python
import functools
import math

import numpy as np
import jax
import jax.numpy as jnp
from jax import lax
import jax.experimental.pallas as pl
import jax.experimental.pallas.tpu as pltpu

S = 2048
M = 1024
H = 32
D = 128
C = 512
DB = 1024
KR = 528

F32 = jnp.float32
BF16 = jnp.bfloat16
U32 = jnp.uint32
NT = (((1,), (1,)), ((), ()))
NEG = -1e30


def _np_bf16(a):
    return np.asarray(a, np.float32).astype(jnp.bfloat16)


def _make_consts():
    th = 2.0 * np.pi / DB
    b = np.arange(128)[None, :]
    k2 = np.arange(64)[:, None]
    lf = []
    for k1 in (1, 2, 3):
        g = np.exp(-1j * th * b * (k1 + 8 * k2))
        gp = np.exp(-1j * th * b * (8 - k1 + 8 * k2))
        lf.append(np.block([[g.real, -g.imag], [g.imag, g.real],
                            [gp.real, gp.imag], [gp.imag, -gp.real]]))
    g0 = np.exp(-1j * th * b * (8 * k2))
    g4 = np.exp(-1j * th * b * (4 + 8 * k2))
    l0 = np.concatenate([g0.real, g0.imag, np.cos(th * b * 512), np.zeros((127, 128))], 0)
    l4 = np.concatenate([g4.real, g4.imag, np.zeros((128, 128))], 0)
    lf.append(np.concatenate([l0, l4], 1))
    sc = 1.0 / (S * DB)
    bb = np.arange(128)[:, None]
    kk = np.arange(64)[None, :]
    li = []
    for k1 in (1, 2, 3):
        ph, pp = th * bb * (k1 + 8 * kk), th * bb * (8 - k1 + 8 * kk)
        c, s_, cp, sp = np.cos(ph), np.sin(ph), np.cos(pp), np.sin(pp)
        li.append(2 * sc * np.block([[c, -s_, cp, -sp], [s_, c, -sp, -cp]]))
    ph = th * bb * (8 * kk)
    c0, s0 = 2 * np.cos(ph), -2 * np.sin(ph)
    c0[:, 0] = 1.0
    s0[:, 0] = np.cos(th * bb[:, 0] * 512)
    i0 = sc * np.concatenate([c0, s0], 1)
    ph = th * bb * (4 + 8 * kk)
    i4 = sc * np.concatenate([2 * np.cos(ph), -2 * np.sin(ph)], 1)
    li.append(np.concatenate([np.concatenate([i0, i4], 1), np.zeros((128, 256))], 0))
    lmat = np.concatenate(lf + li, axis=0)
    p = np.arange(128)[None, :]
    kp = np.arange(128)[:, None]
    gf = []
    for q in range(16):
        g = np.exp(-2j * np.pi * (16 * p + q) * kp / S)
        gf.append(np.block([[g.real.T, g.imag.T], [-g.imag.T, g.real.T]]))
    return _np_bf16(lmat), _np_bf16(np.concatenate(gf, 0))


_L_NP, _GF_NP = _make_consts()


_dot = functools.partial(jnp.dot, preferred_element_type=F32)
_dot_nt = functools.partial(lax.dot_general, dimension_numbers=NT, preferred_element_type=F32)


def _t(x):
    return None if x is None else (1, x)


def _tneg(a):
    return None if a is None else (-a[0], a[1])


def _tadd(a, b):
    if a is None:
        return b
    if b is None:
        return a
    if a[0] == b[0]:
        return (a[0], a[1] + b[1])
    return (1, a[1] - b[1]) if a[0] > 0 else (1, b[1] - a[1])


def _tsub(a, b):
    return _tadd(a, _tneg(b))


def _tscale(a, c):
    return None if a is None else (1, a[1] * (c * a[0]))


def _tmul(a, v):
    return None if a is None else (a[0], a[1] * v)


def _tval(a):
    return a[1] if a[0] > 0 else -a[1]


def _twiddle(z, e, n, sign):
    re, im = z
    if e == 0:
        return re, im
    if 4 * e == n:
        return (_tneg(im), re) if sign > 0 else (im, _tneg(re))
    c = math.cos(2.0 * math.pi * e / n)
    s = sign * math.sin(2.0 * math.pi * e / n)
    if 8 * e % n == 0:
        r = abs(c)
        rc = re if c > 0 else _tneg(re)
        rs = re if s > 0 else _tneg(re)
        ic = im if c > 0 else _tneg(im)
        is_ = im if s > 0 else _tneg(im)
        return _tscale(_tsub(rc, is_), r), _tscale(_tadd(rs, ic), r)
    return (_tsub(_tscale(re, c), _tscale(im, s)), _tadd(_tscale(re, s), _tscale(im, c)))


def _fft(zs, sign):
    n = len(zs)
    if n == 1:
        return [zs[0]]
    ev = _fft(zs[0::2], sign)
    od = _fft(zs[1::2], sign)
    out = [None] * n
    for k in range(n // 2):
        t = _twiddle(od[k], k, n, sign)
        out[k] = (_tadd(ev[k][0], t[0]), _tadd(ev[k][1], t[1]))
        out[k + n // 2] = (_tsub(ev[k][0], t[0]), _tsub(ev[k][1], t[1]))
    return out


def _irfft8(t0, t4, t1, t2, t3):
    r = math.sqrt(0.5)
    a0, a1 = t0 + t4, t0 - t4
    e0, e2 = a0 + t2[0], a0 - t2[0]
    e1, e3 = a1 - t2[1], a1 + t2[1]
    o0 = t1[0] + t3[0]
    o2 = t3[1] - t1[1]
    u, v = t1[0] - t3[0], t1[1] + t3[1]
    o1, o3 = (u - v) * r, (-u - v) * r
    return [e0 + o0, e1 + o1, e2 + o2, e3 + o3, e0 - o0, e1 - o1, e2 - o2, e3 - o3]


def _lo_half(w):
    return pltpu.bitcast(w << 16, F32)


def _hi_half(w):
    return pltpu.bitcast(w & jnp.uint32(0xFFFF0000), F32)


def _pack_words(lo, hi):
    lo = pltpu.bitcast(lo.astype(BF16).astype(F32), U32)
    hi = pltpu.bitcast(hi.astype(BF16).astype(F32), U32)
    return (lo >> 16) | hi


def _interleave(gens):
    live = list(gens)
    while live:
        nxt = []
        for g in live:
            try:
                next(g)
                nxt.append(g)
            except StopIteration:
                pass
        live = nxt


def _drain(g):
    for _ in g:
        pass


BQ = 512
KW = 2
NSPLIT = 4
PM = 512
PM0 = 128
LAG_OUT = 16
F_LAG = 1
F_FILL = 1.0
SCORE_LIMIT = 60.0


def _kernel(x_h, c_h, wq_h, wk_h, wv_h, wo_h, xb_h, wr_h, wi_h, l_h, gf_h,
            out_h,
            x_v, c_v, xs_v, cs_v, wq_raw, wk_raw, wv_raw, wo_v, ws_q, ws_k, ws_v,
            xb_v, wr_v, wi_v, wrn_v, win_v, l_v, gf_v,
            u_v, y_v, z_v,
            acc_v, q_v, k_v, v_v, s_v, nrm_v, bound_s,
            sems, osems, wsems, bsems):
    cp = {}
    nsem = [0]

    def start(name, src, dst, priority=0):
        c = pltpu.make_async_copy(src, dst, sems.at[nsem[0]])
        nsem[0] += 1
        c.start(priority=priority)
        cp[name] = c

    def wait(*names):
        for nm in names:
            cp[nm].wait()

    wq32, wk32, wv32 = wq_h.bitcast(U32), wk_h.bitcast(U32), wv_h.bitcast(U32)

    def pair_copy(t, j):
        src, dst = ((wq32, wq_raw), (wk32, wk_raw), (wv32, wv_raw))[t]
        return pltpu.make_async_copy(src.at[:, j, :], dst.at[j], wsems.at[t, j])

    xb32 = xb_v.bitcast(U32)
    wr32 = wr_v.bitcast(U32)
    wi32 = wi_v.bitcast(U32)

    def word_rows(a, jj):
        return xb32.at[a, pl.ds(pl.multiple_of(4 * jj, 4), 1020)]

    def f1(jj, j0):
        views = [word_rows(a, jj) for a in range(8)]
        for g in range(8):
            words = [v[pl.ds(128 * g + j0, 16, stride=8), :] for v in views]
            for e in range(2):
                half = _lo_half if e == 0 else _hi_half
                o = _fft([(_t(half(w)), None) for w in words], -1)
                r0 = pl.multiple_of((8 * jj + 2 * j0 + e) * 128 + 16 * g, 16)
                parts = [o[0][0], o[4][0], o[1][0], o[1][1], o[2][0], o[2][1], o[3][0], o[3][1]]
                for t in range(8):
                    u_v[pl.ds(r0, 16), t * 128:(t + 1) * 128] = _tval(parts[t]).astype(BF16)

    def f23(q):
        rows = pl.ds(pl.multiple_of(q * 128, 128), 128)
        o = [_dot_nt(l_v[256 * i:256 * (i + 1), :], u_v[rows, 256 * (i + 1):256 * (i + 2)])
             .astype(BF16) for i in range(3)]
        o0 = _dot_nt(l_v[768:912, 0:128], u_v[rows, 0:128]).astype(BF16)
        o4 = _dot_nt(l_v[768:896, 128:256], u_v[rows, 128:256]).astype(BF16)

        def blk(k1, part):
            if k1 == 0:
                return o0[64 * part:64 * part + 64]
            if k1 == 4:
                return o4[64 * part:64 * part + 64]
            if k1 < 4:
                return o[k1 - 1][64 * part:64 * part + 64]
            return o[7 - k1][128 + 64 * part:128 + 64 * part + 64]

        re = jnp.concatenate([blk(k1, 0) for k1 in range(8)] + [o0[128:144]], axis=0)
        im = jnp.concatenate([blk(k1, 1) for k1 in range(8)] + [jnp.zeros((16, 128), BF16)],
                             axis=0)
        y_v[q] = _dot(jnp.concatenate([re, im], axis=1),
                      gf_v[pl.ds(pl.multiple_of(q * 256, 256), 256), :])

    def mid(rows, filt):
        xf = _fft([(_t(y_v[q, rows, 0:128]), _t(y_v[q, rows, 128:256])) for q in range(16)], -1)
        zs = []
        for kq in range(16):
            fr, fi = filt(kq)
            re, im = xf[kq]
            zs.append((_tsub(_tmul(re, fr), _tmul(im, fi)), _tadd(_tmul(re, fi), _tmul(im, fr))))
        us = _fft(zs, +1)
        for q in range(16):
            z_v[q, rows, 0:128] = _tval(us[q][0]).astype(BF16)
            z_v[q, rows, 128:256] = _tval(us[q][1]).astype(BF16)

    def mid_group(g2, k1s):
        base = pl.multiple_of(64 * g2, 64)
        for k1 in k1s:
            half = _lo_half if k1 % 2 == 0 else _hi_half
            sl = pl.ds(k1 // 2, 16, stride=4)

            def filt(kq):
                return (half(wr32.at[kq, pl.ds(base, 64)][sl, :]),
                        half(wi32.at[kq, pl.ds(base, 64)][sl, :]))

            mid(pl.ds(pl.multiple_of(64 * k1 + 16 * g2, 16), 16), filt)

    def mid_nyquist():
        def filt(kq):
            cs = slice(kq * 128, (kq + 1) * 128)
            return (jnp.broadcast_to(wrn_v[:, cs].astype(F32), (16, 128)),
                    jnp.broadcast_to(win_v[:, cs].astype(F32), (16, 128)))

        mid(slice(512, KR), filt)

    srow = lax.broadcasted_iota(jnp.int32, (64, 128), 0)

    def i32(jj, j0, between):
        ys, zs = [], []
        for e in range(2):
            q = 8 * jj + 2 * j0 + e
            zs.append(_dot_nt(z_v[q], gf_v[pl.ds(pl.multiple_of(q * 256, 256), 256), :]))
        between()
        for z in zs:
            zr, zi = z[:, 0:128], z[:, 128:256]
            zi0 = jnp.where(srow == 0, jnp.broadcast_to(zr[512:513], (64, 128)), zi[0:64])
            rhs0 = jnp.concatenate([zr[0:64], zi0], axis=0).astype(BF16)
            t0 = _dot(l_v[1792:1920, 0:128], rhs0)
            rhs4 = jnp.concatenate([zr[256:320], zi[256:320]], axis=0).astype(BF16)
            t4 = _dot(l_v[1792:1920, 128:256], rhs4)
            ts = []
            for k1 in (1, 2, 3):
                kc = 8 - k1
                rhs = jnp.concatenate([zr[64 * k1:64 * k1 + 64], zi[64 * k1:64 * k1 + 64],
                                       zr[64 * kc:64 * kc + 64], zi[64 * kc:64 * kc + 64]],
                                      axis=0).astype(BF16)
                o = _dot(l_v[1024 + 256 * (k1 - 1):1024 + 256 * k1, :], rhs)
                ts.append((o[0:128], o[128:256]))
            ys.append(_irfft8(t0, t4, *ts))
        for a in range(8):
            word_rows(a, jj)[pl.ds(j0, 128, stride=8), :] = _pack_words(ys[0][a], ys[1][a]).T

    nq = S // BQ
    nsub = BQ // 128
    row = lax.broadcasted_iota(jnp.int32, (128, 128), 0)
    col = lax.broadcasted_iota(jnp.int32, (128, 128), 1)
    tri = col <= row
    qscale = (D ** -0.5) * math.log2(math.e)

    def mx(a, b):
        return b if a is None else jnp.maximum(a, b)

    def addn(a, b):
        return b if a is None else a + b

    class St:
        pass

    def split_inputs(src, dst):
        n = src.shape[1] // 2

        def chunk(i, carry):
            top = pl.ds(pl.multiple_of(i * 64, 64), 64)
            bot = pl.ds(pl.multiple_of(S // 2 + i * 64, 64), 64)
            a11, a12 = src[top, 0:n].astype(F32), src[top, n:].astype(F32)
            a21, a22 = src[bot, 0:n].astype(F32), src[bot, n:].astype(F32)
            for t, v in enumerate((a11 + a22, a21 + a22, a11 + a12, a21 - a11, a12 - a22)):
                dst[t, top, :] = v.astype(BF16)
            return carry

        lax.fori_loop(0, S // 128, chunk, 0)

    def unpack_weights(j):
        def unpack(raw, w, r0):
            n = w.shape[1]
            rows = pl.ds(pl.multiple_of(r0, 64), 64)
            up, dn = raw[j, rows, :], raw[j, pl.ds(pl.multiple_of(n + r0, 64), 64), :]
            b11, b12, b21, b22 = _lo_half(up), _hi_half(up), _lo_half(dn), _hi_half(dn)
            for t, v in enumerate((b11 + b22, b11, b12 - b22, b21 - b11, b22,
                                   b11 + b12, b21 + b22)):
                w[t, rows, :] = v.astype(BF16)

        def chunk(i, carry):
            unpack(wq_raw, ws_q, i * 128)
            unpack(wq_raw, ws_q, i * 128 + 64)
            unpack(wk_raw, ws_k, i * 64)
            unpack(wv_raw, ws_v, i * 64)
            return carry

        lax.fori_loop(0, 4, chunk, 0)

    def track(nrm, name, a):
        n2 = jnp.max(jnp.sum(a * a, axis=1, keepdims=True), axis=0, keepdims=True)
        nrm[name] = mx(nrm.get(name), n2)

    def publish(nrm, base, first):
        for t in range(2):
            for w, name in enumerate(("q", "k")):
                old = jnp.where(first, 0.0, nrm_v[base + t, w])
                nrm_v[base + t, w] = jnp.maximum(old, jnp.broadcast_to(nrm[name, t], (8, 128)))

    def set_bound(h):
        bound_s[0] = jnp.max(nrm_v[h & 3, 0] * nrm_v[h & 3, 1])

    def proj(name, src, sums, w, dst, scale, base, r0, nrm, pm=PM):
        n = w.shape[1]
        top = pl.ds(pl.multiple_of(r0, pm), pm)
        bot = pl.ds(pl.multiple_of(S // 2 + r0, pm), pm)
        m1 = _dot(sums[0, top, :], w[0])
        m2 = _dot(sums[1, top, :], w[1])
        m3 = _dot(src[top, 0:n], w[2])
        m4 = _dot(src[bot, n:], w[3])
        m5 = _dot(sums[2, top, :], w[4])
        m6 = _dot(sums[3, top, :], w[5])
        m7 = _dot(sums[4, top, :], w[6])
        outs = ((0, top, (m1 + m4) + (m7 - m5)), (1, top, m3 + m5),
                (0, bot, m2 + m4), (1, bot, (m1 - m2) + (m3 + m6)))
        for t, rows, val in outs:
            if scale is not None:
                val = val * scale
            if name is not None:
                track(nrm, (name, t), val)
            dst[base + t, rows, :] = val.astype(BF16)

    def proj_steps(base, e, pm=PM):
        steps, nrm = [], {}
        for i in range(S // 4 // pm):
            r0 = e * (S // 4) + i * pm
            for cost, args in ((4, ("q", x_v, xs_v, ws_q, q_v, qscale)),
                               (2, ("k", c_v, cs_v, ws_k, k_v, None)),
                               (2, (None, c_v, cs_v, ws_v, v_v, None))):
                steps.append((7 * cost * pm // 128,
                              functools.partial(proj, *args, base, r0, nrm, pm)))
        steps.append((0, functools.partial(publish, nrm, base, e == 0)))
        return steps

    pending = []

    def out_steps(h, i, st, last, nsplit=NSPLIT):
        rows = slice(i * BQ, (i + 1) * BQ)
        w = M // nsplit

        def step(t):
            cs = slice(t * w, (t + 1) * w)
            o = acc_v[rows, cs] + _dot(st.ctx, wo_v[pl.ds(pl.multiple_of(h * D, D), D), cs])
            acc_v[rows, cs] = o
            if last:
                u_v[rows, cs] = o.astype(BF16)
                if i == 0 or t == nsplit - 1:
                    pl.when(h == H - 1)(lambda: out_copy(i, t).start())

        return [(nsub * w // 128, functools.partial(step, t)) for t in range(nsplit)]

    def fast_tiles(i, st, slot):
        r0 = i * BQ
        ntf = r0 // 128
        lacc = [None] * nsub
        acc = [None] * nsub
        left = [ntf + nsub]
        tiles = []

        def done(n):
            left[0] -= n
            if left[0] == 0:
                l = jnp.sum(jnp.concatenate(lacc, axis=0), axis=1, keepdims=True)
                st.ctx = (jnp.concatenate(acc, axis=0) / l).astype(BF16)

        def add_tile(t, c0, w):
            box = []

            def qk_exp():
                s = _dot_nt(q_v[slot, r0 + t * 128:r0 + BQ, :], k_v[slot, c0:c0 + w * 128, :])
                if c0 >= r0:
                    s0 = jnp.where(tri, s[:128], NEG)
                    s = jnp.concatenate([s0, s[128:]], axis=0) if t < nsub - 1 else s0
                p = jnp.exp2(s)
                for u in range(t, nsub):
                    lacc[u] = addn(lacc[u], functools.reduce(jnp.add, [
                        p[(u - t) * 128:(u - t + 1) * 128, j * 128:(j + 1) * 128]
                        for j in range(w)]))
                box.append(p.astype(BF16))

            def pv():
                o = _dot(box.pop(), v_v[slot, c0:c0 + w * 128, :])
                for u in range(t, nsub):
                    acc[u] = addn(acc[u], o[(u - t) * 128:(u - t + 1) * 128])
                done(w)

            tiles.append((w * (nsub - t), qk_exp, pv))

        kt = 0
        while kt < ntf:
            w = min(KW, ntf - kt)
            add_tile(0, kt * 128, w)
            kt += w
        for t in range(nsub):
            add_tile(t, r0 + t * 128, 1)
        return tiles

    def head_fast(h, slot, proj, last=False):
        sts = [St() for _ in range(nq)]
        order = list(range(nq))[::-1]
        tiles, ends = [], {}
        for i in order:
            tiles += fast_tiles(i, sts[i], slot)
            ends[len(tiles) - 1] = i
        proj = list(proj)
        outs = []
        t = [0.0]
        attn = 2 * sum(c for c, _, _ in tiles)
        fill = sum(c for c, _ in proj) + nq * nsub * (M // 128)
        debt = [0.0]

        def filler(force=False):
            while debt[0] > 0 or force:
                if outs and (outs[0][0] <= t[0] or not proj):
                    _, c, fn = outs.pop(0)
                elif proj:
                    c, fn = proj.pop(0)
                else:
                    return
                fn()
                t[0] += c
                debt[0] -= c

        n = len(tiles)
        for k in range(n + F_LAG):
            c = 0
            if k < n:
                tiles[k][1]()
                c += tiles[k][0]
            if k >= F_LAG:
                tiles[k - F_LAG][2]()
                c += tiles[k - F_LAG][0]
            t[0] += c
            if k - F_LAG in ends:
                i = ends[k - F_LAG]
                outs += [(t[0] + LAG_OUT, cc, fn) for cc, fn in out_steps(h, i, sts[i], last)]
            debt[0] += c * fill / attn * F_FILL
            filler()
        filler(force=True)

    def head_safe(h, slot, last=False):
        rr = lax.broadcasted_iota(jnp.int32, (256, 256), 0)
        cc = lax.broadcasted_iota(jnp.int32, (256, 256), 1)

        def q_block(qi, carry):
            rows = pl.ds(pl.multiple_of(qi * 256, 256), 256)
            q = q_v[slot, rows, :]

            def kv_block(kt, mla):
                m, l, acc = mla
                cols = pl.ds(pl.multiple_of(kt * 256, 256), 256)
                s = _dot_nt(q, k_v[slot, cols, :])
                s = jnp.where(cc + (kt - qi) * 256 <= rr, s, NEG)
                m_new = jnp.maximum(m, jnp.max(s, axis=1, keepdims=True))
                alpha = jnp.exp2(m - m_new)
                p = jnp.exp2(s - m_new)
                l = alpha * l + jnp.sum(p, axis=1, keepdims=True)
                acc = alpha * acc + _dot(p.astype(BF16), v_v[slot, cols, :])
                return m_new, l, acc

            init = (jnp.full((256, 1), NEG, F32), jnp.zeros((256, 1), F32),
                    jnp.zeros((256, D), F32))
            _, l, acc = lax.fori_loop(0, qi + 1, kv_block, init)
            ctx = (acc / l).astype(BF16)
            o = acc_v[rows, :] + _dot(ctx, wo_v[pl.ds(pl.multiple_of(h * D, D), D), :])
            acc_v[rows, :] = o
            if last:
                u_v[rows, :] = o.astype(BF16)
            return carry

        lax.fori_loop(0, S // 256, q_block, 0)

    def out_copy(i, t):
        rows, w = slice(i * BQ, (i + 1) * BQ), M // NSPLIT
        cs = slice(t * w, (t + 1) * w) if i == 0 else slice(0, M)
        return pltpu.make_async_copy(u_v.at[rows, cs], out_h.at[rows, cs],
                                     osems.at[t if i == 0 else NSPLIT + i])

    out_pieces = [(i, t) for i in range(nq) for t in range(NSPLIT) if i == 0 or t == NSPLIT - 1]

    def head(h, last=False):
        slot = h & 3
        small = bound_s[0] <= SCORE_LIMIT ** 2

        @pl.when(small)
        def _():
            head_fast(h, slot, [] if last else proj_steps(2 - (h & 2), h & 1), last)
            set_bound(h + 1)

        @pl.when(jnp.logical_not(small))
        def _():
            head_safe(h, slot, last)
            if not last:
                def rows(i, carry):
                    base, r0, nrm = 2 - (h & 2), (h & 1) * (S // 4) + i * 128, {}
                    proj("q", x_v, xs_v, ws_q, q_v, qscale, base, r0, nrm, 128)
                    proj("k", c_v, cs_v, ws_k, k_v, None, base, r0, nrm, 128)
                    proj(None, c_v, cs_v, ws_v, v_v, None, base, r0, nrm, 128)
                    publish(nrm, base, r0 == 0)
                    return carry

                lax.fori_loop(0, S // 4 // 128, rows, 0)
            set_bound(h + 1)
            if last:
                @pl.when(h == H - 1)
                def _():
                    for it in out_pieces:
                        out_copy(*it).start()

    for a in range(8):
        start(f"xb{a}", xb_h.at[:, a * 128:(a + 1) * 128], xb_v.at[a])
    start("l", l_h, l_v)
    start("gf", gf_h, gf_v)
    for t in range(16):
        start(f"wr{t}", wr_h.at[0:512, t * 128:(t + 1) * 128], wr_v.at[t])
        start(f"wi{t}", wi_h.at[0:512, t * 128:(t + 1) * 128], wi_v.at[t])
    start("wrn", wr_h.at[512:513, :], wrn_v)
    start("win", wi_h.at[512:513, :], win_v)
    start("c", c_h, c_v)
    start("x", x_h, x_v)
    for t in range(3):
        pair_copy(t, 0).start()
    start("wo", wo_h, wo_v)
    s_v[...] = jnp.zeros(s_v.shape, F32)
    for i in range(S // 512):
        start(f"z{i}", s_v, acc_v.at[i * 512:(i + 1) * 512], priority=1)
    wait(*[f"xb{a}" for a in range(8)])

    def fft8(jj, carry):
        for j0 in range(4):
            f1(jj, j0)
        return carry

    lax.fori_loop(0, 2, fft8, 0)
    wait("l", "gf")

    def fwd_quarter(i, carry):
        for t in range(3):
            for u in range(3):
                pair_copy(t, 4 * i + 1 + u).start()
        for q in range(4):
            f23(4 * i + q)
        return carry

    lax.fori_loop(0, 4, fwd_quarter, 0)
    for i in range(3):
        for t in range(3):
            pair_copy(t, 4 * i + 4).start()
    wait(*[f"wr{t}" for t in range(16)], *[f"wi{t}" for t in range(16)], "wrn", "win")
    def mid_quarter(g2, carry):
        mid_group(g2, range(8))
        return carry

    lax.fori_loop(0, 4, mid_quarter, 0)
    mid_nyquist()

    wait("c", "x")
    for t in range(3):
        pair_copy(t, 0).wait()
    split_inputs(x_v, xs_v)
    split_inputs(c_v, cs_v)
    unpack_weights(0)

    def inv_half(jj, carry):
        merge = proj_steps(0, jj, PM0)
        for j0 in range(4):
            part = merge[len(merge) * j0 // 4:len(merge) * (j0 + 1) // 4]
            i32(jj, j0, lambda: [fn() for _, fn in part])
        return carry

    lax.fori_loop(0, 2, inv_half, 0)
    for a in range(8):
        c = pltpu.make_async_copy(xb_v.at[a], out_h.at[:, M + a * 128:M + (a + 1) * 128],
                                  bsems.at[a])
        c.start()
        pending.append(c)

    wait("wo", *[f"z{i}" for i in range(S // 512)])
    set_bound(0)
    def body(h, carry):
        @pl.when((h & 1) == 0)
        def _():
            for t in range(3):
                pair_copy(t, (h >> 1) + 1).wait()
            unpack_weights((h >> 1) + 1)

        head(h)
        return carry

    lax.fori_loop(0, H - 2, body, 0)
    def tail(h, carry):
        head(h, last=True)
        return carry

    lax.fori_loop(H - 2, H, tail, 0)
    for c in pending:
        c.wait()
    for it in out_pieces:
        out_copy(*it).wait()


@jax.jit
def pallas_concat_heads__compressed_kv_cla__spectral_gfnet__prompt_kernel(
    A_x: jax.Array,
    A_c_kv: jax.Array,
    A_w_q: jax.Array,
    A_w_uk: jax.Array,
    A_w_uv: jax.Array,
    A_w_o: jax.Array,
    B_x: jax.Array,
    B_w_r: jax.Array,
    B_w_i: jax.Array,
):
    vm = pltpu.VMEM
    scratch = [
        vm((S, M), BF16), vm((S, C), BF16),
        vm((5, S // 2, M // 2), BF16), vm((5, S // 2, C // 2), BF16),
        vm((H // 2, M, D), U32), vm((H // 2, C, D), U32), vm((H // 2, C, D), U32),
        vm((H * D, M), BF16),
        vm((7, M // 2, D), BF16), vm((7, C // 2, D), BF16), vm((7, C // 2, D), BF16),
        vm((8, S, 128), BF16),
        vm((16, 512, 128), BF16), vm((16, 512, 128), BF16),
        vm((1, S), BF16), vm((1, S), BF16),
        vm(_L_NP.shape, BF16), vm(_GF_NP.shape, BF16),
        vm((S, 1024), BF16),
        vm((16, KR, 256), F32), vm((16, KR, 256), BF16),
        vm((S, M), F32),
        vm((4, S, D), BF16), vm((4, S, D), BF16), vm((4, S, D), BF16),
        vm((512, M), F32),
        vm((4, 2, 8, 128), F32), pltpu.SMEM((1,), F32),
        pltpu.SemaphoreType.DMA((64,)),
        pltpu.SemaphoreType.DMA((16,)),
        pltpu.SemaphoreType.DMA((3, H // 2)),
        pltpu.SemaphoreType.DMA((8,)),
    ]
    anyspec = pl.BlockSpec(memory_space=pl.ANY)
    out = pl.pallas_call(
        _kernel,
        out_shape=jax.ShapeDtypeStruct((S, M + DB), BF16),
        in_specs=[anyspec] * 11,
        out_specs=anyspec,
        scratch_shapes=scratch,
        compiler_params=pltpu.CompilerParams(vmem_limit_bytes=122 * 1024 * 1024),
        name="mla_gfnet_fused",
    )(
        A_x.reshape(S, M), A_c_kv.reshape(S, C), A_w_q, A_w_uk, A_w_uv,
        A_w_o.reshape(H * D, M),
        B_x.reshape(S, DB), B_w_r.T, B_w_i.T,
        jnp.asarray(_L_NP), jnp.asarray(_GF_NP),
    )
    return out.reshape(1, S, M + DB)
```
